```python
import jax
import jax.numpy as jnp

def _softmax(x, axis=-1):
    return jax.nn.softmax(x, axis=axis)
def _gelu(x):
    return jax.nn.gelu(x, approximate=True)
def _silu(x):
    return jax.nn.silu(x)
def _sigmoid(x):
    return jax.nn.sigmoid(x)
def _layernorm(x, axis=-1, eps=1e-5):
    m = jnp.mean(x, axis=axis, keepdims=True)
    v = jnp.var(x, axis=axis, keepdims=True)
    return (x - m) / jnp.sqrt(v + eps)
def _scatter_add(tgt, idx, src, axis=0):
    return tgt.at[idx].add(src)
def _segment_sum(src, seg, n):
    return jax.ops.segment_sum(src, seg, n)
class _Rng:
    def __init__(self, key):
        self._k = key
    def _next(self):
        self._k, sub = jax.random.split(self._k)
        return sub
    def normal(self, shape):
        return jax.random.normal(self._next(), shape, dtype=jnp.bfloat16)
    def randint(self, lo, hi, shape):
        return jax.random.randint(self._next(), shape, lo, hi, dtype=jnp.int32)
    def uniform(self, shape, lo=0.0, hi=1.0):
        return jax.random.uniform(self._next(), shape, jnp.bfloat16, lo, hi)
    def permutation(self, n):
        return jax.random.permutation(self._next(), n)


kernel_name = 'concat_heads__sliding_local_dilated__compressed_kv_cla__prompt'

def setup_inputs():
    _rng = _Rng(jax.random.key(int.from_bytes(__import__("os").urandom(4), "little")))
    _w = (lambda a: (lambda t: t.astype(jnp.bfloat16) if jnp.issubdtype(t.dtype, jnp.floating) else t)(jnp.asarray(a)))
    def _A_setup():
        B, S, D = 1, 2048, 1024
        return {
            "x": _w((lambda *s: _rng.normal(s) * 0.05)(B, S, D)),
            "wqkv": _w((lambda *s: _rng.normal(s) * 0.05)(D, 3 * D)),
            "wo": _w((lambda *s: _rng.normal(s) * 0.05)(D, D)),
        }
    _A_in = _A_setup()

    def _B_setup():
        B, H, Sq, Sk, D, M = 1, 32, 2048, 2048, 128, 1024
        Dc = 4 * D
        return {
            "x": _w((lambda *s: _rng.normal(s) * 0.05)(B, Sq, M)),
            "c_kv": _w((lambda *s: _rng.normal(s) * 0.05)(B, Sk, Dc)),
            "w_q": _w((lambda *s: _rng.normal(s) * 0.05)(M, H, D) * (M ** -0.5)),
            "w_uk": _w((lambda *s: _rng.normal(s) * 0.05)(Dc, H, D) * (Dc ** -0.5)),
            "w_uv": _w((lambda *s: _rng.normal(s) * 0.05)(Dc, H, D) * (Dc ** -0.5)),
            "w_o": _w((lambda *s: _rng.normal(s) * 0.05)(H, D, M) * ((H * D) ** -0.5)),
        }
    _B_in = _B_setup()

    return {
        "A_x": _A_in["x"],
        "A_wqkv": _A_in["wqkv"],
        "A_wo": _A_in["wo"],
        "B_x": _B_in["x"],
        "B_c_kv": _B_in["c_kv"],
        "B_w_q": _B_in["w_q"],
        "B_w_uk": _B_in["w_uk"],
        "B_w_uv": _B_in["w_uv"],
        "B_w_o": _B_in["w_o"],
    }

def reference(A_x, A_wqkv, A_wo, B_x, B_c_kv, B_w_q, B_w_uk, B_w_uv, B_w_o):
    def _A_ref(x, wqkv, wo):
        B, S, D = x.shape
        H = 32; Dh = D // H
        W, dil = 8, 2
        qkv = (lambda x, *d: x.transpose(*d))((x @ wqkv).reshape(B, S, 3, H, Dh), 2, 0, 3, 1, 4)
        q, k, v = qkv[0], qkv[1], qkv[2]
        scale = Dh ** -0.5
        pos = jnp.arange(S)
        off = jnp.arange(W) * dil
        idx = pos[:, None] - off[None, :]
        mask = idx >= 0
        idx_c = jnp.where(mask, idx, 0).reshape(-1)
        kg = k[:, :, idx_c, :].reshape(B, H, S, W, Dh)
        vg = v[:, :, idx_c, :].reshape(B, H, S, W, Dh)
        logits = jnp.einsum("bhsd,bhswd->bhsw", q, kg) * scale
        logits = jnp.where(mask[None, None, :, :], logits, -1e9)
        attn = _softmax(logits, axis=-1)
        o = jnp.einsum("bhsw,bhswd->bhsd", attn, vg)
        return (lambda x, *d: x.transpose(*d))(o, 0, 2, 1, 3).reshape(B, S, D) @ wo

    def _B_ref(x, c_kv, w_q, w_uk, w_uv, w_o):
        B, Sq, M = x.shape[0], x.shape[1], x.shape[2]
        Sk = c_kv.shape[1]
        H, D = w_q.shape[1], w_q.shape[2]
        q = jnp.einsum("bqm,mhd->bhqd", x, w_q)
        k = jnp.einsum("bkc,chd->bhkd", c_kv, w_uk)
        v = jnp.einsum("bkc,chd->bhkd", c_kv, w_uv)
        scores = jnp.einsum("bhqd,bhkd->bhqk", q, k) * (D ** -0.5)
        off = Sk - Sq
        qi = jnp.arange(Sq)[:, None]
        kj = jnp.arange(Sk)[None, :]
        cmask = kj <= (qi + off)
        scores = jnp.where(cmask[None, None], scores, -1e9)
        p = _softmax(scores, axis=-1)
        ctx = jnp.einsum("bhqk,bhkd->bhqd", p, v)
        return jnp.einsum("bhqd,hdm->bqm", ctx, w_o)

    a = _A_ref(A_x, A_wqkv, A_wo)
    b = _B_ref(B_x, B_c_kv, B_w_q, B_w_uk, B_w_uv, B_w_o)
    return jnp.concatenate([a, b], axis=-1)
```

```python
import numpy as np

import jax
import jax.numpy as jnp
from jax import lax
import jax.experimental.pallas as pl
import jax.experimental.pallas.tpu as pltpu

F32, BF16, U32 = jnp.float32, jnp.bfloat16, jnp.uint32
LOG2E = float(np.log2(np.e))
NEG = -1e9 * LOG2E
T = 128

S = 2048
DM = 1024
DC = 512
HB = 32
WIN, DIL, DH_A = 8, 2, 32
HALO = 16
PITCH = 17

CFG = dict(la=1, lo=1, nlate=2, tie_gap=4)


def _mm(a, b):
    return jnp.dot(a, b, preferred_element_type=F32)


def _mm_nt(a, b):
    return lax.dot_general(a, b, (((1,), (1,)), ((), ())), preferred_element_type=F32)


def _cat(xs, axis):
    xs = list(xs)
    return xs[0] if len(xs) == 1 else jnp.concatenate(xs, axis)


def _fold(op, xs):
    xs = list(xs)
    acc = xs[0]
    for x in xs[1:]:
        acc = op(acc, x)
    return acc


def _bf(words):
    return pltpu.bitcast(words, BF16)


def _words(x):
    return pltpu.bitcast(x, U32)


def _quads(g, n):
    h = n // 2
    return [{(r, c): g[(r + i * h, c + j * h)] for r in range(h) for c in range(h)}
            for i in range(2) for j in range(2)]


def _gadd(x, y):
    return {k: x[k] + y[k] for k in x}


def _gsub(x, y):
    return {k: x[k] - y[k] for k in x}


def _lhs_operands(g, n):
    if n == 1:
        return [g[(0, 0)]]
    a11, a12, a21, a22 = _quads(g, n)
    parts = [_gadd(a21, a22), a22, _gadd(a11, a12), a11, _gadd(a11, a22), _gsub(a21, a11), _gsub(a12, a22)]
    return [x for p in parts for x in _lhs_operands(p, n // 2)]


def _rhs_operands(g, n):
    if n == 1:
        return [g[(0, 0)]]
    b11, b12, b21, b22 = _quads(g, n)
    parts = [b11, _gsub(b21, b11), b22, _gsub(b12, b22), _gadd(b11, b22), _gadd(b11, b12), _gadd(b21, b22)]
    return [x for p in parts for x in _rhs_operands(p, n // 2)]


def _combine(product, n, base=0):
    if n == 1:
        return {(0, 0): product(base)}
    h = n // 2
    step = 7 ** (h.bit_length() - 1)
    sub = lambda i: _combine(product, h, base + i * step)
    m2 = sub(0)
    m4 = sub(1)
    c21 = _gadd(m2, m4)
    m5 = sub(2)
    u = _gsub(m4, m5)
    m3 = sub(3)
    c12 = _gadd(m3, m5)
    t = _gsub(m3, m2)
    m1 = sub(4)
    t = _gadd(t, m1)
    u = _gadd(u, m1)
    c22 = _gadd(t, sub(5))
    c11 = _gadd(u, sub(6))
    out = {}
    for (i, j), q in (((0, 0), c11), ((0, 1), c12), ((1, 0), c21), ((1, 1), c22)):
        for (r, c), v in q.items():
            out[(r + i * h, c + j * h)] = v
    return out


def _swap_tile_and_lane_bits(tiles):
    lane = lax.broadcasted_iota(jnp.int32, tiles[0].shape, 1)
    for b in range(3):
        s = 4 << b
        low = (lane & s) == 0
        nxt = list(tiles)
        for j in range(8):
            if not j & (1 << b):
                x, y = tiles[j], tiles[j | (1 << b)]
                nxt[j] = jnp.where(low, x, pltpu.roll(y, s, 1))
                nxt[j | (1 << b)] = jnp.where(low, pltpu.roll(x, T - s, 1), y)
        tiles = nxt
    return tiles


class _Background:
    def __init__(self, never, gap):
        self.never, self.gap = never, gap
        self.todo, self.clock, self.last = [], 0, 0

    def tick(self, n):
        self.clock += n

    def attach(self, words):
        k = min(8, len(self.todo), (self.clock - self.last) // self.gap)
        if k <= 0:
            return words
        self.last = self.clock
        parts = [words[: 64 - 8 * k]] if k < 8 else []
        for i in range(8 - k, 8):
            outs = self.todo.pop(0)()
            dep = _fold(lambda a, b: a | b, [o[r:r + 8] for o in outs for r in range(0, o.shape[0], 8)])
            parts.append(jnp.where(self.never, dep, words[8 * i: 8 * i + 8]))
        return _cat(parts, 0)

    def flush(self):
        while self.todo:
            self.todo.pop(0)()


def _weight_operands(tile_words, n, kt):
    ops = []
    for t in range(kt):
        raw = {(r, c): tile_words(r * kt + t, c) for r in range(n) for c in range(n)}
        f = {k: _bf(v).astype(F32) for k, v in raw.items()}
        plain = {id(v): raw[k] for k, v in f.items()}
        ops.append([plain.get(id(x), x) for x in _rhs_operands(f, n)])
    return [[ops[t][i] for t in range(kt)] for i in range(len(ops[0]))]


def _weight_value(tiles, bg=None):
    if tiles[0].dtype == U32:
        if bg is not None:
            tiles = [bg.attach(x) for x in tiles]
        return _bf(_cat(tiles, 0))
    return _cat(tiles, 0).astype(BF16)


def _phase_a(cfg, xa, wqkv, woa, kbuf, vbuf, outa, bg, wait_qv, wait_rest):
    n = 1 << cfg["la"]
    rows = n * T
    kt = DM // T // n
    nchunks = S // rows
    scale = float(DH_A ** -0.5) * LOG2E

    wcache = {}

    def qkv_words(sec, k_tile):
        if (sec, k_tile) not in wcache:
            raw = [_words(wqkv[k_tile * T:(k_tile + 1) * T, (sec * 8 + j) * T:(sec * 8 + j + 1) * T])
                   for j in range(8)]
            wcache[(sec, k_tile)] = _swap_tile_and_lane_bits(raw)
        return wcache[(sec, k_tile)]

    wops = {}

    def qkv_ops(sec, g):
        if (sec, g) not in wops:
            wops[(sec, g)] = _weight_operands(lambda k_tile, c: qkv_words(sec, k_tile)[g * n + c], n, kt)
        return wops[(sec, g)]

    def out_ops(g):
        if ("o", g) not in wops:
            wops[("o", g)] = _weight_operands(
                lambda k_tile, c: _words(woa[k_tile * T:(k_tile + 1) * T, (g * n + c) * T:(g * n + c + 1) * T]),
                n, kt)
        return wops[("o", g)]

    def product(lhs, ops):
        def run(i):
            bg.tick(kt)
            return _mm(lhs[i], _weight_value(ops[i], bg))
        return run

    xops = {}

    def project(c, sec):
        if c not in xops:
            g = {(r, h): xa[c * rows + r * T: c * rows + (r + 1) * T, h * kt * T:(h + 1) * kt * T].astype(F32)
                 for r in range(n) for h in range(n)}
            xops[c] = [x.astype(BF16) for x in _lhs_operands(g, n)]
        res = {}
        for g in range(8 // n):
            for (r, col), val in _combine(product(xops[c], qkv_ops(sec, g)), n).items():
                res[(r, g * n + col)] = val
        if sec == 0:
            return res
        buf = kbuf if sec == 1 else vbuf
        for (r, j), val in res.items():
            buf[c % 2, j, HALO + r * T: HALO + (r + 1) * T, :] = val
            if r == n - 1 and c + 1 < nchunks:
                buf[(c + 1) % 2, j, 0:HALO, :] = val[T - HALO:]
        return None

    lane = lax.broadcasted_iota(jnp.int32, (T, T), 1)
    row = lax.broadcasted_iota(jnp.int32, (T, T), 0)

    def probs(c, q):
        out = []
        for r in range(n):
            logits = []
            for w in range(WIN):
                lo = HALO + r * T - DIL * w
                x = _fold(jnp.add, [q[(r, j)] * kbuf[c % 2, j, lo:lo + T, :] for j in range(8)])
                for s in (1, 2):
                    x = x + jnp.where((lane & s) == 0, pltpu.roll(x, T - s, 1), pltpu.roll(x, s, 1))
                x = x * scale
                if c == 0 and r == 0 and w:
                    x = jnp.where(row >= DIL * w, x, NEG)
                logits.append(x)
            m = _fold(jnp.maximum, logits)
            e = [jnp.exp2(x - m) for x in logits]
            inv = 1.0 / _fold(jnp.add, e)
            out.append([x * inv for x in e])
        return out

    def mix(c, p):
        o = {}
        for r in range(n):
            tiles = []
            for j in range(8):
                tiles.append(_fold(jnp.add, [
                    p[r][w] * vbuf[c % 2, j, HALO + r * T - DIL * w: HALO + (r + 1) * T - DIL * w, :]
                    for w in range(WIN)]))
            tiles = _swap_tile_and_lane_bits(tiles)
            for h in range(n):
                o[(r, h)] = _cat(tiles[h * kt:(h + 1) * kt], 1)
        return [x.astype(BF16) for x in _lhs_operands(o, n)]

    def out_project(c, lhs):
        for g in range(8 // n):
            for (r, col), val in _combine(product(lhs, out_ops(g)), n).items():
                outa[c * rows + r * T: c * rows + (r + 1) * T, (g * n + col) * T:(g * n + col + 1) * T] = (
                    val.astype(BF16))

    pending = None
    for c in range(nchunks):
        project(c, 1)
        if c == 0:
            wait_qv()
        q = project(c, 0)
        p = probs(c, q)
        project(c, 2)
        if c == 0:
            wait_rest()
        if pending is not None:
            out_project(*pending)
        pending = (c, mix(c, p))
    out_project(*pending)


def _schedule_b(nlate):
    ops = []
    for j in range(nlate + 1):
        ops += [("p", j, "k"), ("p", j, "v")]
    ops.append(("p", nlate, "q"))
    units = [(h, 2 * j + b) for j in range(nlate, 8) for b in range(2) for h in range(2)]
    for idx, (h, i) in enumerate(units):
        ops.append(("s", h, i))
        if i // 2 + 1 < 8 and idx % 4 < 3:
            ops.append(("p", i // 2 + 1, "kqv"[idx % 4]))
        if idx:
            ops.append(("o", *units[idx - 1]))
    rest = [("o", *units[-1])]
    for j in range(nlate):
        ops.append(("p", j, "q"))
        ops += rest
        late = [(h, 2 * j + b) for b in range(2) for h in range(2)]
        ops += [("s", *u) for u in late]
        rest = [("o", *u) for u in late]
    return ops + rest


def _pair_body(cfg, p, xops, cops, stq, stk, stv, ctx):
    def weights(st, width):
        w = [st[pl.ds(p + half * (width // 2) * PITCH, width // 2, stride=PITCH), :] for half in range(2)]
        g = {}
        for half in range(2):
            g[(half, 0)] = pltpu.bitcast(w[half] << 16, F32)
            g[(half, 1)] = pltpu.bitcast(w[half] & np.uint32(0xFFFF0000), F32)
        return [x.astype(BF16) for x in _rhs_operands(g, 2)]

    wts = {"k": weights(stk, DC), "q": weights(stq, DM), "v": weights(stv, DC)}
    res = {"q": {}, "k": {}, "v": {}}
    q, k, v = res["q"], res["k"], res["v"]

    def project(j, name):
        src = xops if name == "q" else cops
        out = _combine(lambda i: _mm(_bf(src[i, j * 64:(j + 1) * 64, :]), wts[name][i]), 2)
        for (r, h), val in out.items():
            res[name][(h, 2 * j + r)] = val * (float(T ** -0.5) * LOG2E) if name == "q" else val

    causal = lax.broadcasted_iota(jnp.int32, (T, T), 1) <= lax.broadcasted_iota(jnp.int32, (T, T), 0)

    def scores(h, i):
        s = _mm_nt(q[(h, i)].astype(BF16), _cat([k[(h, t)] for t in range(i + 1)], 0).astype(BF16))
        s = [s[:, t * T:(t + 1) * T] for t in range(i + 1)]
        s[i] = jnp.where(causal, s[i], NEG)
        return s, jnp.max(_fold(jnp.maximum, s), axis=1, keepdims=True)

    def attend(h, i, s, m):
        e = [jnp.exp2(x - m) for x in s]
        acc = _mm(_cat(e, 1).astype(BF16), _cat([v[(h, t)] for t in range(i + 1)], 0).astype(BF16))
        ctx[i, 2 * p + h] = acc * (1.0 / jnp.sum(_fold(jnp.add, e), axis=1, keepdims=True))

    live = {}
    for kind, *arg in _schedule_b(cfg["nlate"]):
        if kind == "p":
            project(*arg)
        elif kind == "s":
            live[tuple(arg)] = scores(*arg)
        else:
            attend(*arg, *live.pop(tuple(arg)))


def _out_chunk(cfg, c, ctx, wob, stage):
    n = 1 << cfg["lo"]
    kt = HB // n
    g = {(r, h): _cat([ctx[c * n + r, h * kt + t] for t in range(kt)], 1) for r in range(n) for h in range(n)}
    lhs = [x.astype(BF16) for x in _lhs_operands(g, n)]
    for grp in range(8 // n):
        ops = _weight_operands(
            lambda k_tile, col: _words(wob[k_tile * T:(k_tile + 1) * T, (grp * n + col) * T:(grp * n + col + 1) * T]),
            n, kt)
        out = _combine(lambda i: _mm(lhs[i], _weight_value(ops[i])), n)
        for (r, col), val in out.items():
            stage[r * T:(r + 1) * T, (grp * n + col) * T:(grp * n + col + 1) * T] = val.astype(BF16)


def _kernel(cfg, xa_h, wqkv_h, woa_h, xb_h, ckv_h, wq_h, wuk_h, wuv_h, wob_h, out_h,
            xops, cops, stq, stk, stv, outa, flag, sems):
    rows_a = (1 << cfg["la"]) * T
    rows_o = (1 << cfg["lo"]) * T
    copy_a = pltpu.make_async_copy(outa, out_h.at[:, pl.ds(0, DM)], sems.at[0])

    def first(xa, wqkv, woa, xb, ckv, wq, wuk, wuv, kbuf, vbuf):
        def cols(sec):
            return pltpu.make_async_copy(wqkv_h.at[:, pl.ds(sec * DM, DM)], wqkv.at[:, pl.ds(sec * DM, DM)],
                                         sems.at[1 + sec])
        head = [pltpu.make_async_copy(xa_h.at[pl.ds(0, rows_a)], xa.at[pl.ds(0, rows_a)], sems.at[4]), cols(1)]
        qv = [cols(0), cols(2)]
        rest = [pltpu.make_async_copy(xa_h.at[pl.ds(rows_a, S - rows_a)], xa.at[pl.ds(rows_a, S - rows_a)],
                                      sems.at[5])]
        rest += [pltpu.make_async_copy(src, dst, sems.at[6 + i]) for i, (src, dst) in enumerate(
            [(woa_h, woa), (wuk_h, wuk), (wuv_h, wuv), (wq_h, wq), (ckv_h, ckv), (xb_h, xb)])]
        flag[0] = 0
        kbuf[0, :, 0:HALO, :] = jnp.zeros((8, HALO, T), F32)
        vbuf[0, :, 0:HALO, :] = jnp.zeros((8, HALO, T), F32)
        for cp in head:
            cp.start()
        for cp in head:
            cp.wait()
        for cp in qv:
            cp.start()

        bg = _Background(flag[0] != 0, cfg["tie_gap"])

        def stage_rows(raw, st, m0, count):
            def run():
                w = _words(raw[m0 * HB:(m0 + count) * HB, :])
                for i in range(count):
                    st[(m0 + i) * PITCH:(m0 + i) * PITCH + 16, :] = w[i * 16:(i + 1) * 16]
                return [w]
            return run

        def activation_operands(src, dst, width, j, r0):
            def run():
                half = width // 2
                g = {(r, h): src[(2 * j + r) * T + r0:(2 * j + r) * T + r0 + 16, h * half:(h + 1) * half].astype(F32)
                     for r in range(2) for h in range(2)}
                outs = [_words(x.astype(BF16)) for x in _lhs_operands(g, 2)]
                for i, x in enumerate(outs):
                    dst[i, j * 64 + r0 // 2:j * 64 + r0 // 2 + 8, :] = x
                return [x[:, t * T:(t + 1) * T] for x in outs for t in range(half // T)]
            return run

        def wait_qv():
            for cp in qv:
                cp.wait()
            for cp in rest:
                cp.start()

        def wait_rest():
            for cp in rest:
                cp.wait()
            for raw, st, width in ((wuk, stk, DC), (wuv, stv, DC), (wq, stq, DM)):
                bg.todo += [stage_rows(raw, st, m0, 8) for m0 in range(0, width, 8)]
            for src, dst, width in ((ckv, cops, DC), (xb, xops, DM)):
                bg.todo += [activation_operands(src, dst, width, j, r0) for j in range(8) for r0 in range(0, T, 16)]
            bg.last = bg.clock

        _phase_a(cfg, xa, wqkv, woa, kbuf, vbuf, outa, bg, wait_qv, wait_rest)
        bg.flush()

    pl.run_scoped(
        first,
        pltpu.VMEM((S, DM), BF16), pltpu.VMEM((DM, 3 * DM), BF16), pltpu.VMEM((DM, DM), BF16),
        pltpu.VMEM((S, DM), BF16), pltpu.VMEM((S, DC), BF16),
        pltpu.VMEM((DM * HB, T), BF16), pltpu.VMEM((DC * HB, T), BF16), pltpu.VMEM((DC * HB, T), BF16),
        pltpu.VMEM((2, 8, HALO + rows_a, T), F32), pltpu.VMEM((2, 8, HALO + rows_a, T), F32))

    def second(ctx, wob, stage):
        load_wo = pltpu.make_async_copy(wob_h, wob, sems.at[1])
        copy_a.start()
        load_wo.start()

        def pair(p, carry):
            _pair_body(cfg, p, xops, cops, stq, stk, stv, ctx)
            return carry
        lax.fori_loop(0, HB // 2, pair, 0)

        copy_a.wait()
        load_wo.wait()
        nchunks = S // rows_o

        def store(c):
            return pltpu.make_async_copy(
                stage.at[c % 2], out_h.at[pl.ds(pl.multiple_of(c * rows_o, rows_o), rows_o), pl.ds(DM, DM)],
                sems.at[2 + c % 2])

        def chunk(c, carry):
            @pl.when(c >= 2)
            def _():
                store(c - 2).wait()
            _out_chunk(cfg, c, ctx, wob, stage.at[c % 2])
            store(c).start()
            return carry
        lax.fori_loop(0, nchunks, chunk, 0)
        store(nchunks - 2).wait()
        store(nchunks - 1).wait()

    pl.run_scoped(second, pltpu.VMEM((S // T, HB, T, T), F32), pltpu.VMEM((HB * T, DM), BF16),
                  pltpu.VMEM((2, rows_o, DM), BF16))


def _call(cfg, A_x, A_wqkv, A_wo, B_x, B_c_kv, B_w_q, B_w_uk, B_w_uv, B_w_o):
    any_spec = pl.BlockSpec(memory_space=pl.ANY)
    out = pl.pallas_call(
        lambda *refs: _kernel(cfg, *refs),
        out_shape=jax.ShapeDtypeStruct((S, 2 * DM), BF16),
        in_specs=[any_spec] * 9,
        out_specs=any_spec,
        scratch_shapes=[
            pltpu.VMEM((7, S // 4, DM // 2), U32),
            pltpu.VMEM((7, S // 4, DC // 2), U32),
            pltpu.VMEM((DM * PITCH, T), U32),
            pltpu.VMEM((DC * PITCH, T), U32),
            pltpu.VMEM((DC * PITCH, T), U32),
            pltpu.VMEM((S, DM), BF16),
            pltpu.SMEM((1,), jnp.int32),
            pltpu.SemaphoreType.DMA((12,)),
        ],
        compiler_params=pltpu.CompilerParams(vmem_limit_bytes=124 * 1024 * 1024),
        name="concat_heads",
    )(A_x.reshape(S, DM), A_wqkv, A_wo, B_x.reshape(S, DM), B_c_kv.reshape(S, DC),
      B_w_q.reshape(DM * HB, T), B_w_uk.reshape(DC * HB, T), B_w_uv.reshape(DC * HB, T),
      B_w_o.reshape(HB * T, DM))
    return out.reshape(1, S, 2 * DM)


@jax.jit
def pallas_concat_heads__sliding_local_dilated__compressed_kv_cla__prompt_kernel(
    A_x: jax.Array,
    A_wqkv: jax.Array,
    A_wo: jax.Array,
    B_x: jax.Array,
    B_c_kv: jax.Array,
    B_w_q: jax.Array,
    B_w_uk: jax.Array,
    B_w_uv: jax.Array,
    B_w_o: jax.Array,
):
    return _call(CFG, A_x, A_wqkv, A_wo, B_x, B_c_kv, B_w_q, B_w_uk, B_w_uv, B_w_o)
```

```python
import numpy as np

import jax
import jax.numpy as jnp
from jax import lax
import jax.experimental.pallas as pl
import jax.experimental.pallas.tpu as pltpu

F32, BF16, U32 = jnp.float32, jnp.bfloat16, jnp.uint32
LOG2E = float(np.log2(np.e))
NEG = -1e9 * LOG2E
T = 128
N = 4
NPROD = 49
ROWS = N * T

S = 2048
DM = 1024
DC = 512
HB = 32
WIN, DIL, HA, DH_A = 8, 2, 32, 32
HALO = 16
G = 16
PITCH_B = 17
PITCH_A = 33

CFG = dict(lag=8, p_j=8, mix_j=4, mix_p=4, pv=4, group=8, o_flush=(42, 48), b_rate=(40, 40), b_wait=6, b_cost=16, b_proj=(0, 0), b_prep=(9, 0),
           steps="""
    |a>bc s1 |b>d x0 w1,0 r58 w1,1 K0,0 |c>e x1 x2 K0,1 r48 K1,0 K1,1 |d>f x3 s0 w0,0 K2,0 K2,1 w0,1 K3,0 K3,1
    |e>gh s2 w2,0 Q0,0 Q0,1 p0 Q1,0 w2,1 Q1,1 Q2,0 Q2,1 Q3,0 Q3,1 |f>ij tq W0 V0,0 V0,1 V1,0
    |g> b0 V1,1 b1 V2,0 p1 V2,1 b2 V3,0 V3,1 b3 W1 P0,0 P0,1 P0,2 P0,3
    |h> m0 W2 P1,0 P1,1 s3 P1,2 P1,3 w3,0 W3 o0 P2,0 P2,1 P2,2 w3,1 P2,3
    |i> W4 tv p2 P3,0 P3,1 P3,2 P3,3 m1 O0,0 O0,1 |>0 W5 o1 P4,0 P4,1 tk P4,2 P4,3
    |j> W6 p3 O1,0 O1,1 |>1 P5,0 P5,1 m2 P5,2 P5,3 W7 o2
    P6,0 m3 P6,1 P6,2 P6,3 o3 O2,0 O2,1 |>2 c0 c1 P7,0 P7,1 c2 c3 U P7,2 P7,3 O3,0 O3,1 |>3""")


def _mm(a, b):
    return jnp.dot(a, b, preferred_element_type=F32)


def _mm_nt(a, b):
    return lax.dot_general(a, b, (((1,), (1,)), ((), ())), preferred_element_type=F32)


def _cat(xs, axis):
    xs = list(xs)
    return xs[0] if len(xs) == 1 else lax.concatenate(xs, axis)


def _rows(x, start, size):
    return lax.slice_in_dim(x, start, start + size, axis=0)


def _fold(op, xs):
    xs = list(xs)
    acc = xs[0]
    for x in xs[1:]:
        acc = op(acc, x)
    return acc


def _bf(words):
    return pltpu.bitcast(words, BF16)


def _words(x):
    return pltpu.bitcast(x, U32)


def _reciprocal(x):
    r = pltpu.reciprocal(x, approx=True)
    return r * (2.0 - x * r)


def _quads(g, n):
    h = n // 2
    return [{(r, c): g[(r + i * h, c + j * h)] for r in range(h) for c in range(h)}
            for i in range(2) for j in range(2)]


def _gadd(x, y):
    return {k: lax.add(x[k], y[k]) for k in x}


def _gsub(x, y):
    return {k: lax.sub(x[k], y[k]) for k in x}


LEFT = ((2, 1, 3), (3,), (0, 1, 3), (0, 1, 1), (2, -1, 0), (0,), (1, -1, 3))
RIGHT = ((0,), (2, -1, 0), (0, 1, 3), (3,), (0, 1, 1), (1, -1, 3), (2, 1, 3))


def _factor(rule, quad):
    if len(rule) == 1:
        return quad(rule[0])
    return (_gadd if rule[1] > 0 else _gsub)(quad(rule[0]), quad(rule[2]))


def _factors(rules, g, n=N):
    if n == 1:
        return [g[(0, 0)]]
    quads = _quads(g, n)
    return [x for rule in rules for x in _factors(rules, _factor(rule, quads.__getitem__), n // 2)]


def _combine(product, emit, n=N, base=0):
    if n == 1:
        return emit(0, 0, product(base))
    h = n // 2
    step = 7 ** (h.bit_length() - 1)
    m2, m4, m5, t, u = {}, {}, {}, {}, {}

    def use(i, r, c, m):
        if i == 0:
            m2[r, c] = m
        elif i == 1:
            m4[r, c] = m
            emit(r + h, c, lax.add(m2[r, c], m))
        elif i == 2:
            u[r, c], t[r, c] = lax.add(m4[r, c], m), lax.sub(m, m2[r, c])
        elif i == 3:
            m5[r, c] = m
            u[r, c] = lax.sub(u[r, c], m)
        elif i == 4:
            t[r, c] = lax.add(t[r, c], m)
        elif i == 5:
            emit(r, c + h, lax.add(m, m5[r, c]))
            emit(r + h, c + h, lax.add(t[r, c], m))
        else:
            emit(r, c, lax.add(u[r, c], m))

    for i in range(7):
        _combine(product, lambda r, c, m, i=i: use(i, r, c, m), h, base + i * step)


class _SideWork:
    def __init__(self, lag, never=None):
        self.lag, self.never = lag, never
        self.urgent, self.todo, self.results = [], [], []
        self.clock, self.credit, self.rate, self.cache = 0, 0.0, 0.0, (None,)

    def after(self, x):
        old = [r for r in self.results if r[0] <= self.clock - self.lag]
        if not old:
            return x
        _, value, row = old[-1]
        key = (self.clock, x.shape, x.dtype == F32)
        if self.cache[0] != key:
            dep = _rows(value, row, 8)
            dep = dep if x.dtype == F32 else _words(dep)
            self.cache = (key, _cat([_cat([dep] * (x.shape[1] // T), 1)] * (x.shape[0] // 8), 0), self.never(x.shape))
        return lax.select(self.cache[2], self.cache[1], x)

    def add(self, cost, run, wait=0, urgent=False):
        (self.urgent if urgent else self.todo).append((self.clock + wait, cost, run))

    def issued(self, tiles, result):
        for i in range(2 * tiles):
            self.clock += 0.5
            self.results = self.results[-40:] + [(self.clock, result, i * 8 // (2 * tiles) * 16)]
            self.credit += 0.5 * self.rate
            while self.credit > 0:
                ready = [x for x in (self.urgent, self.todo) if x and x[0][0] <= self.clock]
                if not ready:
                    break
                _, cost, run = ready[0].pop(0)
                self.credit -= cost
                run()
            self.credit = min(self.credit, 0.0)

    def finish(self, done=lambda: False):
        while (self.urgent or self.todo) and not done():
            (self.urgent or self.todo).pop(0)[2]()


def _queue_factors(side, rules, load, dst):
    def piece(outer):
        def run():
            h = N // 2
            quad = lambda x: {(r, c): load(x // 2 * h + r, x % 2 * h + c) for r in range(h) for c in range(h)}
            for i, x in enumerate(_factors(rules, _factor(rules[outer], quad), h)):
                ref, idx = dst(outer * 7 + i)
                ref[idx] = lax.convert_element_type(x, BF16)
        return run
    for outer in range(7):
        side.add(50, piece(outer))


def _queue_activation(side, src, dst, chunk):
    kt = src.shape[1] // (N * T)
    for t in range(kt):
        for r0 in range(0, T, G):
            def load(r, c, t=t, r0=r0):
                lo, col = chunk * ROWS + r * T + r0, (c * kt + t) * T
                return lax.convert_element_type(_bf(side.after(_words(src[lo:lo + G, col:col + T]))), F32)
            _queue_factors(side, LEFT, load, lambda i, t=t, r0=r0: (dst, (i, t, pl.ds(chunk * T + r0, G))))


def _queue_head_weights(side, columns, kt, scale, wops, slot):
    high, shift = jnp.full((G, T), 0xFFFF0000, U32), jnp.full((G, T), 16, U32)
    for t in range(kt):
        for r0 in range(0, T, G):
            def load(r, c, t=t, r0=r0):
                ref, word, half = columns[c]
                w = side.after(ref[pl.ds(word + ((kt * r + t) * T + r0) * PITCH_B, G, stride=PITCH_B), :])
                w = pltpu.bitcast(lax.bitwise_and(w, high) if half else lax.shift_left(w, shift), F32)
                return w if scale is None else w * scale
            _queue_factors(side, RIGHT, load, lambda i, t=t, r0=r0: (wops, (slot + t, i, pl.ds(r0, G))))


def _queue_kv_weights(side, pair, stk, stv, wops):
    _queue_head_weights(side, [(stk, pair, 0), (stk, pair, 1), (stv, pair, 0), (stv, pair, 1)], 1, None, wops, 0)


def _tile(ref, *idx):
    *lead, row = idx
    return ref.bitcast(U32)[(*lead, pl.ds(row * (T // 2), T // 2))]


def _phase_a(cfg, barrier, x, wqkv, woa, staged, wops, oops, kbuf, vbuf, ckv, xops, cops, stb, qall, outa):
    side = _SideWork(cfg["lag"])
    q = {}
    done = set()

    def check(step, user):
        assert step is None or step in done or cfg.get("nodeps"), (user, "must come after", step)

    def stage(sec, i):
        def run():
            if sec < 3:
                w = _bf(side.after(_words(wqkv[i * T:(i + 1) * T, sec * DM:(sec + 1) * DM]))).T
            else:
                w = _bf(side.after(_words(woa[:, i * T:(i + 1) * T])))
            w = w.astype(F32)
            for h in range(HA):
                staged[i, h * PITCH_A:h * PITCH_A + DH_A, :] = w[h * DH_A:(h + 1) * DH_A]
        return run

    def weights(sec, g, t, r0):
        def permuted(slab, j):
            w = side.after(staged[slab, pl.ds(r0 % HA * PITCH_A + 4 * j + r0 // HA, G, stride=PITCH_A), :])
            return w * (float(DH_A ** -0.5) * LOG2E) if sec == 0 else w

        load = (lambda r, c: permuted(2 * r + t, g * N + c)) if sec < 3 else (
            lambda r, c: permuted(g * N + c, 2 * r + t))
        _queue_factors(side, RIGHT, load, lambda i: (wops[sec == 0], (2 * g + t, i, pl.ds(r0, G))))

    def project(sec, c, g):
        needs = [("w", sec, g), ("o" if sec == 3 else "x", c)]
        side.finish(lambda: cfg.get("nodeps") or all(n in done for n in needs))
        for n in needs:
            check(n, (sec, c, g))

        def product(i):
            w = [_tile(wops[sec == 0], 2 * g + t, i, 0) for t in range(2)]
            if sec < 3:
                out = _mm_nt(_bf(_cat([_tile(xops, i, t, c) for t in range(2)], 1)), _bf(_cat(w, 1)))
            else:
                out = _mm(_bf(_cat([_tile(oops, i, t, c % 2) for t in range(2)], 1)), _bf(_cat(w, 0)))
            side.issued(2, out)
            return out

        def emit(r, col, val):
            r0, j = c * ROWS + r * T, g * N + col
            if sec == 0:
                q[(r0, j)] = val
            elif sec == 3:
                outa[r0:r0 + T, j * T:(j + 1) * T] = val.astype(BF16)
            else:
                (kbuf if sec == 1 else vbuf)[j, HALO + r0:HALO + r0 + T, :] = val

        _combine(product, emit)

    def project_queries(quad, c):
        needs = [("W", quad), ("b", c), ("t", "qqqqvvkk"[quad])]
        side.finish(lambda: cfg.get("nodeps") or all(n in done for n in needs))
        for n in needs:
            check(n, ("P", quad, c))

        def product(i):
            out = _mm(_bf(_cat([_tile(xops, i, t, c) for t in range(2)], 1)),
                      _bf(_cat([_tile(wops[1], quad % 2 * 2 + t, i, 0) for t in range(2)], 0)))
            side.issued(2, out)
            return out

        def emit(r, h, val):
            qall[4 * quad + h, c * ROWS + r * T:c * ROWS + (r + 1) * T, :] = val.astype(BF16)

        _combine(product, emit)

    E = cfg["group"]
    row = lax.broadcasted_iota(jnp.int32, (E, T), 0)

    lane = lax.broadcasted_iota(jnp.int32, (E, T), 1)

    def group_sums(a, b, c, d):
        even, low = (lane & HA) == 0, lane < 2 * HA
        fold = lambda pick, x, y, shift: lax.select(pick, x, y) + pltpu.roll(lax.select(pick, y, x), shift, 1)
        z = fold(low, fold(even, a, b, 3 * HA), fold(even, c, d, 3 * HA), 2 * HA)
        zr = pltpu.roll(z, 2 * HA, 1)
        out = []
        for x in (lax.select(low, z, zr), lax.select(low, zr, z)):
            xr = pltpu.roll(x, HA, 1)
            out += [lax.select(even, x, xr), lax.select(even, xr, x)]
        return out

    def probs(r0):
        def run():
            qs = side.after(_cat([_rows(q[(r0 - r0 % T, j)], r0 % T, E) for j in range(8)], 0)).reshape(8, E, T)
            J = cfg["p_j"]
            qs = [_rows(qs, j, J) for j in range(0, 8, J)]
            parts = []
            for w in range(WIN):
                lo = HALO + r0 - DIL * w
                s = jnp.sum(_fold(lax.add, [lax.mul(qs[j // J], kbuf[j:j + J, lo:lo + E, :]) for j in range(0, 8, J)]), axis=0)
                parts.append(s)
            logits = []
            if cfg.get("rs"):
                for w in range(0, WIN, 4):
                    logits += group_sums(*parts[w:w + 4])
            else:
                for s in parts:
                    s = s + pltpu.roll(s, 2 * HA, 1)
                    logits.append(s + pltpu.roll(s, HA, 1))
            logits = [jnp.where(row + r0 >= DIL * w, s, NEG) if r0 < DIL * w else s for w, s in enumerate(logits)]
            m = _fold(jnp.maximum, logits)
            e = [jnp.exp2(s - m) for s in logits]
            inv = _reciprocal(_fold(jnp.add, e))
            for w in range(WIN):
                kbuf[w, r0:r0 + E, :] = e[w] * inv
        return run

    def mix(r0, js):
        def run():
            J = cfg["mix_j"]
            p = side.after(kbuf[:, r0:r0 + E, :].reshape(WIN * E, T))
            p = [lax.broadcast(_rows(p, w * E, E), (J,)) for w in range(WIN)]
            for j in js:
                vbuf[j:j + J, r0:r0 + E, :] = _fold(lax.add, [
                    lax.mul(p[w], vbuf[j:j + J, HALO + r0 - DIL * w:HALO + r0 - DIL * w + E, :]) for w in range(WIN)])
        return run

    def queue_output(c):
        for t in range(2):
            for r0 in range(0, T, G):
                def load(r, col, t=t, r0=r0):
                    lo = c * ROWS + r * T + r0
                    return side.after(vbuf[2 * col + t, lo:lo + G, :])
                _queue_factors(side, LEFT, load, lambda i, t=t, r0=r0: (oops, (i, t, pl.ds(c % 2 * T + r0, G))))

    def stage_heads(base, st, m0, count):
        def run():
            lo = m0 * HB // 2
            w = side.after(qall.bitcast(U32)[base + lo // (S // 2), pl.ds(lo % (S // 2), count * HB // 2), :])
            for i in range(count):
                st[(m0 + i) * PITCH_B:(m0 + i) * PITCH_B + HB // 2, :] = _rows(w, i * HB // 2, HB // 2)
        return run

    for step in cfg["steps"].split():
        kind, arg = step[0], step[1:]
        num = [int(a) for a in arg.split(",")] if arg[:1].isdigit() else []
        if kind == "|":
            if side.clock == 0:
                side.finish()
            barrier(*arg.split(">"))
            zeros = vbuf[0, HALO + S:HALO + S + 8, :]
            side.results = []
            side.never = lambda shape, z=zeros: _cat([_cat([z] * (shape[1] // T), 1)] * (shape[0] // 8), 0) != 0
        elif kind == "r":
            side.rate = num[0]
        elif kind in "QKVO":
            project("QKVO".index(kind), *num)
            done.add((kind, *num))
        elif kind == "s":
            for i in range(8):
                side.add(320, stage(num[0], i))
        elif kind == "P":
            project_queries(*num)
            done.add((kind, *num))
        elif kind in "wxobW":
            key = (kind, *num)
            frees = {"w": {1: None, 0: None, 2: ("K", 3, num[-1]), 3: ("V", 3, num[-1])}.get(num[0]) if kind == "w" else None,
                     "x": None, "b": ("V", num[0], 1), "o": ("O", num[0] - 2, 1) if num[0] >= 2 else None,
                     "W": ("P", num[0] - 2, 3) if num[0] >= 2 else ("Q", 3, num[0])}[kind]
            side.add(0, lambda frees=frees, key=key: check(frees, key))
            if kind == "w":
                for t in range(2):
                    for r0 in range(0, T, G):
                        weights(*num, t, r0)
            elif kind in "xb":
                _queue_activation(side, x, xops, *num)
            elif kind == "W":
                _queue_head_weights(side, [(stb[0], 2 * num[0] + h // 2, h % 2) for h in range(4)], 2,
                                    float(T ** -0.5) * LOG2E, wops[1], num[0] % 2 * 2)
            else:
                queue_output(*num)
            side.add(0, lambda key=(kind, *num): done.add(key))
        elif kind in "pm":
            check(("Q" if kind == "p" else "V", num[0], 1), step)
            for r0 in range(num[0] * ROWS, (num[0] + 1) * ROWS, E):
                if kind == "p":
                    side.add(28 * E, probs(r0))
                else:
                    for j in range(0, 8, cfg["mix_p"]):
                        side.add(2 * E * cfg["mix_p"] + E, mix(r0, range(j, j + cfg["mix_p"], cfg["mix_j"])))
        elif kind == "c":
            _queue_activation(side, ckv, cops, *num)
        elif kind == "t":
            st = stb["qkv".index(arg)]
            for m0 in range(0, st.shape[0] // PITCH_B, 4):
                side.add(24, stage_heads({"q": 0, "v": 16, "k": 24}[arg], st, m0, 4))
            side.add(0, lambda key=("t", arg): done.add(key))
        elif kind == "U":
            _queue_kv_weights(side, 0, stb[1], stb[2], wops[1])
    side.finish()


def _pair_body(cfg, pair, cops, stk, stv, wops, qall, ctx):
    side = _SideWork(cfg["lag"], lambda shape: lax.broadcast(pair < 0, shape))
    side.rate = cfg["b_rate"][0]
    k, v = {}, {}

    def project(j):
        def product(i):
            out = _mm(_bf(_tile(cops, i, 0, j)), _bf(_tile(wops, 0, i, 0)))
            side.issued(1, out)
            return out

        def emit(r, c, val):
            (k if c < 2 else v)[(c % 2, N * j + r)] = val

        _combine(product, emit)

    causal = lax.broadcasted_iota(jnp.int32, (T, T), 1) <= lax.broadcasted_iota(jnp.int32, (T, T), 0)

    def scores(h, i):
        s = _mm_nt(_bf(_tile(qall, 2 * pair + h, i)), _cat([k[(h, t)] for t in range(i + 1)], 0).astype(BF16))
        s = [s[:, t * T:(t + 1) * T] for t in range(i + 1)]
        for t in range(0, i + 1, 4):
            side.issued(min(4, i + 1 - t), s[t])
        s[i] = jnp.where(causal, s[i], NEG)
        return s, jnp.max(_fold(jnp.maximum, s), axis=1, keepdims=True)

    def attend(h, i, s, m):
        e = [jnp.exp2(x - m) for x in s]
        inv = {}

        def denominator(r0):
            def run():
                part = side.after(_fold(lax.add, [_rows(x, r0, G) for x in e]))
                inv[r0] = _reciprocal(jnp.broadcast_to(jnp.sum(part, axis=1, keepdims=True), (G, T)))
            return run
        for r0 in range(0, T, G):
            side.add(cfg["b_cost"] + 2 * i, denominator(r0), cfg["b_wait"], urgent=True)

        acc = None
        for t in range(0, i + 1, cfg["pv"]):
            ts = range(t, min(t + cfg["pv"], i + 1))
            part = _mm(_cat([e[u] for u in ts], 1).astype(BF16), _cat([v[(h, u)] for u in ts], 0).astype(BF16))
            acc = part if acc is None else acc + part
            side.issued(len(ts), acc)

        def store():
            ctx[i, 2 * pair + h] = acc * _cat([inv[r0] for r0 in range(0, T, G)], 0)
        side.add(0, store, cfg["b_wait"], urgent=True)

    project(0)
    first = [(h, i, *scores(h, i)) for i in range(N) for h in range(2)]
    project(1)
    for unit in first[:-1]:
        attend(*unit)
    live = first[-1]
    for i in range(N, S // T):
        for h in range(2):
            new = (h, i, *scores(h, i))
            if (i % N, h) == tuple(cfg["b_proj"]) and i // N + 1 < S // ROWS:
                project(i // N + 1)
            if (i, h) == tuple(cfg["b_prep"]):
                side.rate = cfg["b_rate"][1]
                _queue_kv_weights(side, jnp.minimum(pair + 1, HB // 2 - 1), stk, stv, wops)
            attend(*live)
            live = new
    attend(*live)
    side.results = []
    side.finish()


def _phase_o(cfg, ctx, wob, stage, out_h, sems):
    kt, mt, width = HB // N, S // T // N, DM // N
    lhs = _factors(LEFT, {
        (r, c): _cat([_cat([ctx[r * mt + m, c * kt + t] for t in range(kt)], 1) for m in range(mt)], 0)
        for r in range(N) for c in range(N)})
    half = kt * T // 2
    rhs = _factors(RIGHT, {
        (r, c): _bf(_cat([wob.bitcast(U32)[2 * (2 * c + t) + r // 2, r % 2 * half:(r % 2 + 1) * half, :]
                          for t in range(2)], 1)).astype(F32) for r in range(N) for c in range(N)})
    ready, started = [], []

    def flush():
        for r, c in ready:
            rows = pl.ds(r * mt * T, mt * T)
            started.append(pltpu.make_async_copy(stage.at[rows, pl.ds(c * width, width)],
                                                 out_h.at[rows, pl.ds(DM + c * width, width)], sems.at[len(started)]))
            started[-1].start()
        ready.clear()

    def product(i):
        if i in cfg["o_flush"]:
            flush()
        return _mm(lhs[i].astype(BF16), rhs[i].astype(BF16))

    def emit(r, c, val):
        stage[r * mt * T:(r + 1) * mt * T, c * width:(c + 1) * width] = val.astype(BF16)
        ready.append((r, c))

    _combine(product, emit)
    flush()
    for cp in started:
        cp.wait()


def _kernel(cfg, xa_h, wqkv_h, woa_h, xb_h, ckv_h, wq_h, wuk_h, wuv_h, wob_h, out_h,
            cops, stk, stv, wops, qall, outa, sems):
    copy_a = [pltpu.make_async_copy(outa.at[pl.ds(c * ROWS, ROWS)], out_h.at[pl.ds(c * ROWS, ROWS), pl.ds(0, DM)],
                                    sems.at[c]) for c in range(S // ROWS)]

    def first(x, wqkv, woa, staged, wops2, oops, kbuf, vbuf, ckv, xops, stq):
        def x_rows(lo, hi):
            return xa_h.at[pl.ds(lo, hi - lo)], x.at[pl.ds(lo, hi - lo)]

        def w_cols(sec):
            return wqkv_h.at[:, pl.ds(sec * DM, DM)], wqkv.at[:, pl.ds(sec * DM, DM)]

        groups = {
            "a": [w_cols(1)],
            "b": [x_rows(0, ROWS)],
            "c": [x_rows(ROWS, 3 * ROWS)],
            "d": [w_cols(0), x_rows(3 * ROWS, S)],
            "e": [w_cols(2), (woa_h, woa)],
            "f": [(wq_h, qall.at[0:16])],
            "g": [(xb_h, x)],
            "h": [(wuv_h, qall.at[16:24])],
            "i": [(wuk_h, qall.at[24:32])],
            "j": [(ckv_h, ckv)],
        }
        slot = iter(range(4, 16))
        copies = {k: [pltpu.make_async_copy(src, dst, sems.at[next(slot)]) for src, dst in v]
                  for k, v in groups.items()}
        copies.update({str(c): [cp] for c, cp in enumerate(copy_a)})

        def barrier(wait, start):
            for name in wait:
                for cp in copies[name]:
                    cp.wait()
            for name in start:
                for cp in copies[name]:
                    cp.start()

        barrier("", "a")
        kbuf[:, 0:HALO, :] = jnp.zeros((8, HALO, T), F32)
        vbuf[:, 0:HALO, :] = jnp.zeros((8, HALO, T), F32)
        vbuf[0, HALO + S:HALO + S + 8, :] = jnp.zeros((8, T), F32)
        _phase_a(cfg, barrier, x, wqkv, woa, staged, (wops2, wops), oops, kbuf, vbuf, ckv,
                 xops, cops, (stq, stk, stv), qall, outa)
        if cfg.get("nodeps"):
            for a, b in ((kbuf.at[0, 0:8], vbuf.at[0, 0:8]), (vbuf.at[1, 0:8], kbuf.at[1, 0:8]), (staged.at[0, 0:8], kbuf.at[2, 0:8]),
                         (wops2.at[0, 0], oops.at[0, 0, 0:T]), (oops.at[1, 0, 0:T], wops2.at[1, 0]), (stq.at[0:8], stk.at[0:8]),
                         (stk.at[8:16], stv.at[0:8]), (stv.at[8:16], stq.at[8:16]), (xops.at[0, 0, 0:T], wops2.at[2, 0])):
                cp = pltpu.make_async_copy(a, b, sems.at[5])
                cp.start()
                cp.wait()

    (pl.run_scoped if not cfg.get("skip_a") else (lambda *a: None))(
        first,
        pltpu.VMEM((S, DM), BF16), pltpu.VMEM((DM, 3 * DM), BF16), pltpu.VMEM((DM, DM), BF16),
        pltpu.VMEM((8, HA * PITCH_A, T), F32), pltpu.VMEM((4, NPROD, T, T), BF16),
        pltpu.VMEM((NPROD, 2, 2 * T, T), BF16),
        pltpu.VMEM((8, HALO + S, T), F32), pltpu.VMEM((8, HALO + S + 8, T), F32),
        pltpu.VMEM((S, DC), BF16),
        pltpu.VMEM((NPROD, 2, S // N, T), BF16),
        pltpu.VMEM((DM * PITCH_B, T), U32))

    def second(ctx):
        load_wo = [pltpu.make_async_copy(wob_h.at[:, :, pl.ds(j * T, T)], qall.at[2 * j:2 * j + 2], sems.at[4 + j])
                   for j in range(8)]

        def pair(i, carry):
            @pl.when(i == 8)
            def _():
                for cp in load_wo:
                    cp.start()
            _pair_body(cfg, i, cops, stk, stv, wops, qall, ctx)
            return carry
        if not cfg.get("skip_b"):
            lax.fori_loop(0, HB // 2, pair, 0)
        else:
            for cp in load_wo:
                cp.start()
        for cp in load_wo + ([] if cfg.get("skip_a") else copy_a):
            cp.wait()
        if not cfg.get("skip_o"):
            _phase_o(cfg, ctx, qall, outa, out_h, sems)

    if cfg.get("only_a"):
        for i, src in enumerate((qall.at[0], cops.at[0, 0], wops.at[0, 0])):
            cp = pltpu.make_async_copy(src, out_h.at[pl.ds(0, src.shape[0]), pl.ds(DM + i * T, T)], sems.at[5])
            cp.start()
            cp.wait()
        if not cfg.get("nodeps"):
            for cp in copy_a:
                cp.wait()
        return
    pl.run_scoped(second, pltpu.VMEM((S // T, HB, T, T), F32))


def _call(cfg, A_x, A_wqkv, A_wo, B_x, B_c_kv, B_w_q, B_w_uk, B_w_uv, B_w_o):
    any_spec = pl.BlockSpec(memory_space=pl.ANY)
    out = pl.pallas_call(
        lambda *refs: _kernel(cfg, *refs),
        out_shape=jax.ShapeDtypeStruct((S, 2 * DM), BF16),
        in_specs=[any_spec] * 9,
        out_specs=any_spec,
        scratch_shapes=[
            pltpu.VMEM((NPROD, 1, S // N, T), BF16),
            pltpu.VMEM((DC * PITCH_B, T), U32),
            pltpu.VMEM((DC * PITCH_B, T), U32),
            pltpu.VMEM((4, NPROD, T, T), BF16),
            pltpu.VMEM((HB, S, T), BF16),
            pltpu.VMEM((S, DM), BF16),
            pltpu.SemaphoreType.DMA((N * N,)),
        ],
        compiler_params=pltpu.CompilerParams(vmem_limit_bytes=126 * 1024 * 1024),
        name="concat_heads",
    )(A_x.reshape(S, DM), A_wqkv, A_wo, B_x.reshape(S, DM), B_c_kv.reshape(S, DC),
      B_w_q.reshape(16, S, T), B_w_uk.reshape(8, S, T), B_w_uv.reshape(8, S, T),
      B_w_o.reshape(2, S, DM))
    return out.reshape(1, S, 2 * DM)


@jax.jit
def pallas_concat_heads__sliding_local_dilated__compressed_kv_cla__prompt_kernel(
    A_x: jax.Array,
    A_wqkv: jax.Array,
    A_wo: jax.Array,
    B_x: jax.Array,
    B_c_kv: jax.Array,
    B_w_q: jax.Array,
    B_w_uk: jax.Array,
    B_w_uv: jax.Array,
    B_w_o: jax.Array,
):
    return _call(CFG, A_x, A_wqkv, A_wo, B_x, B_c_kv, B_w_q, B_w_uk, B_w_uv, B_w_o)
```

```python
import numpy as np

import jax
import jax.numpy as jnp
from jax import lax
import jax.experimental.pallas as pl
import jax.experimental.pallas.tpu as pltpu

F32, BF16, U32 = jnp.float32, jnp.bfloat16, jnp.uint32
LOG2E = float(np.log2(np.e))
NEG = -1e9 * LOG2E
T = 128
N = 4
NPROD = 49
ROWS = N * T

S = 2048
DM = 1024
DC = 512
HB = 32
WIN, DIL, HA, DH_A = 8, 2, 32, 32
HALO = 16
G = 16
PITCH_B = 17
PITCH_A = 33

CFG = dict(lag=8, p_j=8, mix_j=4, mix_p=4, pv=4, group=8, o_flush=(42, 48), b_rate=(40, 40), b_wait=8, b_late=3, b_small=(16, 0), b_each=1, b_deep=6, b_span=8, b_qtie=0, b_wtie=1, b_cost=32, b_proj=(0, 0), b_prep=(9, 0),
           steps="""
    |z>b r56 s1,0,2 F0 |a>c s1,2,4 F1 |b>d r96 s1,4,8 w1,0 F2 |c>e x1 F3 r56 w1,1 K1,0
    |d>f x2 K1,1 r48 x3 K2,0 x0 K2,1 |e>gh s0 w0,0 K3,0 K3,1 w0,1 Q0,0 s2 w2,0 Q0,1 p0 Q1,0 w2,1 Q1,1 Q2,0 Q2,1
    Q3,0 Q3,1 |f>ij tq W0 V0,0 V0,1 V1,0
    |g> b0 V1,1 b1 V2,0 p1 V2,1 b2 V3,0 V3,1 b3 W1 P0,0 P0,1 P0,2 P0,3
    m0 W2 P1,0 P1,1 s3 P1,2 P1,3 w3,0 W3 o0 P2,0 P2,1 P2,2 w3,1 P2,3
    |hij> W4 tv p2 P3,0 P3,1 P3,2 P3,3 m1 O0,0 O0,1 W5 o1 P4,0 P4,1 tk P4,2 P4,3
    W6 p3 O1,0 O1,1 |>01 P5,0 P5,1 m2 P5,2 P5,3 W7 o2
    P6,0 m3 P6,1 P6,2 P6,3 o3 O2,0 O2,1 c0 c1 P7,0 P7,1 c2 c3 U P7,2 P7,3 O3,0 O3,1 |>23""")


def _mm(a, b):
    return jnp.dot(a, b, preferred_element_type=F32)


def _mm_nt(a, b):
    return lax.dot_general(a, b, (((1,), (1,)), ((), ())), preferred_element_type=F32)


def _cat(xs, axis):
    xs = list(xs)
    return xs[0] if len(xs) == 1 else lax.concatenate(xs, axis)


def _rows(x, start, size):
    return lax.slice_in_dim(x, start, start + size, axis=0)


def _fold(op, xs):
    xs = list(xs)
    acc = xs[0]
    for x in xs[1:]:
        acc = op(acc, x)
    return acc


def _bf(words):
    return pltpu.bitcast(words, BF16)


def _words(x):
    return pltpu.bitcast(x, U32)


def _reciprocal(x):
    r = pltpu.reciprocal(x, approx=True)
    return r * (2.0 - x * r)


def _quads(g, n):
    h = n // 2
    return [{(r, c): g[(r + i * h, c + j * h)] for r in range(h) for c in range(h)}
            for i in range(2) for j in range(2)]


def _gadd(x, y):
    return {k: lax.add(x[k], y[k]) for k in x}


def _gsub(x, y):
    return {k: lax.sub(x[k], y[k]) for k in x}


LEFT = ((2, 1, 3), (3,), (0, 1, 3), (0, 1, 1), (2, -1, 0), (0,), (1, -1, 3))
RIGHT = ((0,), (2, -1, 0), (0, 1, 3), (3,), (0, 1, 1), (1, -1, 3), (2, 1, 3))


def _factor(rule, quad):
    if len(rule) == 1:
        return quad(rule[0])
    return (_gadd if rule[1] > 0 else _gsub)(quad(rule[0]), quad(rule[2]))


def _factors(rules, g, n=N):
    if n == 1:
        return [g[(0, 0)]]
    quads = _quads(g, n)
    return [x for rule in rules for x in _factors(rules, _factor(rule, quads.__getitem__), n // 2)]


def _combine(product, emit, n=N, base=0):
    if n == 1:
        return emit(0, 0, product(base))
    h = n // 2
    step = 7 ** (h.bit_length() - 1)
    m2, m4, m5, t, u = {}, {}, {}, {}, {}

    def use(i, r, c, m):
        if i == 0:
            m2[r, c] = m
        elif i == 1:
            m4[r, c] = m
            emit(r + h, c, lax.add(m2[r, c], m))
        elif i == 2:
            u[r, c], t[r, c] = lax.add(m4[r, c], m), lax.sub(m, m2[r, c])
        elif i == 3:
            m5[r, c] = m
            u[r, c] = lax.sub(u[r, c], m)
        elif i == 4:
            t[r, c] = lax.add(t[r, c], m)
        elif i == 5:
            emit(r, c + h, lax.add(m, m5[r, c]))
            emit(r + h, c + h, lax.add(t[r, c], m))
        else:
            emit(r, c, lax.add(u[r, c], m))

    for i in range(7):
        _combine(product, lambda r, c, m, i=i: use(i, r, c, m), h, base + i * step)


class _SideWork:
    def __init__(self, lag, never=None):
        self.lag, self.never = lag, never
        self.urgent, self.todo, self.running, self.results = [], [], [], []
        self.clock, self.credit, self.rate, self.cache = 0, 0.0, 0.0, (None,)

    def after(self, x):
        old = [r for r in self.results if r[0] <= self.clock - self.lag]
        if not old:
            return x
        _, value, row = old[-1]
        key = (self.clock, x.shape, x.dtype == F32)
        if self.cache[0] != key:
            dep = _rows(value, row, 8)
            dep = dep if x.dtype == F32 else _words(dep)
            self.cache = (key, _cat([_cat([dep] * (x.shape[1] // T), 1)] * (x.shape[0] // 8), 0), self.never(x.shape))
        return lax.select(self.cache[2], self.cache[1], x)

    def before(self, words, most):
        due = [x for t, x in self.running[:most] if t <= self.clock]
        if not due:
            return words
        del self.running[:len(due)]
        parts = [_rows(words, r, 8) for r in range(0, T // 2, 8)]
        for i, x in enumerate(due):
            dep = _fold(lax.bitwise_or, [_words(_rows(x, r, 8)) for r in range(0, x.shape[0], 8)])
            parts[i * 8 // len(due)] = lax.select(self.never((8, T)), dep, parts[i * 8 // len(due)])
        return _cat(parts, 0)

    def add(self, cost, run, wait=0, urgent=False):
        (self.urgent if urgent else self.todo).append((self.clock + wait, cost, run))

    def issued(self, tiles, result):
        for i in range(2 * tiles):
            self.clock += 0.5
            self.results = self.results[-40:] + [(self.clock, result, i * 8 // (2 * tiles) * 16)]
            self.credit += 0.5 * self.rate
            while self.credit > 0:
                ready = [x for x in (self.urgent, self.todo) if x and x[0][0] <= self.clock]
                if not ready:
                    break
                _, cost, run = ready[0].pop(0)
                self.credit -= cost
                run()
            self.credit = min(self.credit, 0.0)

    def finish(self, done=lambda: False):
        while (self.urgent or self.todo) and not done():
            (self.urgent or self.todo).pop(0)[2]()


def _queue_factors(side, rules, load, dst):
    def piece(outer):
        def run():
            h = N // 2
            quad = lambda x: {(r, c): load(x // 2 * h + r, x % 2 * h + c) for r in range(h) for c in range(h)}
            for i, x in enumerate(_factors(rules, _factor(rules[outer], quad), h)):
                ref, idx = dst(outer * 7 + i)
                ref[idx] = lax.convert_element_type(x, BF16)
        return run
    for outer in range(7):
        side.add(50, piece(outer))


def _queue_activation(side, src, dst, chunk):
    kt = src.shape[1] // (N * T)
    for t in range(kt):
        for r0 in range(0, T, G):
            def load(r, c, t=t, r0=r0):
                lo, col = chunk * ROWS + r * T + r0, (c * kt + t) * T
                return lax.convert_element_type(_bf(side.after(_words(src[lo:lo + G, col:col + T]))), F32)
            _queue_factors(side, LEFT, load, lambda i, t=t, r0=r0: (dst, (i, t, pl.ds(chunk * T + r0, G))))


def _queue_head_weights(side, columns, kt, scale, wops, slot):
    high, shift = jnp.full((G, T), 0xFFFF0000, U32), jnp.full((G, T), 16, U32)
    for t in range(kt):
        for r0 in range(0, T, G):
            def load(r, c, t=t, r0=r0):
                ref, word, half = columns[c]
                w = side.after(ref[pl.ds(word + ((kt * r + t) * T + r0) * PITCH_B, G, stride=PITCH_B), :])
                w = pltpu.bitcast(lax.bitwise_and(w, high) if half else lax.shift_left(w, shift), F32)
                return w if scale is None else w * scale
            _queue_factors(side, RIGHT, load, lambda i, t=t, r0=r0: (wops, (slot + t, i, pl.ds(r0, G))))


def _queue_kv_weights(side, pair, stk, stv, wops):
    _queue_head_weights(side, [(stk, pair, 0), (stk, pair, 1), (stv, pair, 0), (stv, pair, 1)], 1, None, wops, 0)


def _tile(ref, *idx):
    *lead, row = idx
    return ref.bitcast(U32)[(*lead, pl.ds(row * (T // 2), T // 2))]


def _phase_a(cfg, barrier, x, wqkv, woa, staged, wops, oops, kbuf, vbuf, ckv, xops, cops, stb, qall, outa):
    side = _SideWork(cfg["lag"])
    q = {}
    done = set()

    def check(step, user):
        assert step is None or step in done or cfg.get("nodeps"), (user, "must come after", step)

    def stage(sec, i):
        def run():
            if sec < 3:
                w = _bf(side.after(_words(wqkv[i * T:(i + 1) * T, sec * DM:(sec + 1) * DM]))).T
            else:
                w = _bf(side.after(_words(woa[:, i * T:(i + 1) * T])))
            w = w.astype(F32)
            for h in range(HA):
                staged[i, h * PITCH_A:h * PITCH_A + DH_A, :] = w[h * DH_A:(h + 1) * DH_A]
        return run

    def weights(sec, g, t, r0):
        def permuted(slab, j):
            w = side.after(staged[slab, pl.ds(r0 % HA * PITCH_A + 4 * j + r0 // HA, G, stride=PITCH_A), :])
            return w * (float(DH_A ** -0.5) * LOG2E) if sec == 0 else w

        load = (lambda r, c: permuted(2 * r + t, g * N + c)) if sec < 3 else (
            lambda r, c: permuted(g * N + c, 2 * r + t))
        _queue_factors(side, RIGHT, load, lambda i: (wops[sec == 0], (2 * g + t, i, pl.ds(r0, G))))

    def project(sec, c, g):
        needs = [("w", sec, g), ("o" if sec == 3 else "x", c)]
        side.finish(lambda: cfg.get("nodeps") or all(n in done for n in needs))
        for n in needs:
            check(n, (sec, c, g))

        def product(i):
            w = [_tile(wops[sec == 0], 2 * g + t, i, 0) for t in range(2)]
            if sec < 3:
                out = _mm_nt(_bf(_cat([_tile(xops, i, t, c) for t in range(2)], 1)), _bf(_cat(w, 1)))
            else:
                out = _mm(_bf(_cat([_tile(oops, i, t, c % 2) for t in range(2)], 1)), _bf(_cat(w, 0)))
            side.issued(2, out)
            return out

        def emit(r, col, val):
            r0, j = c * ROWS + r * T, g * N + col
            if sec == 0:
                q[(r0, j)] = val
            elif sec == 3:
                outa[r0:r0 + T, j * T:(j + 1) * T] = val.astype(BF16)
            else:
                (kbuf if sec == 1 else vbuf)[j, HALO + r0:HALO + r0 + T, :] = val

        _combine(product, emit)

    def first_keys(r):
        side.finish(lambda: ("s", 1, 2 * r + 1) in done)
        for j in range(8):
            w = _cat([_cat([staged[slab, pl.ds(4 * j + d, HA, stride=PITCH_A), :] for d in range(4)], 0)
                      for slab in (2 * r, 2 * r + 1)], 1)
            out = _mm_nt(x[0:ROWS, 2 * r * T:(2 * r + 2) * T], w.astype(BF16))
            side.issued(2 * N, _rows(out, ROWS - T, T))
            kbuf[j, HALO:HALO + ROWS, :] = out + kbuf[j, HALO:HALO + ROWS, :] if r else out

    def project_queries(quad, c):
        needs = [("W", quad), ("b", c), ("t", "qqqqvvkk"[quad])]
        side.finish(lambda: cfg.get("nodeps") or all(n in done for n in needs))
        for n in needs:
            check(n, ("P", quad, c))

        def product(i):
            out = _mm(_bf(_cat([_tile(xops, i, t, c) for t in range(2)], 1)),
                      _bf(_cat([_tile(wops[1], quad % 2 * 2 + t, i, 0) for t in range(2)], 0)))
            side.issued(2, out)
            return out

        def emit(r, h, val):
            qall[4 * quad + h, c * ROWS + r * T:c * ROWS + (r + 1) * T, :] = val.astype(BF16)

        _combine(product, emit)

    E = cfg["group"]
    row = lax.broadcasted_iota(jnp.int32, (E, T), 0)

    lane = lax.broadcasted_iota(jnp.int32, (E, T), 1)

    def group_sums(a, b, c, d):
        even, low = (lane & HA) == 0, lane < 2 * HA
        fold = lambda pick, x, y, shift: lax.select(pick, x, y) + pltpu.roll(lax.select(pick, y, x), shift, 1)
        z = fold(low, fold(even, a, b, 3 * HA), fold(even, c, d, 3 * HA), 2 * HA)
        zr = pltpu.roll(z, 2 * HA, 1)
        out = []
        for x in (lax.select(low, z, zr), lax.select(low, zr, z)):
            xr = pltpu.roll(x, HA, 1)
            out += [lax.select(even, x, xr), lax.select(even, xr, x)]
        return out

    def probs(r0):
        def run():
            qs = side.after(_cat([_rows(q[(r0 - r0 % T, j)], r0 % T, E) for j in range(8)], 0)).reshape(8, E, T)
            J = cfg["p_j"]
            qs = [_rows(qs, j, J) for j in range(0, 8, J)]
            parts = []
            for w in range(WIN):
                lo = HALO + r0 - DIL * w
                s = jnp.sum(_fold(lax.add, [lax.mul(qs[j // J], kbuf[j:j + J, lo:lo + E, :]) for j in range(0, 8, J)]), axis=0)
                parts.append(s)
            logits = []
            if cfg.get("rs"):
                for w in range(0, WIN, 4):
                    logits += group_sums(*parts[w:w + 4])
            else:
                for s in parts:
                    s = s + pltpu.roll(s, 2 * HA, 1)
                    logits.append(s + pltpu.roll(s, HA, 1))
            logits = [jnp.where(row + r0 >= DIL * w, s, NEG) if r0 < DIL * w else s for w, s in enumerate(logits)]
            m = _fold(jnp.maximum, logits)
            e = [jnp.exp2(s - m) for s in logits]
            inv = _reciprocal(_fold(jnp.add, e))
            for w in range(WIN):
                kbuf[w, r0:r0 + E, :] = e[w] * inv
        return run

    def mix(r0, js):
        def run():
            J = cfg["mix_j"]
            p = side.after(kbuf[:, r0:r0 + E, :].reshape(WIN * E, T))
            p = [lax.broadcast(_rows(p, w * E, E), (J,)) for w in range(WIN)]
            for j in js:
                vbuf[j:j + J, r0:r0 + E, :] = _fold(lax.add, [
                    lax.mul(p[w], vbuf[j:j + J, HALO + r0 - DIL * w:HALO + r0 - DIL * w + E, :]) for w in range(WIN)])
        return run

    def queue_output(c):
        for t in range(2):
            for r0 in range(0, T, G):
                def load(r, col, t=t, r0=r0):
                    lo = c * ROWS + r * T + r0
                    return side.after(vbuf[2 * col + t, lo:lo + G, :])
                _queue_factors(side, LEFT, load, lambda i, t=t, r0=r0: (oops, (i, t, pl.ds(c % 2 * T + r0, G))))

    def stage_heads(base, st, m0, count):
        def run():
            lo = m0 * HB // 2
            w = side.after(qall.bitcast(U32)[base + lo // (S // 2), pl.ds(lo % (S // 2), count * HB // 2), :])
            for i in range(count):
                st[(m0 + i) * PITCH_B:(m0 + i) * PITCH_B + HB // 2, :] = _rows(w, i * HB // 2, HB // 2)
        return run

    scope = []
    for step in cfg["steps"].split():
        kind, arg = step[0], step[1:]
        num = [int(a) for a in arg.split(",")] if arg[:1].isdigit() else []
        if kind == "|":
            if side.clock == 0:
                side.finish()
            if cfg.get("scopes"):
                if scope:
                    scope.pop().__exit__(None, None, None)
                with jax.named_scope(f"wait_{side.clock:06.0f}_{arg}"):
                    barrier(*arg.split(">"))
                scope.append(jax.named_scope(f"block_{side.clock:06.0f}_{arg}"))
                scope[-1].__enter__()
            else:
                barrier(*arg.split(">"))
            zeros = vbuf[0, HALO + S:HALO + S + 8, :]
            side.results = []
            side.never = lambda shape, z=zeros: _cat([_cat([z] * (shape[1] // T), 1)] * (shape[0] // 8), 0) != 0
        elif kind == "r":
            side.rate = num[0]
        elif kind in "QKVO":
            project("QKVO".index(kind), *num)
            done.add((kind, *num))
        elif kind == "s":
            for i in range(*num[1:]) if num[1:] else range(8):
                side.add(320, stage(num[0], i))
                side.add(0, lambda key=("s", num[0], i): done.add(key))
        elif kind == "F":
            first_keys(*num)
        elif kind == "P":
            project_queries(*num)
            done.add((kind, *num))
        elif kind in "wxobW":
            key = (kind, *num)
            frees = {"w": {1: None, 0: None, 2: ("K", 3, num[-1]), 3: ("V", 3, num[-1])}.get(num[0]) if kind == "w" else None,
                     "x": None, "b": ("V", num[0], 1), "o": ("O", num[0] - 2, 1) if num[0] >= 2 else None,
                     "W": ("P", num[0] - 2, 3) if num[0] >= 2 else ("Q", 3, num[0])}[kind]
            side.add(0, lambda frees=frees, key=key: check(frees, key))
            if kind == "w":
                for t in range(2):
                    for r0 in range(0, T, G):
                        weights(*num, t, r0)
            elif kind in "xb":
                _queue_activation(side, x, xops, *num)
            elif kind == "W":
                _queue_head_weights(side, [(stb[0], 2 * num[0] + h // 2, h % 2) for h in range(4)], 2,
                                    float(T ** -0.5) * LOG2E, wops[1], num[0] % 2 * 2)
            else:
                queue_output(*num)
            side.add(0, lambda key=(kind, *num): done.add(key))
        elif kind in "pm":
            check(("Q" if kind == "p" else "V", num[0], 1), step)
            for r0 in range(num[0] * ROWS, (num[0] + 1) * ROWS, E):
                if kind == "p":
                    side.add(28 * E, probs(r0))
                else:
                    for j in range(0, 8, cfg["mix_p"]):
                        side.add(2 * E * cfg["mix_p"] + E, mix(r0, range(j, j + cfg["mix_p"], cfg["mix_j"])))
        elif kind == "c":
            _queue_activation(side, ckv, cops, *num)
        elif kind == "t":
            st = stb["qkv".index(arg)]
            for m0 in range(0, st.shape[0] // PITCH_B, 4):
                side.add(24, stage_heads({"q": 0, "v": 16, "k": 24}[arg], st, m0, 4))
            side.add(0, lambda key=("t", arg): done.add(key))
        elif kind == "U":
            _queue_kv_weights(side, 0, stb[1], stb[2], wops[1])
    side.finish()
    if scope:
        scope.pop().__exit__(None, None, None)


def _pair_body(cfg, pair, cops, stk, stv, wops, qall, ctx):
    side = _SideWork(cfg["lag"], lambda shape: lax.broadcast(pair < 0, shape))
    side.rate = cfg["b_rate"][0]
    k, v = {}, {}

    def project(j):
        def product(i):
            out = _mm(_bf(side.before(_tile(cops, i, 0, j), 1)), _bf(side.before(_tile(wops, 0, i, 0), cfg["b_wtie"])))
            side.issued(1, out)
            return out

        def emit(r, c, val):
            (k if c < 2 else v)[(c % 2, N * j + r)] = val

        _combine(product, emit)

    causal = lax.broadcasted_iota(jnp.int32, (T, T), 1) <= lax.broadcasted_iota(jnp.int32, (T, T), 0)

    def scores(h, i):
        s = _mm_nt(_bf(side.before(_tile(qall, 2 * pair + h, i), cfg["b_qtie"])), _cat([k[(h, t)] for t in range(i + 1)], 0).astype(BF16))
        s = [s[:, t * T:(t + 1) * T] for t in range(i + 1)]
        for t in range(0, i + 1, 4):
            side.issued(min(4, i + 1 - t), s[t])
        s[i] = jnp.where(causal, s[i], NEG)
        return s, jnp.max(_fold(jnp.maximum, s), axis=1, keepdims=True)

    def attend(h, i, s, m):
        e = [jnp.exp2(x - m) for x in s]
        acc = None
        for t in range(0, i + 1, cfg["pv"]):
            ts = range(t, min(t + cfg["pv"], i + 1))
            part = _mm(_cat([e[u] for u in ts], 1).astype(BF16), _cat([v[(h, u)] for u in ts], 0).astype(BF16))
            acc = part if acc is None else acc + part
            side.issued(len(ts), acc)

        def normalize(r0):
            def run():
                part = side.after(_fold(lax.add, [_rows(x, r0, G) for x in e]))
                out = _rows(acc, r0, G) * _reciprocal(jnp.sum(part, axis=1, keepdims=True))
                ctx[i, 2 * pair + h, r0:r0 + G, :] = out
                side.running.append((side.clock + cfg["b_span"], out))
            return run
        for r0 in range(0, T, G):
            side.add(cfg["b_cost"] + 2 * i, normalize(r0), cfg["b_wait"], urgent=True)

    late = cfg["b_late"]
    project(0)
    project(1)
    live, last, small = [], [], [(h, i) for i in reversed(range(late)) for h in range(2)]
    for i in range(late, S // T):
        for h in range(2):
            live.append((h, i, *scores(h, i)))
            if (i % N, h) == tuple(cfg["b_proj"]) and 0 < i // N < S // ROWS - 1:
                project(i // N + 1)
            if (i, h) == tuple(cfg["b_prep"]):
                side.rate = cfg["b_rate"][1]
                _queue_kv_weights(side, jnp.minimum(pair + 1, HB // 2 - 1), stk, stv, wops)
            if small and (i, h) >= tuple(cfg["b_small"]):
                for _ in range(cfg["b_each"]):
                    u = small.pop(0)
                    last.append((*u, *scores(*u)))
            while len(live) > (2 if i < cfg["b_deep"] else 1):
                attend(*live.pop(0))
    for unit in live + last + [(*u, *scores(*u)) for u in small]:
        attend(*unit)
    side.results = []
    side.finish()


def _phase_o(cfg, ctx, wob, stage, out_h, sems):
    kt, mt, width = HB // N, S // T // N, DM // N
    lhs = _factors(LEFT, {
        (r, c): _cat([_cat([ctx[r * mt + m, c * kt + t] for t in range(kt)], 1) for m in range(mt)], 0)
        for r in range(N) for c in range(N)})
    half = kt * T // 2
    rhs = _factors(RIGHT, {
        (r, c): _bf(_cat([wob.bitcast(U32)[2 * (2 * c + t) + r // 2, r % 2 * half:(r % 2 + 1) * half, :]
                          for t in range(2)], 1)).astype(F32) for r in range(N) for c in range(N)})
    ready, started = [], []

    def flush():
        for r, c in ready:
            rows = pl.ds(r * mt * T, mt * T)
            started.append(pltpu.make_async_copy(stage.at[rows, pl.ds(c * width, width)],
                                                 out_h.at[rows, pl.ds(DM + c * width, width)], sems.at[len(started)]))
            started[-1].start()
        ready.clear()

    def product(i):
        if i in cfg["o_flush"]:
            flush()
        return _mm(lhs[i].astype(BF16), rhs[i].astype(BF16))

    def emit(r, c, val):
        stage[r * mt * T:(r + 1) * mt * T, c * width:(c + 1) * width] = val.astype(BF16)
        ready.append((r, c))

    _combine(product, emit)
    flush()
    for cp in started:
        cp.wait()


def _kernel(cfg, xa_h, wqkv_h, woa_h, xb_h, ckv_h, wq_h, wuk_h, wuv_h, wob_h, out_h,
            cops, stk, stv, wops, qall, outa, sems):
    copy_a = [pltpu.make_async_copy(outa.at[pl.ds(c * ROWS, ROWS)], out_h.at[pl.ds(c * ROWS, ROWS), pl.ds(0, DM)],
                                    sems.at[c]) for c in range(S // ROWS)]

    def first(x, wqkv, woa, staged, wops2, oops, kbuf, vbuf, ckv, xops, stq):
        def x_rows(lo, hi):
            return xa_h.at[pl.ds(lo, hi - lo)], x.at[pl.ds(lo, hi - lo)]

        def w_cols(sec):
            return wqkv_h.at[:, pl.ds(sec * DM, DM)], wqkv.at[:, pl.ds(sec * DM, DM)]

        def quarter(r):
            k = pl.ds(r * DM // N, DM // N)
            return [(wqkv_h.at[k, pl.ds(DM, DM)], wqkv.at[k, pl.ds(DM, DM)]),
                    (xa_h.at[pl.ds(0, ROWS), k], x.at[pl.ds(0, ROWS), k])]

        groups = {
            "z": quarter(0), "a": quarter(1), "b": quarter(2) + quarter(3),
            "c": [x_rows(ROWS, 2 * ROWS)],
            "d": [x_rows(2 * ROWS, S)],
            "e": [w_cols(0), w_cols(2), (woa_h, woa)],
            "f": [(wq_h, qall.at[0:16])],
            "g": [(xb_h, x)],
            "h": [(wuv_h, qall.at[16:24])],
            "i": [(wuk_h, qall.at[24:32])],
            "j": [(ckv_h, ckv)],
        }
        slot = iter(range(4, 24))
        copies = {k: [pltpu.make_async_copy(src, dst, sems.at[next(slot)]) for src, dst in v]
                  for k, v in groups.items()}
        copies.update({str(c): [cp] for c, cp in enumerate(copy_a)})

        def barrier(wait, start):
            for name in wait:
                for cp in copies[name]:
                    cp.wait()
            for name in start:
                for cp in copies[name]:
                    cp.start()

        barrier("", "za")
        kbuf[:, 0:HALO, :] = jnp.zeros((8, HALO, T), F32)
        vbuf[:, 0:HALO, :] = jnp.zeros((8, HALO, T), F32)
        vbuf[0, HALO + S:HALO + S + 8, :] = jnp.zeros((8, T), F32)
        _phase_a(cfg, barrier, x, wqkv, woa, staged, (wops2, wops), oops, kbuf, vbuf, ckv,
                 xops, cops, (stq, stk, stv), qall, outa)
        if cfg.get("nodeps"):
            for a, b in ((kbuf.at[0, 0:8], vbuf.at[0, 0:8]), (vbuf.at[1, 0:8], kbuf.at[1, 0:8]), (staged.at[0, 0:8], kbuf.at[2, 0:8]),
                         (wops2.at[0, 0], oops.at[0, 0, 0:T]), (oops.at[1, 0, 0:T], wops2.at[1, 0]), (stq.at[0:8], stk.at[0:8]),
                         (stk.at[8:16], stv.at[0:8]), (stv.at[8:16], stq.at[8:16]), (xops.at[0, 0, 0:T], wops2.at[2, 0])):
                cp = pltpu.make_async_copy(a, b, sems.at[5])
                cp.start()
                cp.wait()

    (pl.run_scoped if not cfg.get("skip_a") else (lambda *a: None))(
        first,
        pltpu.VMEM((S, DM), BF16), pltpu.VMEM((DM, 3 * DM), BF16), pltpu.VMEM((DM, DM), BF16),
        pltpu.VMEM((8, HA * PITCH_A, T), F32), pltpu.VMEM((4, NPROD, T, T), BF16),
        pltpu.VMEM((NPROD, 2, 2 * T, T), BF16),
        pltpu.VMEM((8, HALO + S, T), F32), pltpu.VMEM((8, HALO + S + 8, T), F32),
        pltpu.VMEM((S, DC), BF16),
        pltpu.VMEM((NPROD, 2, S // N, T), BF16),
        pltpu.VMEM((DM * PITCH_B, T), U32))

    def second(ctx):
        load_wo = [pltpu.make_async_copy(wob_h.at[:, :, pl.ds(j * T, T)], qall.at[2 * j:2 * j + 2], sems.at[4 + j])
                   for j in range(8)]

        def pair(i, carry):
            @pl.when(i == 8)
            def _():
                for cp in load_wo:
                    cp.start()
            _pair_body(cfg, i, cops, stk, stv, wops, qall, ctx)
            return carry
        if not cfg.get("skip_b"):
            if cfg.get("scopes"):
                with jax.named_scope("block_B"):
                    lax.fori_loop(0, HB // 2, pair, 0)
            else:
                lax.fori_loop(0, HB // 2, pair, 0)
        else:
            for cp in load_wo:
                cp.start()
        for cp in load_wo + ([] if cfg.get("skip_a") else copy_a):
            cp.wait()
        if cfg.get("skip_o"):
            cp = pltpu.make_async_copy(ctx.at[0, 0], ctx.at[1, 1], sems.at[0])
            cp.start()
            cp.wait()
        else:
            if cfg.get("scopes"):
                with jax.named_scope("block_O"):
                    _phase_o(cfg, ctx, qall, outa, out_h, sems)
            else:
                _phase_o(cfg, ctx, qall, outa, out_h, sems)

    if cfg.get("only_a"):
        for i, src in enumerate((qall.at[0], cops.at[0, 0], wops.at[0, 0])):
            cp = pltpu.make_async_copy(src, out_h.at[pl.ds(0, src.shape[0]), pl.ds(DM + i * T, T)], sems.at[5])
            cp.start()
            cp.wait()
        if not cfg.get("nodeps"):
            for cp in copy_a:
                cp.wait()
        return
    pl.run_scoped(second, pltpu.VMEM((S // T, HB, T, T), F32))


def _call(cfg, A_x, A_wqkv, A_wo, B_x, B_c_kv, B_w_q, B_w_uk, B_w_uv, B_w_o):
    any_spec = pl.BlockSpec(memory_space=pl.ANY)
    out = pl.pallas_call(
        lambda *refs: _kernel(cfg, *refs),
        out_shape=jax.ShapeDtypeStruct((S, 2 * DM), BF16),
        in_specs=[any_spec] * 9,
        out_specs=any_spec,
        scratch_shapes=[
            pltpu.VMEM((NPROD, 1, S // N, T), BF16),
            pltpu.VMEM((DC * PITCH_B, T), U32),
            pltpu.VMEM((DC * PITCH_B, T), U32),
            pltpu.VMEM((4, NPROD, T, T), BF16),
            pltpu.VMEM((HB, S, T), BF16),
            pltpu.VMEM((S, DM), BF16),
            pltpu.SemaphoreType.DMA((24,)),
        ],
        compiler_params=pltpu.CompilerParams(vmem_limit_bytes=126 * 1024 * 1024),
        name="concat_heads",
    )(A_x.reshape(S, DM), A_wqkv, A_wo, B_x.reshape(S, DM), B_c_kv.reshape(S, DC),
      B_w_q.reshape(16, S, T), B_w_uk.reshape(8, S, T), B_w_uv.reshape(8, S, T),
      B_w_o.reshape(2, S, DM))
    return out.reshape(1, S, 2 * DM)


@jax.jit
def pallas_concat_heads__sliding_local_dilated__compressed_kv_cla__prompt_kernel(
    A_x: jax.Array,
    A_wqkv: jax.Array,
    A_wo: jax.Array,
    B_x: jax.Array,
    B_c_kv: jax.Array,
    B_w_q: jax.Array,
    B_w_uk: jax.Array,
    B_w_uv: jax.Array,
    B_w_o: jax.Array,
):
    return _call(CFG, A_x, A_wqkv, A_wo, B_x, B_c_kv, B_w_q, B_w_uk, B_w_uv, B_w_o)
```

```python
import functools

import numpy as np

import jax
import jax.numpy as jnp
from jax import lax
import jax.experimental.pallas as pl
import jax.experimental.pallas.tpu as pltpu

F32, BF16, U32 = jnp.float32, jnp.bfloat16, jnp.uint32
LOG2E = float(np.log2(np.e))
NEG = -1e9 * LOG2E
T = 128
N = 4
NPROD = 49
ROWS = N * T

S = 2048
DM = 1024
DC = 512
HB = 32
WIN, DIL, HA, DH_A = 8, 2, 32, 32
HALO = 16
G = 16
PITCH_B = 17
PITCH_A = 33

CFG = dict(a_order="x", b_order="x", lag=8, p_j=8, mix_j=4, mix_p=4, pv=4, group=8, o_flush=(315, 329, 336, 339, 341, 342), o_piece=128, o_lag=2, o_cap=250, o_span=49, o_start=1, o_end=1, o_order="y",  b_lag=6, b_rate=(40, 32), b_wait=6, b_late=4, b_small=(16, 0), b_each=1, b_deep=4, b_span=8, b_qtie=0, b_wtie=1, b_cost=32, b_proj=(0, 0), b_prep=(9, 1),
           steps="""
    |z>b r56 s1,0,2 F0 |a>c s1,2,4 F1 |b>d r96 s1,4,8 w1,0 F2 |c>e x1 F3 r56 w1,1 K1,0
    |d>f x2 K1,1 r48 x3 K2,0 x0 K2,1 |e>gh s0 w0,0 K3,0 K3,1 w0,1 Q0,0 s2 w2,0 Q0,1 p0 Q1,0 w2,1 Q1,1 Q2,0 Q2,1
    Q3,0 Q3,1 |f>ij tq W0 V0,0 V0,1 V1,0
    |g> b0 V1,1 b1 V2,0 p1 V2,1 b2 V3,0 V3,1 b3 W1 P0,0 P0,1 P0,2 P0,3
    m0 W2 P1,0 P1,1 s3 P1,2 P1,3 w3,0 W3 o0 P2,0 P2,1 P2,2 w3,1 P2,3
    |hij> W4 tv p2 P3,0 P3,1 P3,2 P3,3 m1 O0,0 O0,1 W5 o1 P4,0 P4,1 tk P4,2 P4,3
    W6 p3 O1,0 O1,1 |>01 P5,0 P5,1 m2 P5,2 P5,3 W7 o2
    P6,0 m3 P6,1 P6,2 P6,3 o3 O2,0 O2,1 c0 c1 P7,0 P7,1 c2 c3 U P7,2 P7,3 O3,0 O3,1 |>23""")


def _mm(a, b):
    return jnp.dot(a, b, preferred_element_type=F32)


def _mm_nt(a, b):
    return lax.dot_general(a, b, (((1,), (1,)), ((), ())), preferred_element_type=F32)


def _cat(xs, axis):
    xs = list(xs)
    return xs[0] if len(xs) == 1 else lax.concatenate(xs, axis)


def _rows(x, start, size):
    return lax.slice_in_dim(x, start, start + size, axis=0)


def _fold(op, xs):
    xs = list(xs)
    acc = xs[0]
    for x in xs[1:]:
        acc = op(acc, x)
    return acc


def _bf(words):
    return pltpu.bitcast(words, BF16)


def _words(x):
    return pltpu.bitcast(x, U32)


def _reciprocal(x):
    r = pltpu.reciprocal(x, approx=True)
    return r * (2.0 - x * r)


def _quads(g, n):
    h = n // 2
    return [{(r, c): g[(r + i * h, c + j * h)] for r in range(h) for c in range(h)}
            for i in range(2) for j in range(2)]


def _gadd(x, y):
    return {k: lax.add(x[k], y[k]) for k in x}


def _gsub(x, y):
    return {k: lax.sub(x[k], y[k]) for k in x}


ORDERS = {
    "x": (((2, 1, 3), (0, 1, 1), (3,), (1, -1, 3), (0, 1, 3), (0,), (2, -1, 0)),
          ((0,), (3,), (2, -1, 0), (2, 1, 3), (0, 1, 3), (1, -1, 3), (0, 1, 1))),
    "y": (((0,), (3,), (2, 1, 3), (2, -1, 0), (0, 1, 3), (0, 1, 1), (1, -1, 3)),
          ((1, -1, 3), (2, -1, 0), (0,), (0, 1, 1), (0, 1, 3), (3,), (2, 1, 3)))}
LEFT, RIGHT = ORDERS["x"]


def _factor(rule, quad):
    if len(rule) == 1:
        return quad(rule[0])
    return (_gadd if rule[1] > 0 else _gsub)(quad(rule[0]), quad(rule[2]))


def _factors(rules, g, n=N):
    if n == 1:
        return [g[(0, 0)]]
    quads = _quads(g, n)
    return [x for rule in rules for x in _factors(rules, _factor(rule, quads.__getitem__), n // 2)]


def _combine(product, emit, n=N, base=0, order="x"):
    if n == 1:
        return emit(0, 0, product(base))
    h = n // 2
    a, b, s = {}, {}, {}

    def use(i, r, c, m):
        k = r, c
        if i == 0:
            a[k] = m
        elif i == 1:
            b[k] = m
        elif i == 2:
            emit(r + h, c, lax.add(a[k], m))
            s[k] = lax.sub(m, b[k])
        elif i == 3:
            s[k] = lax.add(s[k], m)
        elif i == 4:
            emit(r, c, lax.add(s[k], m))
            s[k] = lax.sub(m, a[k])
        elif i == 5:
            emit(r, c + h, lax.add(b[k], m))
            s[k] = lax.add(s[k], m)
        else:
            emit(r + h, c + h, lax.add(s[k], m))

    def use_y(i, r, c, m):
        k = r, c
        if i == 0:
            a[k] = m
        elif i == 1:
            b[k] = m
        elif i == 2:
            emit(r + h, c, lax.add(b[k], m))
            s[k] = lax.sub(a[k], m)
        elif i == 3:
            s[k] = lax.add(s[k], m)
        elif i == 4:
            emit(r + h, c + h, lax.add(s[k], m))
            s[k] = lax.add(b[k], m)
        elif i == 5:
            emit(r, c + h, lax.add(a[k], m))
            s[k] = lax.sub(s[k], m)
        else:
            emit(r, c, lax.add(s[k], m))

    for i in range(7):
        _combine(product, lambda r, c, m, i=i: (use if order == "x" else use_y)(i, r, c, m), h,
                 base + i * 7 ** (h.bit_length() - 1), order)


class _SideWork:
    def __init__(self, lag, never=None):
        self.lag, self.never = lag, never
        self.urgent, self.todo, self.running, self.results = [], [], [], []
        self.clock, self.credit, self.rate, self.cache = 0, 0.0, 0.0, (None,)

    def after(self, x, groups=1):
        old = [r for r in self.results if r[0] <= self.clock - self.lag]
        if not old:
            return x
        key = (self.clock, x.shape, x.dtype == F32)
        if self.cache[0] != key:
            deps = [_rows(value, row, 8) for _, value, row in
                    (old[max(0, len(old) - 1 - 2 * n)] for n in reversed(range(groups)))]
            deps = [_cat([dep if x.dtype == F32 else _words(dep)] * (x.shape[1] // T), 1) for dep in deps]
            self.cache = (key, _cat([dep for dep in deps for _ in range(x.shape[0] // 8 // groups)], 0), self.never(x.shape))
        return lax.select(self.cache[2], self.cache[1], x)

    def before(self, words, most):
        due = [x for t, x in self.running[:most] if t <= self.clock]
        if not due:
            return words
        del self.running[:len(due)]
        parts = [_rows(words, r, 8) for r in range(0, T // 2, 8)]
        for i, x in enumerate(due):
            dep = _fold(lax.bitwise_or, [_words(_rows(x, r, 8)) for r in range(0, x.shape[0], 8)])
            parts[i * 8 // len(due)] = lax.select(self.never((8, T)), dep, parts[i * 8 // len(due)])
        return _cat(parts, 0)

    def add(self, cost, run, wait=0, urgent=False):
        (self.urgent if urgent else self.todo).append((self.clock + wait, cost, run))

    def issued(self, tiles, result):
        for i in range(2 * tiles):
            self.clock += 0.5
            self.results = self.results[-40:] + [(self.clock, result, i * (result.shape[0] // G) // (2 * tiles) * G)]
            self.credit += 0.5 * self.rate
            while self.credit > 0:
                ready = [x for x in (self.urgent, self.todo) if x and x[0][0] <= self.clock]
                if not ready:
                    break
                _, cost, run = ready[0].pop(0)
                self.credit -= cost
                run()
            self.credit = min(self.credit, 0.0)

    def finish(self, done=lambda: False):
        while (self.urgent or self.todo) and not done():
            (self.urgent or self.todo).pop(0)[2]()


def _queue_factors(side, rules, load, dst):
    def piece(outer):
        def run():
            h = N // 2
            quad = lambda x: {(r, c): load(x // 2 * h + r, x % 2 * h + c) for r in range(h) for c in range(h)}
            for i, x in enumerate(_factors(rules, _factor(rules[outer], quad), h)):
                ref, idx = dst(outer * 7 + i)
                ref[idx] = lax.convert_element_type(x, BF16)
        return run
    for outer in range(7):
        side.add(50, piece(outer))


def _queue_activation(side, src, dst, chunk, order):
    kt = src.shape[1] // (N * T)
    for t in range(kt):
        for r0 in range(0, T, G):
            def load(r, c, t=t, r0=r0):
                lo, col = chunk * ROWS + r * T + r0, (c * kt + t) * T
                return lax.convert_element_type(_bf(side.after(_words(src[lo:lo + G, col:col + T]))), F32)
            _queue_factors(side, ORDERS[order][0], load, lambda i, t=t, r0=r0: (dst[chunk], (i, t, pl.ds(r0, G))))


def _queue_head_weights(side, columns, kt, scale, wops, order):
    high, shift = jnp.full((G, T), 0xFFFF0000, U32), jnp.full((G, T), 16, U32)
    for t in range(kt):
        for r0 in range(0, T, G):
            def load(r, c, t=t, r0=r0):
                ref, word, half = columns[c]
                w = side.after(ref[pl.ds(word + ((kt * r + t) * T + r0) * PITCH_B, G, stride=PITCH_B), :])
                w = pltpu.bitcast(lax.bitwise_and(w, high) if half else lax.shift_left(w, shift), F32)
                return w if scale is None else w * scale
            _queue_factors(side, ORDERS[order][1], load, lambda i, t=t, r0=r0: (wops, (i, t, pl.ds(r0, G))))


def _queue_kv_weights(side, pair, stk, stv, wops, order):
    _queue_head_weights(side, [(stk, pair, 0), (stk, pair, 1), (stv, pair, 0), (stv, pair, 1)], 1, None, wops, order)


def _tile(ref, *idx):
    *lead, row = idx
    return ref.bitcast(U32)[(*lead, pl.ds(row * (T // 2), T // 2))]


def _phase_a(cfg, barrier, x, wqkv, woa, staged, wops, oops, kbuf, vbuf, ckv, xops, cops, stb, qall, outa):
    side = _SideWork(cfg["lag"])
    q = {}
    done = set()

    def check(step, user):
        assert step is None or step in done or cfg.get("nodeps"), (user, "must come after", step)

    def stage(sec, i):
        def run():
            if sec < 3:
                w = _bf(side.after(_words(wqkv[i * T:(i + 1) * T, sec * DM:(sec + 1) * DM]))).T
            else:
                w = _bf(side.after(_words(woa[:, i * T:(i + 1) * T])))
            w = w.astype(F32)
            for h in range(HA):
                staged[i, h * PITCH_A:h * PITCH_A + DH_A, :] = w[h * DH_A:(h + 1) * DH_A]
        return run

    def weights(sec, g, t, r0):
        def permuted(slab, j):
            w = side.after(staged[slab, pl.ds(r0 % HA * PITCH_A + 4 * j + r0 // HA, G, stride=PITCH_A), :])
            return w * (float(DH_A ** -0.5) * LOG2E) if sec == 0 else w

        load = (lambda r, c: permuted(2 * r + t, g * N + c)) if sec < 3 else (
            lambda r, c: permuted(g * N + c, 2 * r + t))
        _queue_factors(side, ORDERS[cfg["a_order"]][1], load, lambda i: (wops[sec == 0][g], (i, t, pl.ds(r0, G))))

    def project(sec, c, g):
        needs = [("w", sec, g), ("o" if sec == 3 else "x", c)]
        side.finish(lambda: cfg.get("nodeps") or all(n in done for n in needs))
        for n in needs:
            check(n, (sec, c, g))

        left, right = xops[c] if sec < 3 else oops[c % 2], wops[sec == 0][g]

        def product(i):
            a, w = (_cat([_tile(left, i, t, 0) for t in range(2)], 1), [_tile(right, i, t, 0) for t in range(2)])
            out = _mm_nt(_bf(a), _bf(_cat(w, 1))) if sec < 3 else _mm(_bf(a), _bf(_cat(w, 0)))
            side.issued(2, out)
            return out

        def emit(r, col, val):
            r0, j = c * ROWS + r * T, g * N + col
            if sec == 0:
                q[(r0, j)] = val
            elif sec == 3:
                outa[r0:r0 + T, j * T:(j + 1) * T] = val.astype(BF16)
            else:
                (kbuf if sec == 1 else vbuf)[j, HALO + r0:HALO + r0 + T, :] = val

        _combine(product, emit, order=cfg["a_order"])

    def first_keys(r):
        side.finish(lambda: ("s", 1, 2 * r + 1) in done)
        for j in range(8):
            w = _cat([_cat([staged[slab, pl.ds(4 * j + d, HA, stride=PITCH_A), :] for d in range(4)], 0)
                      for slab in (2 * r, 2 * r + 1)], 1)
            out = _mm_nt(x[0:ROWS, 2 * r * T:(2 * r + 2) * T], w.astype(BF16))
            side.issued(2 * N, _rows(out, ROWS - T, T))
            kbuf[j, HALO:HALO + ROWS, :] = out + kbuf[j, HALO:HALO + ROWS, :] if r else out

    def project_queries(quad, c):
        needs = [("W", quad), ("b", c), ("t", "qqqqvvkk"[quad])]
        side.finish(lambda: cfg.get("nodeps") or all(n in done for n in needs))
        for n in needs:
            check(n, ("P", quad, c))

        left, right = xops[c], wops[1][quad % 2]

        def product(i):
            out = _mm(_bf(_cat([_tile(left, i, t, 0) for t in range(2)], 1)),
                      _bf(_cat([_tile(right, i, t, 0) for t in range(2)], 0)))
            side.issued(2, out)
            return out

        def emit(r, h, val):
            qall[4 * quad + h, c * ROWS + r * T:c * ROWS + (r + 1) * T, :] = val.astype(BF16)

        _combine(product, emit, order=cfg["a_order"])

    E = cfg["group"]
    row = lax.broadcasted_iota(jnp.int32, (E, T), 0)

    lane = lax.broadcasted_iota(jnp.int32, (E, T), 1)

    def group_sums(a, b, c, d):
        even, low = (lane & HA) == 0, lane < 2 * HA
        fold = lambda pick, x, y, shift: lax.select(pick, x, y) + pltpu.roll(lax.select(pick, y, x), shift, 1)
        z = fold(low, fold(even, a, b, 3 * HA), fold(even, c, d, 3 * HA), 2 * HA)
        zr = pltpu.roll(z, 2 * HA, 1)
        out = []
        for x in (lax.select(low, z, zr), lax.select(low, zr, z)):
            xr = pltpu.roll(x, HA, 1)
            out += [lax.select(even, x, xr), lax.select(even, xr, x)]
        return out

    def probs(r0):
        def run():
            qs = side.after(_cat([_rows(q[(r0 - r0 % T, j)], r0 % T, E) for j in range(8)], 0)).reshape(8, E, T)
            J = cfg["p_j"]
            qs = [_rows(qs, j, J) for j in range(0, 8, J)]
            parts = []
            for w in range(WIN):
                lo = HALO + r0 - DIL * w
                s = jnp.sum(_fold(lax.add, [lax.mul(qs[j // J], kbuf[j:j + J, lo:lo + E, :]) for j in range(0, 8, J)]), axis=0)
                parts.append(s)
            logits = []
            if cfg.get("rs"):
                for w in range(0, WIN, 4):
                    logits += group_sums(*parts[w:w + 4])
            else:
                for s in parts:
                    s = s + pltpu.roll(s, 2 * HA, 1)
                    logits.append(s + pltpu.roll(s, HA, 1))
            logits = [jnp.where(row + r0 >= DIL * w, s, NEG) if r0 < DIL * w else s for w, s in enumerate(logits)]
            m = _fold(jnp.maximum, logits)
            e = [jnp.exp2(s - m) for s in logits]
            inv = _reciprocal(_fold(jnp.add, e))
            for w in range(WIN):
                kbuf[w, r0:r0 + E, :] = e[w] * inv
        return run

    def mix(r0, js):
        def run():
            J = cfg["mix_j"]
            p = side.after(kbuf[:, r0:r0 + E, :].reshape(WIN * E, T))
            p = [lax.broadcast(_rows(p, w * E, E), (J,)) for w in range(WIN)]
            for j in js:
                vbuf[j:j + J, r0:r0 + E, :] = _fold(lax.add, [
                    lax.mul(p[w], vbuf[j:j + J, HALO + r0 - DIL * w:HALO + r0 - DIL * w + E, :]) for w in range(WIN)])
        return run

    def queue_output(c):
        for t in range(2):
            for r0 in range(0, T, G):
                def load(r, col, t=t, r0=r0):
                    lo = c * ROWS + r * T + r0
                    return side.after(vbuf[2 * col + t, lo:lo + G, :])
                _queue_factors(side, ORDERS[cfg["a_order"]][0], load, lambda i, t=t, r0=r0: (oops[c % 2], (i, t, pl.ds(r0, G))))

    def stage_heads(base, st, m0, count):
        def run():
            lo = m0 * HB // 2
            w = side.after(qall.bitcast(U32)[base + lo // (S // 2), pl.ds(lo % (S // 2), count * HB // 2), :])
            for i in range(count):
                st[(m0 + i) * PITCH_B:(m0 + i) * PITCH_B + HB // 2, :] = _rows(w, i * HB // 2, HB // 2)
        return run

    scope = []
    for step in cfg["steps"].split():
        kind, arg = step[0], step[1:]
        num = [int(a) for a in arg.split(",")] if arg[:1].isdigit() else []
        if kind == "|":
            if side.clock == 0:
                side.finish()
            if cfg.get("scopes"):
                if scope:
                    scope.pop().__exit__(None, None, None)
                with jax.named_scope(f"wait_{side.clock:06.0f}_{arg}"):
                    barrier(*arg.split(">"))
                scope.append(jax.named_scope(f"block_{side.clock:06.0f}_{arg}"))
                scope[-1].__enter__()
            else:
                barrier(*arg.split(">"))
            zeros = vbuf[0, HALO + S:HALO + S + 8, :]
            side.results = []
            side.never = lambda shape, z=zeros: _cat([_cat([z] * (shape[1] // T), 1)] * (shape[0] // 8), 0) != 0
        elif kind == "r":
            side.rate = num[0]
        elif kind in "QKVO":
            project("QKVO".index(kind), *num)
            done.add((kind, *num))
        elif kind == "s":
            for i in range(*num[1:]) if num[1:] else range(8):
                side.add(320, stage(num[0], i))
                side.add(0, lambda key=("s", num[0], i): done.add(key))
        elif kind == "F":
            first_keys(*num)
        elif kind == "P":
            project_queries(*num)
            done.add((kind, *num))
        elif kind in "wxobW":
            key = (kind, *num)
            frees = {"w": {1: None, 0: None, 2: ("K", 3, num[-1]), 3: ("V", 3, num[-1])}.get(num[0]) if kind == "w" else None,
                     "x": None, "b": ("V", num[0], 1), "o": ("O", num[0] - 2, 1) if num[0] >= 2 else None,
                     "W": ("P", num[0] - 2, 3) if num[0] >= 2 else ("Q", 3, num[0])}[kind]
            side.add(0, lambda frees=frees, key=key: check(frees, key))
            if kind == "w":
                for t in range(2):
                    for r0 in range(0, T, G):
                        weights(*num, t, r0)
            elif kind in "xb":
                _queue_activation(side, x, xops, *num, cfg["a_order"])
            elif kind == "W":
                _queue_head_weights(side, [(stb[0], 2 * num[0] + h // 2, h % 2) for h in range(4)], 2,
                                    float(T ** -0.5) * LOG2E, wops[1][num[0] % 2], cfg["a_order"])
            else:
                queue_output(*num)
            side.add(0, lambda key=(kind, *num): done.add(key))
        elif kind in "pm":
            check(("Q" if kind == "p" else "V", num[0], 1), step)
            for r0 in range(num[0] * ROWS, (num[0] + 1) * ROWS, E):
                if kind == "p":
                    side.add(28 * E, probs(r0))
                else:
                    for j in range(0, 8, cfg["mix_p"]):
                        side.add(2 * E * cfg["mix_p"] + E, mix(r0, range(j, j + cfg["mix_p"], cfg["mix_j"])))
        elif kind == "c":
            _queue_activation(side, ckv, cops, *num, cfg["b_order"])
        elif kind == "t":
            st = stb["qkv".index(arg)]
            for m0 in range(0, st.shape[0] // PITCH_B, 4):
                side.add(24, stage_heads({"q": 0, "v": 16, "k": 24}[arg], st, m0, 4))
            side.add(0, lambda key=("t", arg): done.add(key))
        elif kind == "U":
            _queue_kv_weights(side, 0, stb[1], stb[2], wops[1][0], cfg["b_order"])
    side.finish()
    if scope:
        scope.pop().__exit__(None, None, None)


def _pair_body(cfg, pair, cops, stk, stv, wops, qall, ctx):
    side = _SideWork(cfg["b_lag"], lambda shape: lax.broadcast(pair < 0, shape))
    side.rate = cfg["b_rate"][0]
    k, v = {}, {}

    def product(j, i):
        out = _mm(_bf(side.before(_tile(cops[j], i, 0, 0), 1)), _bf(side.before(_tile(wops, i, 0, 0), cfg["b_wtie"])))
        side.issued(1, out)
        return out

    def project(j):
        def emit(r, c, val):
            (k if c < 2 else v)[(c % 2, N * j + r)] = val

        _combine(functools.partial(product, j), emit, order=cfg["b_order"])

    causal = lax.broadcasted_iota(jnp.int32, (T, T), 1) <= lax.broadcasted_iota(jnp.int32, (T, T), 0)

    def scores(h, i):
        s = _mm_nt(_bf(side.before(_tile(qall, 2 * pair + h, i), cfg["b_qtie"])), _cat([k[(h, t)] for t in range(i + 1)], 0).astype(BF16))
        s = [s[:, t * T:(t + 1) * T] for t in range(i + 1)]
        for t in range(0, i + 1, 4):
            side.issued(min(4, i + 1 - t), s[t])
        s[i] = jnp.where(causal, s[i], NEG)
        return s, jnp.max(_fold(jnp.maximum, s), axis=1, keepdims=True)

    def attend(h, i, s, m):
        e = [jnp.exp2(x - m) for x in s]
        acc = None
        for t in range(0, i + 1, cfg["pv"]):
            ts = range(t, min(t + cfg["pv"], i + 1))
            part = _mm(_cat([e[u] for u in ts], 1).astype(BF16), _cat([v[(h, u)] for u in ts], 0).astype(BF16))
            acc = part if acc is None else acc + part
            side.issued(len(ts), acc)

        def normalize(r0):
            def run():
                part = side.after(_fold(lax.add, [_rows(x, r0, G) for x in e]))
                out = _rows(acc, r0, G) * _reciprocal(jnp.sum(part, axis=1, keepdims=True))
                ctx[i, 2 * pair + h, r0:r0 + G, :] = out
                side.running.append((side.clock + cfg["b_span"], out))
            return run
        for r0 in range(0, T, G):
            side.add(cfg["b_cost"] + 2 * i, normalize(r0), cfg["b_wait"], urgent=True)

    late = cfg["b_late"]
    project(0)
    project(1)
    live, last, small = [], [], [(h, i) for i in reversed(range(late)) for h in range(2)]
    for i in range(late, S // T):
        for h in range(2):
            live.append((h, i, *scores(h, i)))
            if (i % N, h) == tuple(cfg["b_proj"]) and 0 < i // N < S // ROWS - 1:
                project(i // N + 1)
            if (i, h) == tuple(cfg["b_prep"]):
                side.rate = cfg["b_rate"][1]
                _queue_kv_weights(side, jnp.minimum(pair + 1, HB // 2 - 1), stk, stv, wops, cfg["b_order"])
            if small and (i, h) >= tuple(cfg["b_small"]):
                for _ in range(cfg["b_each"]):
                    u = small.pop(0)
                    last.append((*u, *scores(*u)))
            while len(live) > (2 if i < cfg["b_deep"] else 1):
                attend(*live.pop(0))
    for unit in live + last + [(*u, *scores(*u)) for u in small]:
        attend(*unit)
    side.results = []
    side.finish()


def _phase_o(cfg, ctx, wob, sums, spare, stage, out_h, sems):
    n = 2 * N
    kt, mt = HB // n, S // T // n
    rules = ORDERS[cfg["o_order"]]
    P = cfg["o_piece"]
    zeros = stage.bitcast(U32)[S // 2:S // 2 + 8, 0:T]
    side = _SideWork(cfg["o_lag"], lambda shape: _cat([zeros] * (shape[0] // 8), 0) != 0)

    def context(r, c):
        return [lambda lo, size, m=m, t=t: ctx[r * mt + m, c * kt + t, lo:lo + size, :]
                for m in range(mt) for t in range(kt)]

    def weight(r, c):
        return [lambda lo, size, t=t: _bf(wob.bitcast(U32)[
            2 * c + r // N, pl.ds(((r % N * kt + t) * T + lo) // 2, size // 2), :]).astype(F32) for t in range(kt)]

    def lazy(rule, g, n):
        quads = _quads(g, n)
        if len(rule) == 1:
            return quads[rule[0]]
        op = lax.add if rule[1] > 0 else lax.sub
        return {k: [functools.cache(lambda lo, size, x=x, y=y: op(x(lo, size), y(lo, size)))
                    for x, y in zip(quads[rule[0]][k], quads[rule[2]][k])] for k in quads[0]}

    def stored(rules, rule, g, slots, jobs):
        quads = _quads(g, n)
        first = _quads(quads[rule[0]], n // 2)
        out = [first[inner[0]] if len(rule + inner) == 2 else {k: [] for k in first[0]} for inner in rules]
        for k in first[0]:
            for t in range(len(first[0][k])):
                where = {j: next(slots) for j, inner in enumerate(rules) if len(rule + inner) > 2}
                for j, slot in where.items():
                    out[j][k].append(lambda lo, size, slot=slot: pltpu.bitcast(slot[0][(*slot[1:-1], pl.ds(slot[-1] + lo, size))], F32))
                for lo in range(0, T, P):
                    def run(k=k, t=t, lo=lo, where=where):
                        def load(q):
                            tie = (lambda x: side.after(x, P // G)) if q == rule[0] else lambda x: x
                            return {i: tie(x[k][t](lo, P)) for i, x in enumerate(_quads(quads[q], n // 2))}
                        top = _factor(rule, load)
                        for j, slot in where.items():
                            slot[0][(*slot[1:-1], pl.ds(slot[-1] + lo, P))] = _words(_factor(rules[j], lambda q: {0: top[q]})[0])
                    jobs.append((len(where) * P // 8, run))
        return out

    a = {(r, c): context(r, c) for r in range(n) for c in range(n)}
    b = {(r, c): weight(r, c) for r in range(n) for c in range(n)}
    jobs = [[] for _ in range(8)]
    operands = []
    for i in range(7):
        slots = [(sums[i % 2], lo) for lo in range(0, sums[i % 2].shape[0], T)]
        if i % 2:
            slots += [(ref, lo) for ref in spare for lo in range(0, ref.shape[0] - T + 1, T)]
            slots += [(wob.bitcast(U32), h, lo) for h in range(HB // 2, HB) for lo in range(0, S // 2, T)]
        slots = iter(slots)
        mid = [stored(rules[s], rules[s][i], g, slots, jobs[i]) if i else
               [lazy(rule, top, n // 2) for top in [lazy(rules[s][i], g, n)] for rule in rules[s]] for s, g in enumerate((a, b))]
        operands += [[lazy(rules[s][k], mid[s][j], n // 4)[0, 0] for s in range(2)] for j in range(7) for k in range(7)]

    def room(i):
        left, level = cfg["o_cap"], i
        for _ in range(3):
            left -= mt * 16 * (level % 7 != 6)
            if level % 7 not in (2, 4, 5, 6):
                break
            level //= 7
        for s, size in enumerate((mt * kt * 16, kt * 16)) if i < NPROD else ():
            seen = {q for k in range(i % 7) for q in rules[s][k][::2]}
            left -= size * len(set(rules[s][i % 7][::2]) - seen) * (len(rules[s][i // 7 % 7]) > 1)
        return max(left, 0)

    ready, started = [], []

    def send(r, c, size):
        rows, cols = pl.ds(r * mt * T, size * mt * T), pl.ds(c * T, size * T)
        started.append(pltpu.make_async_copy(stage.at[rows, cols], out_h.at[rows, pl.ds(DM + c * T, size * T)], sems.at[0]))
        started[-1].start()

    def flush():
        if len(ready) == N * N:
            send(*min(ready), N)
        else:
            for r, c in ready:
                send(r, c, 1)
        ready.clear()

    def emit(r, c, val):
        stage[r * mt * T:(r + 1) * mt * T, c * T:(c + 1) * T] = val.astype(BF16)
        ready.append((r, c))

    zero = pltpu.bitcast(zeros, jnp.int32)[0, 0]

    def product(i):
        if i % NPROD == 0 and i:
            @pl.when(zero > 0)
            def _():
                for ref in sums:
                    ref[pl.ds(pl.multiple_of(8 * jnp.clip(zero, 0, 1), 8), 8), :] = jnp.zeros((8, T), U32)
            side.results = []
        if i % NPROD == 0 or i in cfg["o_flush"]:
            flush()
        x, y = ([tile(0, T) for tile in g] for g in operands[i])
        out = _mm(_cat([_cat(x[m * kt:(m + 1) * kt], 1) for m in range(mt)], 0).astype(BF16), _cat(y, 0).astype(BF16))
        queue = jobs[i // NPROD + 1]
        left = sum(room(k) for k in range(i, i - i % NPROD + cfg["o_span"]))
        share = sum(cost for cost, _ in queue) * (1 if left <= room(i) else room(i) / left)
        side.rate, side.credit = share / (mt * kt), 0.0
        while share > 0 and queue:
            share -= queue[0][0]
            side.add(*queue.pop(0))
        side.issued(mt * kt, out)
        side.finish()
        return out

    _combine(product, emit, n, 0, cfg["o_order"])
    flush()
    for cp in started:
        cp.wait()


def _kernel(cfg, xa_h, wqkv_h, woa_h, xb_h, ckv_h, wq_h, wuk_h, wuv_h, wob_h, out_h,
            cops, stk, stv, wops, qall, outa, sems):
    copy_a = [pltpu.make_async_copy(outa.at[pl.ds(c * ROWS, ROWS)], out_h.at[pl.ds(c * ROWS, ROWS), pl.ds(0, DM)],
                                    sems.at[c]) for c in range(S // ROWS)]

    def first(x, wqkv, woa, staged, wops2, oops, kbuf, vbuf, ckv, xops, stq):
        def x_rows(lo, hi):
            return xa_h.at[pl.ds(lo, hi - lo)], x.at[pl.ds(lo, hi - lo)]

        def w_cols(sec):
            return wqkv_h.at[:, pl.ds(sec * DM, DM)], wqkv.at[:, pl.ds(sec * DM, DM)]

        def quarter(r):
            k = pl.ds(r * DM // N, DM // N)
            return [(wqkv_h.at[k, pl.ds(DM, DM)], wqkv.at[k, pl.ds(DM, DM)]),
                    (xa_h.at[pl.ds(0, ROWS), k], x.at[pl.ds(0, ROWS), k])]

        groups = {
            "z": quarter(0), "a": quarter(1), "b": quarter(2) + quarter(3),
            "c": [x_rows(ROWS, 2 * ROWS)],
            "d": [x_rows(2 * ROWS, S)],
            "e": [w_cols(0), w_cols(2), (woa_h, woa)],
            "f": [(wq_h, qall.at[0:16])],
            "g": [(xb_h, x)],
            "h": [(wuv_h, qall.at[16:24])],
            "i": [(wuk_h, qall.at[24:32])],
            "j": [(ckv_h, ckv)],
        }
        slot = iter(range(4, 24))
        copies = {k: [pltpu.make_async_copy(src, dst, sems.at[next(slot)]) for src, dst in v]
                  for k, v in groups.items()}
        copies.update({str(c): [cp] for c, cp in enumerate(copy_a)})

        def barrier(wait, start):
            for name in wait:
                for cp in copies[name]:
                    cp.wait()
            for name in start:
                for cp in copies[name]:
                    cp.start()

        barrier("", "za")
        kbuf[:, 0:HALO, :] = jnp.zeros((8, HALO, T), F32)
        vbuf[:, 0:HALO, :] = jnp.zeros((8, HALO, T), F32)
        vbuf[0, HALO + S:HALO + S + 8, :] = jnp.zeros((8, T), F32)
        _phase_a(cfg, barrier, x, wqkv, woa, staged, (wops2[:2], [wops, wops2[2]]), oops, kbuf, vbuf, ckv,
                 xops, cops, (stq, stk, stv), qall, outa)

    factors = pltpu.VMEM((NPROD, 2, T, T), BF16)
    (pl.run_scoped if not cfg.get("skip_a") else (lambda *a: None))(
        first,
        pltpu.VMEM((S, DM), BF16), pltpu.VMEM((DM, 3 * DM), BF16), pltpu.VMEM((DM, DM), BF16),
        pltpu.VMEM((8, HA * PITCH_A, T), F32), [factors] * 3, [factors] * 2,
        pltpu.VMEM((8, HALO + S, T), F32), pltpu.VMEM((8, HALO + S + 8, T), F32),
        pltpu.VMEM((S, DC), BF16),
        [factors] * 4,
        pltpu.VMEM((DM * PITCH_B, T), U32))

    def second(ctx, sums):
        outa[S:S + 16, 0:T] = jnp.zeros((16, T), BF16)
        load_wo = [pltpu.make_async_copy(wob_h.at[:, :, pl.ds(j * T, T)], qall.at[2 * j:2 * j + 2], sems.at[4 + j])
                   for j in range(8)]

        def pair(i, carry):
            @pl.when(i == 8)
            def _():
                for cp in load_wo:
                    cp.start()
            _pair_body(cfg, i, cops, stk, stv, wops, qall, ctx)
            return carry
        if not cfg.get("skip_b"):
            if cfg.get("scopes"):
                with jax.named_scope("block_B"):
                    lax.fori_loop(0, HB // 2, pair, 0)
            else:
                lax.fori_loop(0, HB // 2, pair, 0)
        else:
            for cp in load_wo:
                cp.start()
        for cp in load_wo + ([] if cfg.get("skip_a") else copy_a):
            cp.wait()
        if cfg.get("skip_o"):
            cp = pltpu.make_async_copy(ctx.at[0, 0], ctx.at[1, 1], sems.at[0])
            cp.start()
            cp.wait()
        else:
            if cfg.get("scopes"):
                with jax.named_scope("block_O"):
                    _phase_o(cfg, ctx, qall, sums, (stk, stv), outa, out_h, sems)
            else:
                _phase_o(cfg, ctx, qall, sums, (stk, stv), outa, out_h, sems)

    if cfg.get("only_a"):
        for i, src in enumerate((qall.at[0], *[c.at[0, 0] for c in cops], wops.at[0, 0])):
            cp = pltpu.make_async_copy(src, out_h.at[pl.ds(0, src.shape[0]), pl.ds(DM + i * T, T)], sems.at[5])
            cp.start()
            cp.wait()
        if not cfg.get("nodeps"):
            for cp in copy_a:
                cp.wait()
        return
    pl.run_scoped(second, pltpu.VMEM((S // T, HB, T, T), F32), [pltpu.VMEM((336 * T, T), U32), pltpu.VMEM((72 * T, T), U32)])


def _call(cfg, A_x, A_wqkv, A_wo, B_x, B_c_kv, B_w_q, B_w_uk, B_w_uv, B_w_o):
    any_spec = pl.BlockSpec(memory_space=pl.ANY)
    out = pl.pallas_call(
        lambda *refs: _kernel(cfg, *refs),
        out_shape=jax.ShapeDtypeStruct((S, 2 * DM), BF16),
        in_specs=[any_spec] * 9,
        out_specs=any_spec,
        scratch_shapes=[
            [pltpu.VMEM((NPROD, 1, T, T), BF16)] * 4,
            pltpu.VMEM((DC * PITCH_B, T), U32),
            pltpu.VMEM((DC * PITCH_B, T), U32),
            pltpu.VMEM((NPROD, 2, T, T), BF16),
            pltpu.VMEM((HB, S, T), BF16),
            pltpu.VMEM((S + 16, DM), BF16),
            pltpu.SemaphoreType.DMA((24,)),
        ],
        compiler_params=pltpu.CompilerParams(vmem_limit_bytes=126 * 1024 * 1024),
        name="concat_heads",
    )(A_x.reshape(S, DM), A_wqkv, A_wo, B_x.reshape(S, DM), B_c_kv.reshape(S, DC),
      B_w_q.reshape(16, S, T), B_w_uk.reshape(8, S, T), B_w_uv.reshape(8, S, T),
      B_w_o.reshape(2, S, DM))
    return out.reshape(1, S, 2 * DM)


@jax.jit
def pallas_concat_heads__sliding_local_dilated__compressed_kv_cla__prompt_kernel(
    A_x: jax.Array,
    A_wqkv: jax.Array,
    A_wo: jax.Array,
    B_x: jax.Array,
    B_c_kv: jax.Array,
    B_w_q: jax.Array,
    B_w_uk: jax.Array,
    B_w_uv: jax.Array,
    B_w_o: jax.Array,
):
    return _call(CFG, A_x, A_wqkv, A_wo, B_x, B_c_kv, B_w_q, B_w_uk, B_w_uv, B_w_o)
```

```python
import functools

import numpy as np

import jax
import jax.numpy as jnp
from jax import lax
import jax.experimental.pallas as pl
import jax.experimental.pallas.tpu as pltpu

F32, BF16, U32 = jnp.float32, jnp.bfloat16, jnp.uint32
LOG2E = float(np.log2(np.e))
NEG = -1e9 * LOG2E
T = 128
N = 4
NPROD = 49
ROWS = N * T

S = 2048
DM = 1024
DC = 512
HB = 32
WIN, DIL, HA, DH_A = 8, 2, 32, 32
HALO = 16
G = 16
PITCH_B = 17
PITCH_A = 33

CFG = dict(s_heads=8, s_cost=10, t_cost=30, p_cost=28, m_cost=8, spill=2, a_order="x", b_order="x", lag=8, p_j=8, mix_j=2, mix_p=2, pv=4, group=8, o_flush=(315, 329, 336, 339, 341, 342), o_piece=128, o_lag=2, o_cap=250, o_span=49, o_start=1, o_end=1, o_order="y",  b_lag=6, b_rate=(40, 32), b_wait=6, b_late=4, b_small=(16, 0), b_each=1, b_deep=4, b_span=8, b_qtie=0, b_wtie=1, b_cost=32, b_proj=(0, 0), b_prep=(9, 1),
           steps="""
    |y>b s1,0,2 |z>k F0,0 |a>c s1,2,4 r40 F0,1 F1,0 |b>d s1,4,6 F1,1 |k r92 s1,6,8 w1,0 F2,0 F2,1 |c>e r88 x1 F3,0 F3,1 r58 w1,1 K1,0 |d>f r42 x2 K1,1 x3 K2,0 K2,1
    |e r52 s0 w0,0 x0 K3,0 K3,1 w0,1 Q1,0 >ghij r47 s2 w2,0 w2,1 Q2,0 Q0,0 Q0,1 p0 Q1,1 Q3,0 Q2,1 Q3,1
    |fg r495 p1,0,32 tq p1,32,64 W0 b0 b1 V0,0 V0,1 V1,0 V1,1 b2 b3 V2,0 V2,1 V3,0 V3,1 W1 m0 P0,0 P0,1 P0,2 P0,3 W2 p2,0,16 s3 o0 w3,1 P1,0 P1,1 P1,2 P1,3 W3 P2,0 P2,1 P2,2 P2,3
    |hij r48 W4 tv m1 w3,0 p2,16,64 P3,0 P3,1 P3,2 P3,3 W5 p3 P4,0 P4,1 P4,2 P4,3 O0,0 O0,1 tk W6 o1 m2 P5,0 P5,1 P5,2 P5,3 W7 o2 m3 P6,0 P6,1 P6,2 P6,3 O1,0 O1,1 >01 r38 o3 U c0 c1 c2 P7,0 P7,1 P7,2 P7,3 O2,0 O2,1 c3 O3,0 O3,1 >23""")


def _mm(a, b):
    return jnp.dot(a, b, preferred_element_type=F32)


def _mm_nt(a, b):
    return lax.dot_general(a, b, (((1,), (1,)), ((), ())), preferred_element_type=F32)


def _cat(xs, axis):
    xs = list(xs)
    return xs[0] if len(xs) == 1 else lax.concatenate(xs, axis)


def _rows(x, start, size):
    return lax.slice_in_dim(x, start, start + size, axis=0)


def _fold(op, xs):
    xs = list(xs)
    acc = xs[0]
    for x in xs[1:]:
        acc = op(acc, x)
    return acc


def _bf(words):
    return pltpu.bitcast(words, BF16)


def _words(x):
    return pltpu.bitcast(x, U32)


def _reciprocal(x):
    r = pltpu.reciprocal(x, approx=True)
    return r * (2.0 - x * r)


def _quads(g, n):
    h = n // 2
    return [{(r, c): g[(r + i * h, c + j * h)] for r in range(h) for c in range(h)}
            for i in range(2) for j in range(2)]


def _gadd(x, y):
    return {k: lax.add(x[k], y[k]) for k in x}


def _gsub(x, y):
    return {k: lax.sub(x[k], y[k]) for k in x}


ORDERS = {
    "x": (((2, 1, 3), (0, 1, 1), (3,), (1, -1, 3), (0, 1, 3), (0,), (2, -1, 0)),
          ((0,), (3,), (2, -1, 0), (2, 1, 3), (0, 1, 3), (1, -1, 3), (0, 1, 1))),
    "y": (((0,), (3,), (2, 1, 3), (2, -1, 0), (0, 1, 3), (0, 1, 1), (1, -1, 3)),
          ((1, -1, 3), (2, -1, 0), (0,), (0, 1, 1), (0, 1, 3), (3,), (2, 1, 3)))}
LEFT, RIGHT = ORDERS["x"]


def _factor(rule, quad):
    if len(rule) == 1:
        return quad(rule[0])
    return (_gadd if rule[1] > 0 else _gsub)(quad(rule[0]), quad(rule[2]))


def _factors(rules, g, n=N):
    if n == 1:
        return [g[(0, 0)]]
    quads = _quads(g, n)
    return [x for rule in rules for x in _factors(rules, _factor(rule, quads.__getitem__), n // 2)]


def _combine(product, emit, n=N, base=0, order="x"):
    if n == 1:
        return emit(0, 0, product(base))
    h = n // 2
    a, b, s = {}, {}, {}

    def use(i, r, c, m):
        k = r, c
        if i == 0:
            a[k] = m
        elif i == 1:
            b[k] = m
        elif i == 2:
            emit(r + h, c, lax.add(a[k], m))
            s[k] = lax.sub(m, b[k])
        elif i == 3:
            s[k] = lax.add(s[k], m)
        elif i == 4:
            emit(r, c, lax.add(s[k], m))
            s[k] = lax.sub(m, a[k])
        elif i == 5:
            emit(r, c + h, lax.add(b[k], m))
            s[k] = lax.add(s[k], m)
        else:
            emit(r + h, c + h, lax.add(s[k], m))

    def use_y(i, r, c, m):
        k = r, c
        if i == 0:
            a[k] = m
        elif i == 1:
            b[k] = m
        elif i == 2:
            emit(r + h, c, lax.add(b[k], m))
            s[k] = lax.sub(a[k], m)
        elif i == 3:
            s[k] = lax.add(s[k], m)
        elif i == 4:
            emit(r + h, c + h, lax.add(s[k], m))
            s[k] = lax.add(b[k], m)
        elif i == 5:
            emit(r, c + h, lax.add(a[k], m))
            s[k] = lax.sub(s[k], m)
        else:
            emit(r, c, lax.add(s[k], m))

    for i in range(7):
        _combine(product, lambda r, c, m, i=i: (use if order == "x" else use_y)(i, r, c, m), h,
                 base + i * 7 ** (h.bit_length() - 1), order)


class _SideWork:
    def __init__(self, lag, never=None):
        self.lag, self.never = lag, never
        self.urgent, self.todo, self.running, self.results = [], [], [], []
        self.clock, self.credit, self.rate, self.cache = 0, 0.0, 0.0, (None,)

    def after(self, x, groups=1):
        old = [r for r in self.results if r[0] <= self.clock - self.lag]
        if not old:
            return x
        key = (self.clock, x.shape, x.dtype == F32)
        if self.cache[0] != key:
            deps = [_rows(value, row, 8) for _, value, row in
                    (old[max(0, len(old) - 1 - 2 * n)] for n in reversed(range(groups)))]
            deps = [_cat([dep if x.dtype == F32 else _words(dep)] * (x.shape[1] // T), 1) for dep in deps]
            self.cache = (key, _cat([dep for dep in deps for _ in range(x.shape[0] // 8 // groups)], 0), self.never(x.shape))
        return lax.select(self.cache[2], self.cache[1], x)

    def before(self, words, most):
        due = [x for t, x in self.running[:most] if t <= self.clock]
        if not due:
            return words
        del self.running[:len(due)]
        parts = [_rows(words, r, 8) for r in range(0, T // 2, 8)]
        for i, x in enumerate(due):
            dep = _fold(lax.bitwise_or, [_words(_rows(x, r, 8)) for r in range(0, x.shape[0], 8)])
            parts[i * 8 // len(due)] = lax.select(self.never((8, T)), dep, parts[i * 8 // len(due)])
        return _cat(parts, 0)

    def add(self, cost, run, wait=0, urgent=False):
        (self.urgent if urgent else self.todo).append((self.clock + wait, cost, run))

    def issued(self, tiles, result):
        for i in range(2 * tiles):
            self.clock += 0.5
            self.results = self.results[-40:] + [(self.clock, result, i * (result.shape[0] // G) // (2 * tiles) * G)]
            self.credit += 0.5 * self.rate
            while self.credit > 0:
                ready = [x for x in (self.urgent, self.todo) if x and x[0][0] <= self.clock]
                if not ready:
                    break
                _, cost, run = ready[0].pop(0)
                self.credit -= cost
                run()
            self.credit = min(self.credit, 0.0)

    def finish(self, done=lambda: False):
        while (self.urgent or self.todo) and not done():
            (self.urgent or self.todo).pop(0)[2]()


def _queue_factors(side, rules, load, dst):
    def piece(outer):
        def run():
            h = N // 2
            quad = lambda x: {(r, c): load(x // 2 * h + r, x % 2 * h + c) for r in range(h) for c in range(h)}
            for i, x in enumerate(_factors(rules, _factor(rules[outer], quad), h)):
                ref, idx = dst(outer * 7 + i)
                ref[idx] = lax.convert_element_type(x, BF16)
        return run
    for outer in range(7):
        side.add(50, piece(outer))


def _queue_activation(side, src, dst, chunk, order):
    kt = src.shape[1] // (N * T)
    for t in range(kt):
        for r0 in range(0, T, G):
            def load(r, c, t=t, r0=r0):
                lo, col = chunk * ROWS + r * T + r0, (c * kt + t) * T
                return lax.convert_element_type(_bf(side.after(_words(src[lo:lo + G, col:col + T]))), F32)
            _queue_factors(side, ORDERS[order][0], load, lambda i, t=t, r0=r0: (dst[chunk], (i, t, pl.ds(r0, G))))


def _queue_head_weights(side, columns, kt, scale, wops, order):
    high, shift = jnp.full((G, T), 0xFFFF0000, U32), jnp.full((G, T), 16, U32)
    for t in range(kt):
        for r0 in range(0, T, G):
            def load(r, c, t=t, r0=r0):
                ref, word, half = columns[c]
                w = side.after(ref[pl.ds(word + ((kt * r + t) * T + r0) * PITCH_B, G, stride=PITCH_B), :])
                w = pltpu.bitcast(lax.bitwise_and(w, high) if half else lax.shift_left(w, shift), F32)
                return w if scale is None else w * scale
            _queue_factors(side, ORDERS[order][1], load, lambda i, t=t, r0=r0: (wops, (i, t, pl.ds(r0, G))))


def _queue_kv_weights(side, pair, stk, stv, wops, order):
    _queue_head_weights(side, [(stk, pair, 0), (stk, pair, 1), (stv, pair, 0), (stv, pair, 1)], 1, None, wops, order)


def _tile(ref, *idx):
    *lead, row = idx
    return ref.bitcast(U32)[(*lead, pl.ds(row * (T // 2), T // 2))]


def _phase_a(cfg, barrier, x, wqkv, woa, staged, wops, oops, kbuf, vbuf, ckv, xops, cops, stb, qall, outa):
    side = _SideWork(cfg["lag"])
    q = {}
    done = set()

    def check(step, user):
        assert step is None or step in done or cfg.get("nodeps"), (user, "must come after", step)

    def stage(sec, i, heads):
        def run():
            lo, hi = heads[0] * DH_A, (heads[-1] + 1) * DH_A
            if sec < 3:
                w = _bf(side.after(_words(wqkv[i * T:(i + 1) * T, sec * DM + lo:sec * DM + hi]))).T
            else:
                w = _bf(side.after(_words(woa[lo:hi, i * T:(i + 1) * T])))
            w = w.astype(F32)
            for h in heads:
                staged[i, h * PITCH_A:h * PITCH_A + DH_A, :] = _rows(w, h * DH_A - lo, DH_A)
        return run

    def weights(sec, g, t, r0):
        def permuted(slab, j):
            w = side.after(staged[slab, pl.ds(r0 % HA * PITCH_A + 4 * j + r0 // HA, G, stride=PITCH_A), :])
            return w * (float(DH_A ** -0.5) * LOG2E) if sec == 0 else w

        load = (lambda r, c: permuted(2 * r + t, g * N + c)) if sec < 3 else (
            lambda r, c: permuted(g * N + c, 2 * r + t))
        _queue_factors(side, ORDERS[cfg["a_order"]][1], load, lambda i: (wops[sec == 0][g], (i, t, pl.ds(r0, G))))

    def project(sec, c, g):
        left, right = xops[c] if sec < 3 else oops[c % 2], wops[sec == 0][g]

        def product(i):
            a, w = (_cat([_tile(left, i, t, 0) for t in range(2)], 1), [_tile(right, i, t, 0) for t in range(2)])
            out = _mm_nt(_bf(a), _bf(_cat(w, 1))) if sec < 3 else _mm(_bf(a), _bf(_cat(w, 0)))
            side.issued(2, out)
            return out

        def emit(r, col, val):
            r0, j = c * ROWS + r * T, g * N + col
            if sec == 0:
                q[(r0, j)] = val
            elif sec == 3:
                outa[r0:r0 + T, j * T:(j + 1) * T] = val.astype(BF16)
            else:
                (kbuf if sec == 1 else vbuf)[j, HALO + r0:HALO + r0 + T, :] = val

        _combine(product, emit, order=cfg["a_order"])

    def first_keys(r, half):
        for j in range(N * half, N * half + N):
            w = _cat([_cat([staged[slab, pl.ds(4 * j + d, HA, stride=PITCH_A), :] for d in range(4)], 0)
                      for slab in (2 * r, 2 * r + 1)], 1)
            out = _mm_nt(x[0:ROWS, 2 * r * T:(2 * r + 2) * T], w.astype(BF16))
            side.issued(2 * N, _rows(out, ROWS - T, T))
            kbuf[j, HALO:HALO + ROWS, :] = out + kbuf[j, HALO:HALO + ROWS, :] if r else out

    def project_queries(quad, c):
        left, right = xops[c], wops[quad != cfg['spill']][quad % 2]

        def product(i):
            out = _mm(_bf(_cat([_tile(left, i, t, 0) for t in range(2)], 1)),
                      _bf(_cat([_tile(right, i, t, 0) for t in range(2)], 0)))
            side.issued(2, out)
            return out

        def emit(r, h, val):
            qall[4 * quad + h, c * ROWS + r * T:c * ROWS + (r + 1) * T, :] = val.astype(BF16)

        _combine(product, emit, order=cfg["a_order"])

    E = cfg["group"]
    row = lax.broadcasted_iota(jnp.int32, (E, T), 0)

    lane = lax.broadcasted_iota(jnp.int32, (E, T), 1)

    def group_sums(a, b, c, d):
        even, low = (lane & HA) == 0, lane < 2 * HA
        fold = lambda pick, x, y, shift: lax.select(pick, x, y) + pltpu.roll(lax.select(pick, y, x), shift, 1)
        z = fold(low, fold(even, a, b, 3 * HA), fold(even, c, d, 3 * HA), 2 * HA)
        zr = pltpu.roll(z, 2 * HA, 1)
        out = []
        for x in (lax.select(low, z, zr), lax.select(low, zr, z)):
            xr = pltpu.roll(x, HA, 1)
            out += [lax.select(even, x, xr), lax.select(even, xr, x)]
        return out

    def probs(r0):
        def run():
            qs = side.after(_cat([_rows(q[(r0 - r0 % T, j)], r0 % T, E) for j in range(8)], 0)).reshape(8, E, T)
            J = cfg["p_j"]
            qs = [_rows(qs, j, J) for j in range(0, 8, J)]
            parts = []
            for w in range(WIN):
                lo = HALO + r0 - DIL * w
                s = jnp.sum(_fold(lax.add, [lax.mul(qs[j // J], kbuf[j:j + J, lo:lo + E, :]) for j in range(0, 8, J)]), axis=0)
                parts.append(s)
            logits = []
            if cfg.get("rs"):
                for w in range(0, WIN, 4):
                    logits += group_sums(*parts[w:w + 4])
            else:
                for s in parts:
                    s = s + pltpu.roll(s, 2 * HA, 1)
                    logits.append(s + pltpu.roll(s, HA, 1))
            logits = [jnp.where(row + r0 >= DIL * w, s, NEG) if r0 < DIL * w else s for w, s in enumerate(logits)]
            m = _fold(jnp.maximum, logits)
            e = [jnp.exp2(s - m) for s in logits]
            inv = _reciprocal(_fold(jnp.add, e))
            for w in range(WIN):
                kbuf[w, r0:r0 + E, :] = e[w] * inv
        return run

    def mix(r0, js):
        def run():
            J = cfg["mix_j"]
            p = side.after(kbuf[:, r0:r0 + E, :].reshape(WIN * E, T))
            p = [lax.broadcast(_rows(p, w * E, E), (J,)) for w in range(WIN)]
            for j in js:
                vbuf[j:j + J, r0:r0 + E, :] = _fold(lax.add, [
                    lax.mul(p[w], vbuf[j:j + J, HALO + r0 - DIL * w:HALO + r0 - DIL * w + E, :]) for w in range(WIN)])
        return run

    def queue_output(c):
        for t in range(2):
            for r0 in range(0, T, G):
                def load(r, col, t=t, r0=r0):
                    lo = c * ROWS + r * T + r0
                    return side.after(vbuf[2 * col + t, lo:lo + G, :])
                _queue_factors(side, ORDERS[cfg["a_order"]][0], load, lambda i, t=t, r0=r0: (oops[c % 2], (i, t, pl.ds(r0, G))))

    def stage_heads(base, st, m0, count):
        def run():
            lo = m0 * HB // 2
            w = side.after(qall.bitcast(U32)[base + lo // (S // 2), pl.ds(lo % (S // 2), count * HB // 2), :])
            for i in range(count):
                st[(m0 + i) * PITCH_B:(m0 + i) * PITCH_B + HB // 2, :] = _rows(w, i * HB // 2, HB // 2)
        return run

    def needs(kind, num):
        if kind == "F":
            return [("s", 1, 2 * num[0] + 1)]
        if kind == "P":
            return [("W", num[0]), ("b", num[1]), ("t", "qqqqvvkk"[num[0]])]
        return [("w", "QKVO".index(kind), num[1]), ("o" if kind == "O" else "x", num[0])] if kind in "QKVO" else []

    scope = []
    steps = [(s[0], s[1:], [int(a) for a in s[1:].split(",")] if s[1:2].isdigit() and s[0] not in "|>" else [])
             for s in cfg["steps"].split()]
    for n, (kind, arg, num) in enumerate(steps):
        side.finish(lambda: all(key in done for key in needs(kind, num)))
        for key in needs(kind, num):
            check(key, (kind, num))
        if kind == "|":
            side.finish()
            side.credit = 0.0
            if cfg.get("scopes"):
                if scope:
                    scope.pop().__exit__(None, None, None)
                with jax.named_scope(f"wait_{side.clock:06.0f}_{arg}"):
                    barrier(*arg.split(">"))
                scope.append(jax.named_scope(f"block_{side.clock:06.0f}_{arg}"))
                scope[-1].__enter__()
            else:
                barrier(*arg.split(">"))
            zeros = vbuf[0, HALO + S:HALO + S + 8, :]
            side.results = []
            side.never = lambda shape, z=zeros: _cat([_cat([z] * (shape[1] // T), 1)] * (shape[0] // 8), 0) != 0
        elif kind == ">":
            if "g" in arg:
                side.finish(lambda: all(("x", c) in done for c in range(S // ROWS)))
            barrier("", arg)
        elif kind == "r":
            side.rate = num[0] / (10 if num[0] > 200 else 1)
        elif kind in "QKVO":
            project("QKVO".index(kind), *num)
            done.add((kind, *num))
        elif kind == "s":
            for i in range(*num[1:]) if num[1:] else range(8):
                for h in range(0, HA, cfg["s_heads"]):
                    side.add(cfg["s_cost"] * cfg["s_heads"], stage(num[0], i, range(h, h + cfg["s_heads"])))
                side.add(0, lambda key=("s", num[0], i): done.add(key))
        elif kind == "F":
            first_keys(*num)
        elif kind == "P":
            project_queries(*num)
            done.add((kind, *num))
        elif kind in "wxobW":
            key = (kind, *num)
            frees = {"w": {1: None, 0: None, 2: ("K", 3, num[-1]),
                           3: ("P", cfg["spill"], 3) if cfg["spill"] % 2 == num[-1] else ("V", 3, num[-1])}.get(num[0]) if kind == "w" else None,
                     "x": None, "b": ("V", num[0], 1), "o": ("O", num[0] - 2, 1) if num[0] >= 2 else None,
                     "W": ("V", 3, num[0] % 2) if num[0] == cfg["spill"] else ("P", num[0] - 4, 3) if num[0] - 2 == cfg["spill"]
                     else ("P", num[0] - 2, 3) if num[0] >= 2 else ("Q", 3, num[0])}[kind]
            side.add(0, lambda frees=frees, key=key: check(frees, key))
            if kind == "w":
                for t in range(2):
                    for r0 in range(0, T, G):
                        weights(*num, t, r0)
            elif kind in "xb":
                _queue_activation(side, x, xops, *num, cfg["a_order"])
            elif kind == "W":
                side.add(0, lambda key=key: check(("t", "q"), key))
                _queue_head_weights(side, [(stb[0], 2 * num[0] + h // 2, h % 2) for h in range(4)], 2,
                                    float(T ** -0.5) * LOG2E, wops[num[0] != cfg["spill"]][num[0] % 2], cfg["a_order"])
            else:
                queue_output(*num)
            side.add(0, lambda key=(kind, *num): done.add(key))
        elif kind in "pm":
            check(("Q" if kind == "p" else "V", num[0], 1), (kind, num))
            for r0 in range(num[0] * ROWS, (num[0] + 1) * ROWS, E)[slice(*num[1:] or [None])]:
                if kind == "p":
                    side.add(cfg["p_cost"] * E, probs(r0))
                else:
                    for j in range(0, 8, cfg["mix_p"]):
                        side.add(2 * E * cfg["mix_p"] + cfg["m_cost"], mix(r0, range(j, j + cfg["mix_p"], cfg["mix_j"])))
        elif kind == "c":
            _queue_activation(side, ckv, cops, *num, cfg["b_order"])
        elif kind == "t":
            st = stb["qkv".index(arg)]
            for m0 in range(0, st.shape[0] // PITCH_B, 4):
                side.add(cfg["t_cost"], stage_heads({"q": 0, "v": 16, "k": 24}[arg], st, m0, 4))
            side.add(0, lambda key=("t", arg): done.add(key))
        elif kind == "U":
            side.add(0, lambda: [check(key, "U") for key in (("t", "v"), ("t", "k"), ("P", 6, 3))])
            _queue_kv_weights(side, 0, stb[1], stb[2], wops[1][0], cfg["b_order"])
    side.finish()
    if scope:
        scope.pop().__exit__(None, None, None)


def _pair_body(cfg, pair, cops, stk, stv, wops, qall, ctx):
    side = _SideWork(cfg["b_lag"], lambda shape: lax.broadcast(pair < 0, shape))
    side.rate = cfg["b_rate"][0]
    k, v = {}, {}

    def product(j, i):
        out = _mm(_bf(side.before(_tile(cops[j], i, 0, 0), 1)), _bf(side.before(_tile(wops, i, 0, 0), cfg["b_wtie"])))
        side.issued(1, out)
        return out

    def project(j):
        def emit(r, c, val):
            (k if c < 2 else v)[(c % 2, N * j + r)] = val

        _combine(functools.partial(product, j), emit, order=cfg["b_order"])

    causal = lax.broadcasted_iota(jnp.int32, (T, T), 1) <= lax.broadcasted_iota(jnp.int32, (T, T), 0)

    def scores(h, i):
        s = _mm_nt(_bf(side.before(_tile(qall, 2 * pair + h, i), cfg["b_qtie"])), _cat([k[(h, t)] for t in range(i + 1)], 0).astype(BF16))
        s = [s[:, t * T:(t + 1) * T] for t in range(i + 1)]
        for t in range(0, i + 1, 4):
            side.issued(min(4, i + 1 - t), s[t])
        s[i] = jnp.where(causal, s[i], NEG)
        return s, jnp.max(_fold(jnp.maximum, s), axis=1, keepdims=True)

    def attend(h, i, s, m):
        e = [jnp.exp2(x - m) for x in s]
        acc = None
        for t in range(0, i + 1, cfg["pv"]):
            ts = range(t, min(t + cfg["pv"], i + 1))
            part = _mm(_cat([e[u] for u in ts], 1).astype(BF16), _cat([v[(h, u)] for u in ts], 0).astype(BF16))
            acc = part if acc is None else acc + part
            side.issued(len(ts), acc)

        def normalize(r0):
            def run():
                part = side.after(_fold(lax.add, [_rows(x, r0, G) for x in e]))
                out = _rows(acc, r0, G) * _reciprocal(jnp.sum(part, axis=1, keepdims=True))
                ctx[i, 2 * pair + h, r0:r0 + G, :] = out
                side.running.append((side.clock + cfg["b_span"], out))
            return run
        for r0 in range(0, T, G):
            side.add(cfg["b_cost"] + 2 * i, normalize(r0), cfg["b_wait"], urgent=True)

    late = cfg["b_late"]
    project(0)
    project(1)
    live, last, small = [], [], [(h, i) for i in reversed(range(late)) for h in range(2)]
    for i in range(late, S // T):
        for h in range(2):
            live.append((h, i, *scores(h, i)))
            if (i % N, h) == tuple(cfg["b_proj"]) and 0 < i // N < S // ROWS - 1:
                project(i // N + 1)
            if (i, h) == tuple(cfg["b_prep"]):
                side.rate = cfg["b_rate"][1]
                _queue_kv_weights(side, jnp.minimum(pair + 1, HB // 2 - 1), stk, stv, wops, cfg["b_order"])
            if small and (i, h) >= tuple(cfg["b_small"]):
                for _ in range(cfg["b_each"]):
                    u = small.pop(0)
                    last.append((*u, *scores(*u)))
            while len(live) > (2 if i < cfg["b_deep"] else 1):
                attend(*live.pop(0))
    for unit in live + last + [(*u, *scores(*u)) for u in small]:
        attend(*unit)
    side.results = []
    side.finish()


def _phase_o(cfg, ctx, wob, sums, spare, stage, out_h, sems):
    n = 2 * N
    kt, mt = HB // n, S // T // n
    rules = ORDERS[cfg["o_order"]]
    P = cfg["o_piece"]
    zeros = stage.bitcast(U32)[S // 2:S // 2 + 8, 0:T]
    side = _SideWork(cfg["o_lag"], lambda shape: _cat([zeros] * (shape[0] // 8), 0) != 0)

    def context(r, c):
        return [lambda lo, size, m=m, t=t: ctx[r * mt + m, c * kt + t, lo:lo + size, :]
                for m in range(mt) for t in range(kt)]

    def weight(r, c):
        return [lambda lo, size, t=t: _bf(wob.bitcast(U32)[
            2 * c + r // N, pl.ds(((r % N * kt + t) * T + lo) // 2, size // 2), :]).astype(F32) for t in range(kt)]

    def lazy(rule, g, n):
        quads = _quads(g, n)
        if len(rule) == 1:
            return quads[rule[0]]
        op = lax.add if rule[1] > 0 else lax.sub
        return {k: [functools.cache(lambda lo, size, x=x, y=y: op(x(lo, size), y(lo, size)))
                    for x, y in zip(quads[rule[0]][k], quads[rule[2]][k])] for k in quads[0]}

    def stored(rules, rule, g, slots, jobs):
        quads = _quads(g, n)
        first = _quads(quads[rule[0]], n // 2)
        out = [first[inner[0]] if len(rule + inner) == 2 else {k: [] for k in first[0]} for inner in rules]
        for k in first[0]:
            for t in range(len(first[0][k])):
                where = {j: next(slots) for j, inner in enumerate(rules) if len(rule + inner) > 2}
                for j, slot in where.items():
                    out[j][k].append(lambda lo, size, slot=slot: pltpu.bitcast(slot[0][(*slot[1:-1], pl.ds(slot[-1] + lo, size))], F32))
                for lo in range(0, T, P):
                    def run(k=k, t=t, lo=lo, where=where):
                        def load(q):
                            tie = (lambda x: side.after(x, P // G)) if q == rule[0] else lambda x: x
                            return {i: tie(x[k][t](lo, P)) for i, x in enumerate(_quads(quads[q], n // 2))}
                        top = _factor(rule, load)
                        for j, slot in where.items():
                            slot[0][(*slot[1:-1], pl.ds(slot[-1] + lo, P))] = _words(_factor(rules[j], lambda q: {0: top[q]})[0])
                    jobs.append((len(where) * P // 8, run))
        return out

    a = {(r, c): context(r, c) for r in range(n) for c in range(n)}
    b = {(r, c): weight(r, c) for r in range(n) for c in range(n)}
    jobs = [[] for _ in range(8)]
    operands = []
    for i in range(7):
        slots = [(sums, lo) for lo in range(0, sums.shape[0] - T, T)]
        if i % 2:
            slots = [(ref, lo) for ref in spare[:2] for lo in range(0, ref.shape[0] - T + 1, T)]
            slots += [(spare[3].bitcast(U32), h, lo) for h in range(HB) for lo in range(0, S // 2, T)]
        slots = iter(slots)
        mid = [stored(rules[s], rules[s][i], g, slots, jobs[i]) if i else
               [lazy(rule, top, n // 2) for top in [lazy(rules[s][i], g, n)] for rule in rules[s]] for s, g in enumerate((a, b))]
        operands += [[lazy(rules[s][k], mid[s][j], n // 4)[0, 0] for s in range(2)] for j in range(7) for k in range(7)]

    def room(i):
        left, level = cfg["o_cap"], i
        for _ in range(3):
            left -= mt * 16 * (level % 7 != 6)
            if level % 7 not in (2, 4, 5, 6):
                break
            level //= 7
        for s, size in enumerate((mt * kt * 16, kt * 16)) if i < NPROD else ():
            seen = {q for k in range(i % 7) for q in rules[s][k][::2]}
            left -= size * len(set(rules[s][i % 7][::2]) - seen) * (len(rules[s][i // 7 % 7]) > 1)
        return max(left, 0)

    ready, started = [], []

    def send(r, c, size):
        rows, cols = pl.ds(r * mt * T, size * mt * T), pl.ds(c * T, size * T)
        started.append(pltpu.make_async_copy(stage.at[rows, cols], out_h.at[rows, pl.ds(DM + c * T, size * T)], sems.at[0]))
        started[-1].start()

    def flush():
        if len(ready) == N * N:
            send(*min(ready), N)
        else:
            for r, c in ready:
                send(r, c, 1)
        ready.clear()

    def emit(r, c, val):
        stage[r * mt * T:(r + 1) * mt * T, c * T:(c + 1) * T] = val.astype(BF16)
        ready.append((r, c))

    def product(i):
        if i % NPROD == 0:
            while started:
                started.pop().wait()
            side.results = []
            started.append(pltpu.make_async_copy(wob.bitcast(U32).at[0, 0:8], sums.at[sums.shape[0] - 8:], sems.at[0]))
            started[-1].start()
        if i % NPROD == 0 or i in cfg["o_flush"]:
            flush()
        x, y = ([tile(0, T) for tile in g] for g in operands[i])
        out = _mm(_cat([_cat(x[m * kt:(m + 1) * kt], 1) for m in range(mt)], 0).astype(BF16), _cat(y, 0).astype(BF16))
        queue = jobs[i // NPROD + 1]
        left = sum(room(k) for k in range(i, i - i % NPROD + cfg["o_span"]))
        share = sum(cost for cost, _ in queue) * (1 if left <= room(i) else room(i) / left)
        side.rate, side.credit = share / (mt * kt), 0.0
        while share > 0 and queue:
            share -= queue[0][0]
            side.add(*queue.pop(0))
        side.issued(mt * kt, out)
        side.finish()
        return out

    _combine(product, emit, n, 0, cfg["o_order"])
    flush()
    for cp in started:
        cp.wait()


def _kernel(cfg, xa_h, wqkv_h, woa_h, xb_h, ckv_h, wq_h, wuk_h, wuv_h, wob_h, out_h,
            cops, stk, stv, wops, qall, outa, sems):
    copy_a = [pltpu.make_async_copy(outa.at[pl.ds(c * ROWS, ROWS)], out_h.at[pl.ds(c * ROWS, ROWS), pl.ds(0, DM)],
                                    sems.at[c]) for c in range(S // ROWS)]

    def first(x, wqkv, woa, staged, wops2, oops, kbuf, vbuf, ckv, xops, stq):
        def x_rows(lo, hi):
            return xa_h.at[pl.ds(lo, hi - lo)], x.at[pl.ds(lo, hi - lo)]

        def w_cols(sec):
            return wqkv_h.at[:, pl.ds(sec * DM, DM)], wqkv.at[:, pl.ds(sec * DM, DM)]

        def quarter(r):
            k = pl.ds(r * DM // N, DM // N)
            return [(wqkv_h.at[k, pl.ds(DM, DM)], wqkv.at[k, pl.ds(DM, DM)]),
                    (xa_h.at[pl.ds(0, ROWS), k], x.at[pl.ds(0, ROWS), k])]

        groups = {
            "y": quarter(0)[:1], "z": quarter(0)[1:], "a": quarter(1), "b": quarter(2), "k": quarter(3),
            "c": [x_rows(ROWS, 2 * ROWS)],
            "d": [x_rows(2 * ROWS, S)],
            "e": [w_cols(0), w_cols(2), (woa_h, woa)],
            "f": [(wq_h, qall.at[0:16])],
            "g": [(xb_h, x)],
            "h": [(wuv_h, qall.at[16:24])],
            "i": [(wuk_h, qall.at[24:32])],
            "j": [(ckv_h, ckv)],
        }
        slot = iter(range(4, 24))
        copies = {k: [pltpu.make_async_copy(src, dst, sems.at[next(slot)]) for src, dst in v]
                  for k, v in groups.items()}
        copies.update({str(c): [cp] for c, cp in enumerate(copy_a)})

        def barrier(wait, start=""):
            for name in wait:
                for cp in copies[name]:
                    cp.wait()
            for name in start:
                for cp in copies[name]:
                    cp.start()

        barrier("", "yza")
        kbuf[:, 0:HALO, :] = jnp.zeros((8, HALO, T), F32)
        vbuf[:, 0:HALO, :] = jnp.zeros((8, HALO, T), F32)
        vbuf[0, HALO + S:HALO + S + 8, :] = jnp.zeros((8, T), F32)
        _phase_a(cfg, barrier, x, wqkv, woa, staged, (wops2[:2], [wops, wops2[2]]), oops, kbuf, vbuf, ckv,
                 xops, cops, (stq, stk, stv), qall, outa)

    factors = pltpu.VMEM((NPROD, 2, T, T), BF16)
    (pl.run_scoped if not cfg.get("skip_a") else (lambda *a: None))(
        first,
        pltpu.VMEM((S, DM), BF16), pltpu.VMEM((DM, 3 * DM), BF16), pltpu.VMEM((DM, DM), BF16),
        pltpu.VMEM((8, HA * PITCH_A, T), F32), [factors] * 3, [factors] * 2,
        pltpu.VMEM((8, HALO + S, T), F32), pltpu.VMEM((8, HALO + S + 8, T), F32),
        pltpu.VMEM((S, DC), BF16),
        [factors] * 4,
        pltpu.VMEM((DM * PITCH_B, T), U32))

    def second(ctx, wob, sums):
        outa[S:S + 16, 0:T] = jnp.zeros((16, T), BF16)
        load_wo = [pltpu.make_async_copy(wob_h.at[:, :, pl.ds(j * T, T)], wob.at[2 * j:2 * j + 2], sems.at[4 + j])
                   for j in range(8)]

        def pair(i, carry):
            _pair_body(cfg, i, cops, stk, stv, wops, qall, ctx)
            return carry
        for cp in load_wo:
            cp.start()
        if not cfg.get("skip_b"):
            if cfg.get("scopes"):
                with jax.named_scope("block_B"):
                    lax.fori_loop(0, HB // 2, pair, 0)
            else:
                lax.fori_loop(0, HB // 2, pair, 0)
        for cp in load_wo + ([] if cfg.get("skip_a") else copy_a):
            cp.wait()
        if cfg.get("skip_o"):
            cp = pltpu.make_async_copy(ctx.at[0, 0], ctx.at[1, 1], sems.at[0])
            cp.start()
            cp.wait()
        else:
            if cfg.get("scopes"):
                with jax.named_scope("block_O"):
                    _phase_o(cfg, ctx, wob, sums, (stk, stv, wops, qall), outa, out_h, sems)
            else:
                _phase_o(cfg, ctx, wob, sums, (stk, stv, wops, qall), outa, out_h, sems)

    if cfg.get("only_a"):
        for i, src in enumerate((qall.at[0], *[c.at[0, 0] for c in cops], wops.at[0, 0])):
            cp = pltpu.make_async_copy(src, out_h.at[pl.ds(0, src.shape[0]), pl.ds(DM + i * T, T)], sems.at[5])
            cp.start()
            cp.wait()
        if ">23" in cfg["steps"]:
            for cp in copy_a:
                cp.wait()
        return
    pl.run_scoped(second, pltpu.VMEM((S // T, HB, T, T), F32), pltpu.VMEM((16, S, T), BF16), pltpu.VMEM((336 * T + 8, T), U32))


def _call(cfg, A_x, A_wqkv, A_wo, B_x, B_c_kv, B_w_q, B_w_uk, B_w_uv, B_w_o):
    any_spec = pl.BlockSpec(memory_space=pl.ANY)
    out = pl.pallas_call(
        lambda *refs: _kernel(cfg, *refs),
        out_shape=jax.ShapeDtypeStruct((S, 2 * DM), BF16),
        in_specs=[any_spec] * 9,
        out_specs=any_spec,
        scratch_shapes=[
            [pltpu.VMEM((NPROD, 1, T, T), BF16)] * 4,
            pltpu.VMEM((DC * PITCH_B, T), U32),
            pltpu.VMEM((DC * PITCH_B, T), U32),
            pltpu.VMEM((NPROD, 2, T, T), BF16),
            pltpu.VMEM((HB, S, T), BF16),
            pltpu.VMEM((S + 16, DM), BF16),
            pltpu.SemaphoreType.DMA((24,)),
        ],
        compiler_params=pltpu.CompilerParams(vmem_limit_bytes=126 * 1024 * 1024),
        name="concat_heads",
    )(A_x.reshape(S, DM), A_wqkv, A_wo, B_x.reshape(S, DM), B_c_kv.reshape(S, DC),
      B_w_q.reshape(16, S, T), B_w_uk.reshape(8, S, T), B_w_uv.reshape(8, S, T),
      B_w_o.reshape(2, S, DM))
    return out.reshape(1, S, 2 * DM)


@jax.jit
def pallas_concat_heads__sliding_local_dilated__compressed_kv_cla__prompt_kernel(
    A_x: jax.Array,
    A_wqkv: jax.Array,
    A_wo: jax.Array,
    B_x: jax.Array,
    B_c_kv: jax.Array,
    B_w_q: jax.Array,
    B_w_uk: jax.Array,
    B_w_uv: jax.Array,
    B_w_o: jax.Array,
):
    return _call(CFG, A_x, A_wqkv, A_wo, B_x, B_c_kv, B_w_q, B_w_uk, B_w_uv, B_w_o)
```

```python
import functools

import numpy as np

import jax
import jax.numpy as jnp
from jax import lax
import jax.experimental.pallas as pl
import jax.experimental.pallas.tpu as pltpu

F32, BF16, U32 = jnp.float32, jnp.bfloat16, jnp.uint32
LOG2E = float(np.log2(np.e))
NEG = -1e9 * LOG2E
T = 128
N = 4
NPROD = 49
ROWS = N * T

S = 2048
DM = 1024
DC = 512
HB = 32
WIN, DIL, HA, DH_A = 8, 2, 32, 32
HALO = 16
G = 16
PITCH_B = 17
MT, KT = S // T // (2 * N), HB // (2 * N)
PITCH_A = 33

CFG = dict(r_cost=2.5, s_heads=8, s_cost=10, t_cost=30, p_cost=28, m_cost=8, spill=2, a_order="x", b_order="x", lag=8, p_j=8, mix_j=2, mix_p=2, pv=4, group=8, o_flush=(315, 329, 336, 339, 341, 342), o_lag=1, o_cap=235, o_span=49,  b_lag=4, b_rate=(40, 40), b_wait=8, b_late=4, b_small=(16, 0), b_each=1, b_deep=4, b_span=6, b_qtie=0, b_wtie=1, b_cost=40, b_proj=(0, 1), b_prep=(9, 0),
           steps="""
    l2 |y>b s1,0,2 |z>k F0,0 |a>c s1,2,4 r40 F0,1 F1,0 |b>d s1,4,6 F1,1 |k r88 s1,6,8 w1,0 F2,0 F2,1 |c>e r96 x1 F3,0 F3,1 r54 w1,1 K1,0 |d>f r64 x2 K1,1 r30 x3 K2,0 K2,1
    |e r50 s0 w0,0 x0 K3,0 K3,1 w0,1 Q1,0 >ghij r48 s2 w2,0 w2,1 Q2,0 Q0,0 Q0,1 p0 Q1,1 Q3,0 Q2,1 Q3,1
    |fg l8 r485 p1,0,32 tq p1,32,64 W0 b0 b1 V0,0 V0,1 V1,0 V1,1 b2 b3 V2,0 V2,1 V3,0 V3,1 W1 m0 P0,0 P0,1 P0,2 P0,3 W2 p2,0,16 s3 w3,1 o0 P1,0 P1,1 P1,2 P1,3 W3 P2,0 P2,1 P2,2 P2,3
    |hij r48 W4 tv m1 w3,0 p2,16,64 P3,0 P3,1 P3,2 P3,3 W5 p3,0,48 P4,0 P4,1 P4,2 P4,3 O0,0 O0,1 W6 p3,48,64 tk o1 m2 P5,0 P5,1 P5,2 P5,3 W7 o2 m3 P6,0 P6,1 P6,2 P6,3 O1,0 O1,1 >01 r41 o3 U c0 c1 R c2 P7,0 P7,1 P7,2 P7,3 O2,0 O2,1 c3 O3,0 O3,1 >23""")


def _mm(a, b):
    return jnp.dot(a, b, preferred_element_type=F32)


def _mm_nt(a, b):
    return lax.dot_general(a, b, (((1,), (1,)), ((), ())), preferred_element_type=F32)


def _cat(xs, axis):
    xs = list(xs)
    return xs[0] if len(xs) == 1 else lax.concatenate(xs, axis)


def _rows(x, start, size):
    return lax.slice_in_dim(x, start, start + size, axis=0)


def _fold(op, xs):
    xs = list(xs)
    acc = xs[0]
    for x in xs[1:]:
        acc = op(acc, x)
    return acc


def _bf(words):
    return pltpu.bitcast(words, BF16)


def _words(x):
    return pltpu.bitcast(x, U32)


def _reciprocal(x):
    r = pltpu.reciprocal(x, approx=True)
    return r * (2.0 - x * r)


def _quads(g, n):
    h = n // 2
    return [{(r, c): g[(r + i * h, c + j * h)] for r in range(h) for c in range(h)}
            for i in range(2) for j in range(2)]


def _gadd(x, y):
    return {k: lax.add(x[k], y[k]) for k in x}


def _gsub(x, y):
    return {k: lax.sub(x[k], y[k]) for k in x}


ORDERS = {
    "x": (((2, 1, 3), (0, 1, 1), (3,), (1, -1, 3), (0, 1, 3), (0,), (2, -1, 0)),
          ((0,), (3,), (2, -1, 0), (2, 1, 3), (0, 1, 3), (1, -1, 3), (0, 1, 1))),
    "y": (((0,), (3,), (2, 1, 3), (2, -1, 0), (0, 1, 3), (0, 1, 1), (1, -1, 3)),
          ((1, -1, 3), (2, -1, 0), (0,), (0, 1, 1), (0, 1, 3), (3,), (2, 1, 3)))}
LEFT, RIGHT = ORDERS["x"]


def _factor(rule, quad):
    if len(rule) == 1:
        return quad(rule[0])
    return (_gadd if rule[1] > 0 else _gsub)(quad(rule[0]), quad(rule[2]))


def _factors(rules, g, n=N):
    if n == 1:
        return [g[(0, 0)]]
    quads = _quads(g, n)
    return [x for rule in rules for x in _factors(rules, _factor(rule, quads.__getitem__), n // 2)]


def _combine(product, emit, n=N, base=0, order="x"):
    if n == 1:
        return emit(0, 0, product(base))
    h = n // 2
    a, b, s = {}, {}, {}

    def use(i, r, c, m):
        k = r, c
        if i == 0:
            a[k] = m
        elif i == 1:
            b[k] = m
        elif i == 2:
            emit(r + h, c, lax.add(a[k], m))
            s[k] = lax.sub(m, b[k])
        elif i == 3:
            s[k] = lax.add(s[k], m)
        elif i == 4:
            emit(r, c, lax.add(s[k], m))
            s[k] = lax.sub(m, a[k])
        elif i == 5:
            emit(r, c + h, lax.add(b[k], m))
            s[k] = lax.add(s[k], m)
        else:
            emit(r + h, c + h, lax.add(s[k], m))

    def use_y(i, r, c, m):
        k = r, c
        if i == 0:
            a[k] = m
        elif i == 1:
            b[k] = m
        elif i == 2:
            emit(r + h, c, lax.add(b[k], m))
            s[k] = lax.sub(a[k], m)
        elif i == 3:
            s[k] = lax.add(s[k], m)
        elif i == 4:
            emit(r + h, c + h, lax.add(s[k], m))
            s[k] = lax.add(b[k], m)
        elif i == 5:
            emit(r, c + h, lax.add(a[k], m))
            s[k] = lax.sub(s[k], m)
        else:
            emit(r, c, lax.add(s[k], m))

    for i in range(7):
        _combine(product, lambda r, c, m, i=i: (use if order == "x" else use_y)(i, r, c, m), h,
                 base + i * 7 ** (h.bit_length() - 1), order)


class _SideWork:
    def __init__(self, lag, never=None):
        self.lag, self.never = lag, never
        self.urgent, self.todo, self.running, self.results = [], [], [], []
        self.clock, self.credit, self.rate, self.cache = 0, 0.0, 0.0, (None,)

    def after(self, x, groups=1):
        old = [r for r in self.results if r[0] <= self.clock - self.lag]
        if not old:
            return x
        key = (self.clock, x.shape, x.dtype == F32)
        if self.cache[0] != key:
            deps = [_rows(value, row, 8) for _, value, row in
                    (old[max(0, len(old) - 1 - 2 * n)] for n in reversed(range(groups)))]
            deps = [_cat([dep if x.dtype == F32 else _words(dep)] * (x.shape[1] // T), 1) for dep in deps]
            self.cache = (key, _cat([dep for dep in deps for _ in range(x.shape[0] // 8 // groups)], 0), self.never(x.shape))
        return lax.select(self.cache[2], self.cache[1], x)

    def before(self, words, most):
        due = [x for t, x in self.running[:most] if t <= self.clock]
        if not due:
            return words
        del self.running[:len(due)]
        parts = [_rows(words, r, 8) for r in range(0, T // 2, 8)]
        for i, x in enumerate(due):
            dep = _fold(lax.bitwise_or, [_words(_rows(x, r, 8)) for r in range(0, x.shape[0], 8)])
            parts[i * 8 // len(due)] = lax.select(self.never((8, T)), dep, parts[i * 8 // len(due)])
        return _cat(parts, 0)

    def add(self, cost, run, wait=0, urgent=False):
        (self.urgent if urgent else self.todo).append((self.clock + wait, cost, run))

    def issued(self, tiles, result):
        for i in range(2 * tiles):
            self.clock += 0.5
            self.results = self.results[-40:] + [(self.clock, result, i * (result.shape[0] // G) // (2 * tiles) * G)]
            self.credit += 0.5 * self.rate
            while self.credit > 0:
                ready = [x for x in (self.urgent, self.todo) if x and x[0][0] <= self.clock]
                if not ready:
                    break
                _, cost, run = ready[0].pop(0)
                self.credit -= cost
                run()
            self.credit = min(self.credit, 0.0)

    def finish(self, done=lambda: False):
        while (self.urgent or self.todo) and not done():
            (self.urgent or self.todo).pop(0)[2]()


def _queue_factors(side, rules, load, dst):
    def piece(outer):
        def run():
            h = N // 2
            quad = lambda x: {(r, c): load(x // 2 * h + r, x % 2 * h + c) for r in range(h) for c in range(h)}
            for i, x in enumerate(_factors(rules, _factor(rules[outer], quad), h)):
                ref, idx = dst(outer * 7 + i)
                ref[idx] = lax.convert_element_type(x, BF16)
        return run
    for outer in range(7):
        side.add(50, piece(outer))


def _queue_activation(side, src, dst, chunk, order):
    kt = src.shape[1] // (N * T)
    for t in range(kt):
        for r0 in range(0, T, G):
            def load(r, c, t=t, r0=r0):
                lo, col = chunk * ROWS + r * T + r0, (c * kt + t) * T
                return lax.convert_element_type(_bf(side.after(_words(src[lo:lo + G, col:col + T]))), F32)
            _queue_factors(side, ORDERS[order][0], load, lambda i, t=t, r0=r0: (dst[chunk], (i, t, pl.ds(r0, G))))


def _queue_head_weights(side, columns, kt, scale, wops, order):
    high, shift = jnp.full((G, T), 0xFFFF0000, U32), jnp.full((G, T), 16, U32)
    for t in range(kt):
        for r0 in range(0, T, G):
            def load(r, c, t=t, r0=r0):
                ref, word, half = columns[c]
                w = side.after(ref[pl.ds(word + ((kt * r + t) * T + r0) * PITCH_B, G, stride=PITCH_B), :])
                w = pltpu.bitcast(lax.bitwise_and(w, high) if half else lax.shift_left(w, shift), F32)
                return w if scale is None else w * scale
            _queue_factors(side, ORDERS[order][1], load, lambda i, t=t, r0=r0: (wops, (i, t, pl.ds(r0, G))))


def _queue_kv_weights(side, pair, stk, stv, wops, order):
    _queue_head_weights(side, [(stk, pair, 0), (stk, pair, 1), (stv, pair, 0), (stv, pair, 1)], 1, None, wops, order)


def _tile(ref, *idx):
    *lead, row = idx
    return ref.bitcast(U32)[(*lead, pl.ds(row * (T // 2), T // 2))]


def _phase_a(cfg, barrier, x, wqkv, woa, staged, wops, oops, kbuf, vbuf, ckv, xops, cops, stb, qall, outa, wob, ahead):
    side = _SideWork(cfg["lag"])
    q = {}
    done = set()

    def check(step, user):
        assert step is None or step in done or cfg.get("nodeps"), (user, "must come after", step)

    def stage(sec, i, heads):
        def run():
            lo, hi = heads[0] * DH_A, (heads[-1] + 1) * DH_A
            if sec < 3:
                w = _bf(side.after(_words(wqkv[i * T:(i + 1) * T, sec * DM + lo:sec * DM + hi]))).T
            else:
                w = _bf(side.after(_words(woa[lo:hi, i * T:(i + 1) * T])))
            w = w.astype(F32)
            for h in heads:
                staged[i, h * PITCH_A:h * PITCH_A + DH_A, :] = _rows(w, h * DH_A - lo, DH_A)
        return run

    def weights(sec, g, t, r0):
        def permuted(slab, j):
            w = side.after(staged[slab, pl.ds(r0 % HA * PITCH_A + 4 * j + r0 // HA, G, stride=PITCH_A), :])
            return w * (float(DH_A ** -0.5) * LOG2E) if sec == 0 else w

        load = (lambda r, c: permuted(2 * r + t, g * N + c)) if sec < 3 else (
            lambda r, c: permuted(g * N + c, 2 * r + t))
        _queue_factors(side, ORDERS[cfg["a_order"]][1], load, lambda i: (wops[sec == 0][g], (i, t, pl.ds(r0, G))))

    def project(sec, c, g):
        left, right = xops[c] if sec < 3 else oops[c % 2], wops[sec == 0][g]

        def product(i):
            a, w = (_cat([_tile(left, i, t, 0) for t in range(2)], 1), [_tile(right, i, t, 0) for t in range(2)])
            out = _mm_nt(_bf(a), _bf(_cat(w, 1))) if sec < 3 else _mm(_bf(a), _bf(_cat(w, 0)))
            side.issued(2, out)
            return out

        def emit(r, col, val):
            r0, j = c * ROWS + r * T, g * N + col
            if sec == 0:
                q[(r0, j)] = val
            elif sec == 3:
                outa[r0:r0 + T, j * T:(j + 1) * T] = val.astype(BF16)
            else:
                (kbuf if sec == 1 else vbuf)[j, HALO + r0:HALO + r0 + T, :] = val

        _combine(product, emit, order=cfg["a_order"])

    def first_keys(r, half):
        for j in range(N * half, N * half + N):
            w = _cat([_cat([staged[slab, pl.ds(4 * j + d, HA, stride=PITCH_A), :] for d in range(4)], 0)
                      for slab in (2 * r, 2 * r + 1)], 1)
            out = _mm_nt(x[0:ROWS, 2 * r * T:(2 * r + 2) * T], w.astype(BF16))
            side.issued(2 * N, _rows(out, ROWS - T, T))
            kbuf[j, HALO:HALO + ROWS, :] = out + kbuf[j, HALO:HALO + ROWS, :] if r else out

    def project_queries(quad, c):
        left, right = xops[c], wops[quad != cfg['spill']][quad % 2]

        def product(i):
            out = _mm(_bf(_cat([_tile(left, i, t, 0) for t in range(2)], 1)),
                      _bf(_cat([_tile(right, i, t, 0) for t in range(2)], 0)))
            side.issued(2, out)
            return out

        def emit(r, h, val):
            qall[4 * quad + h, c * ROWS + r * T:c * ROWS + (r + 1) * T, :] = val.astype(BF16)

        _combine(product, emit, order=cfg["a_order"])

    E = cfg["group"]
    row = lax.broadcasted_iota(jnp.int32, (E, T), 0)

    lane = lax.broadcasted_iota(jnp.int32, (E, T), 1)

    def group_sums(a, b, c, d):
        even, low = (lane & HA) == 0, lane < 2 * HA
        fold = lambda pick, x, y, shift: lax.select(pick, x, y) + pltpu.roll(lax.select(pick, y, x), shift, 1)
        z = fold(low, fold(even, a, b, 3 * HA), fold(even, c, d, 3 * HA), 2 * HA)
        zr = pltpu.roll(z, 2 * HA, 1)
        out = []
        for x in (lax.select(low, z, zr), lax.select(low, zr, z)):
            xr = pltpu.roll(x, HA, 1)
            out += [lax.select(even, x, xr), lax.select(even, xr, x)]
        return out

    def probs(r0):
        def run():
            qs = side.after(_cat([_rows(q[(r0 - r0 % T, j)], r0 % T, E) for j in range(8)], 0)).reshape(8, E, T)
            J = cfg["p_j"]
            qs = [_rows(qs, j, J) for j in range(0, 8, J)]
            parts = []
            for w in range(WIN):
                lo = HALO + r0 - DIL * w
                s = jnp.sum(_fold(lax.add, [lax.mul(qs[j // J], kbuf[j:j + J, lo:lo + E, :]) for j in range(0, 8, J)]), axis=0)
                parts.append(s)
            logits = []
            if cfg.get("rs"):
                for w in range(0, WIN, 4):
                    logits += group_sums(*parts[w:w + 4])
            else:
                for s in parts:
                    s = s + pltpu.roll(s, 2 * HA, 1)
                    logits.append(s + pltpu.roll(s, HA, 1))
            logits = [jnp.where(row + r0 >= DIL * w, s, NEG) if r0 < DIL * w else s for w, s in enumerate(logits)]
            m = _fold(jnp.maximum, logits)
            e = [jnp.exp2(s - m) for s in logits]
            inv = _reciprocal(_fold(jnp.add, e))
            for w in range(WIN):
                kbuf[w, r0:r0 + E, :] = e[w] * inv
        return run

    def mix(r0, js):
        def run():
            J = cfg["mix_j"]
            p = side.after(kbuf[:, r0:r0 + E, :].reshape(WIN * E, T))
            p = [lax.broadcast(_rows(p, w * E, E), (J,)) for w in range(WIN)]
            for j in js:
                vbuf[j:j + J, r0:r0 + E, :] = _fold(lax.add, [
                    lax.mul(p[w], vbuf[j:j + J, HALO + r0 - DIL * w:HALO + r0 - DIL * w + E, :]) for w in range(WIN)])
        return run

    def queue_output(c):
        for t in range(2):
            for r0 in range(0, T, G):
                def load(r, col, t=t, r0=r0):
                    lo = c * ROWS + r * T + r0
                    return side.after(vbuf[2 * col + t, lo:lo + G, :])
                _queue_factors(side, ORDERS[cfg["a_order"]][0], load, lambda i, t=t, r0=r0: (oops[c % 2], (i, t, pl.ds(r0, G))))

    def stage_heads(base, st, m0, count):
        def run():
            lo = m0 * HB // 2
            w = side.after(qall.bitcast(U32)[base + lo // (S // 2), pl.ds(lo % (S // 2), count * HB // 2), :])
            for i in range(count):
                st[(m0 + i) * PITCH_B:(m0 + i) * PITCH_B + HB // 2, :] = _rows(w, i * HB // 2, HB // 2)
        return run

    def needs(kind, num):
        if kind == "F":
            return [("s", 1, 2 * num[0] + 1)]
        if kind == "P":
            return [("W", num[0]), ("b", num[1]), ("t", "qqqqvvkk"[num[0]])]
        return [("w", "QKVO".index(kind), num[1]), ("o" if kind == "O" else "x", num[0])] if kind in "QKVO" else []

    scope = []
    steps = [(s[0], s[1:], [int(a) for a in s[1:].split(",")] if s[1:2].isdigit() and s[0] not in "|>" else [])
             for s in cfg["steps"].split()]
    for n, (kind, arg, num) in enumerate(steps):
        side.finish(lambda: all(key in done for key in needs(kind, num)))
        for key in needs(kind, num):
            check(key, (kind, num))
        if kind == "|":
            side.finish()
            side.credit = 0.0
            if cfg.get("scopes"):
                if scope:
                    scope.pop().__exit__(None, None, None)
                with jax.named_scope(f"wait_{side.clock:06.0f}_{arg}"):
                    barrier(*arg.split(">"))
                scope.append(jax.named_scope(f"block_{side.clock:06.0f}_{arg}"))
                scope[-1].__enter__()
            else:
                barrier(*arg.split(">"))
            zeros = vbuf[0, HALO + S:HALO + S + 8, :]
            side.results = []
            side.never = lambda shape, z=zeros: _cat([_cat([z] * (shape[1] // T), 1)] * (shape[0] // 8), 0) != 0
        elif kind == ">":
            if "g" in arg:
                side.finish(lambda: all(("x", c) in done for c in range(S // ROWS)))
            barrier("", arg)
        elif kind == "l":
            side.lag = num[0]
        elif kind == "r":
            side.rate = num[0] / (10 if num[0] > 200 else 1)
        elif kind in "QKVO":
            project("QKVO".index(kind), *num)
            done.add((kind, *num))
        elif kind == "s":
            for i in range(*num[1:]) if num[1:] else range(8):
                for h in range(0, HA, cfg["s_heads"]):
                    side.add(cfg["s_cost"] * cfg["s_heads"], stage(num[0], i, range(h, h + cfg["s_heads"])))
                side.add(0, lambda key=("s", num[0], i): done.add(key))
        elif kind == "F":
            first_keys(*num)
        elif kind == "P":
            project_queries(*num)
            done.add((kind, *num))
        elif kind in "wxobW":
            key = (kind, *num)
            frees = {"w": {1: None, 0: None, 2: ("K", 3, num[-1]),
                           3: ("P", cfg["spill"], 3) if cfg["spill"] % 2 == num[-1] else ("V", 3, num[-1])}.get(num[0]) if kind == "w" else None,
                     "x": None, "b": ("V", num[0], 1), "o": ("O", num[0] - 2, 1) if num[0] >= 2 else None,
                     "W": ("V", 3, num[0] % 2) if num[0] == cfg["spill"] else ("P", num[0] - 4, 3) if num[0] - 2 == cfg["spill"]
                     else ("P", num[0] - 2, 3) if num[0] >= 2 else ("Q", 3, num[0])}[kind]
            side.add(0, lambda frees=frees, key=key: check(frees, key))
            if kind == "w":
                for t in range(2):
                    for r0 in range(0, T, G):
                        weights(*num, t, r0)
            elif kind in "xb":
                _queue_activation(side, x, xops, *num, cfg["a_order"])
            elif kind == "W":
                side.add(0, lambda key=key: check(("t", "q"), key))
                _queue_head_weights(side, [(stb[0], 2 * num[0] + h // 2, h % 2) for h in range(4)], 2,
                                    float(T ** -0.5) * LOG2E, wops[num[0] != cfg["spill"]][num[0] % 2], cfg["a_order"])
            else:
                queue_output(*num)
            side.add(0, lambda key=(kind, *num): done.add(key))
        elif kind in "pm":
            check(("Q" if kind == "p" else "V", num[0], 1), (kind, num))
            for r0 in range(num[0] * ROWS, (num[0] + 1) * ROWS, E)[slice(*num[1:] or [None])]:
                if kind == "p":
                    side.add(cfg["p_cost"] * E, probs(r0))
                else:
                    for j in range(0, 8, cfg["mix_p"]):
                        side.add(2 * E * cfg["mix_p"] + cfg["m_cost"], mix(r0, range(j, j + cfg["mix_p"], cfg["mix_j"])))
        elif kind == "c":
            _queue_activation(side, ckv, cops, *num, cfg["b_order"])
        elif kind == "t":
            st = stb["qkv".index(arg)]
            for m0 in range(0, st.shape[0] // PITCH_B, 4):
                side.add(cfg["t_cost"], stage_heads({"q": 0, "v": 16, "k": 24}[arg], st, m0, 4))
            side.add(0, lambda key=("t", arg): done.add(key))
        elif kind == "R":
            rules = ORDERS["y"][1]
            for cost, run in _stored_factors(side, rules, rules[0], _weight_blocks(wob), iter(_slots(ahead)))[1]:
                side.add(cfg["r_cost"] * cost, run)
        elif kind == "U":
            side.add(0, lambda: [check(key, "U") for key in (("t", "v"), ("t", "k"), ("P", 6, 3))])
            _queue_kv_weights(side, 0, stb[1], stb[2], wops[1][0], cfg["b_order"])
    side.finish()
    if scope:
        scope.pop().__exit__(None, None, None)


def _pair_body(cfg, pair, cops, stk, stv, wops, qall, ctx):
    side = _SideWork(cfg["b_lag"], lambda shape: lax.broadcast(pair < 0, shape))
    side.rate = cfg["b_rate"][0]
    k, v = {}, {}

    def product(j, i):
        out = _mm(_bf(side.before(_tile(cops[j], i, 0, 0), 1)), _bf(side.before(_tile(wops, i, 0, 0), cfg["b_wtie"])))
        side.issued(1, out)
        return out

    def project(j):
        def emit(r, c, val):
            (k if c < 2 else v)[(c % 2, N * j + r)] = val

        _combine(functools.partial(product, j), emit, order=cfg["b_order"])

    causal = lax.broadcasted_iota(jnp.int32, (T, T), 1) <= lax.broadcasted_iota(jnp.int32, (T, T), 0)

    def scores(h, i):
        s = _mm_nt(_bf(side.before(_tile(qall, 2 * pair + h, i), cfg["b_qtie"])), _cat([k[(h, t)] for t in range(i + 1)], 0).astype(BF16))
        s = [s[:, t * T:(t + 1) * T] for t in range(i + 1)]
        for t in range(0, i + 1, 4):
            side.issued(min(4, i + 1 - t), s[t])
        s[i] = jnp.where(causal, s[i], NEG)
        return s, jnp.max(_fold(jnp.maximum, s), axis=1, keepdims=True)

    def attend(h, i, s, m):
        e = [jnp.exp2(x - m) for x in s]
        acc = None
        for t in range(0, i + 1, cfg["pv"]):
            ts = range(t, min(t + cfg["pv"], i + 1))
            part = _mm(_cat([e[u] for u in ts], 1).astype(BF16), _cat([v[(h, u)] for u in ts], 0).astype(BF16))
            acc = part if acc is None else acc + part
            side.issued(len(ts), acc)

        def normalize(r0):
            def run():
                part = side.after(_fold(lax.add, [_rows(x, r0, G) for x in e]))
                out = _rows(acc, r0, G) * _reciprocal(jnp.sum(part, axis=1, keepdims=True))
                ctx[i, 2 * pair + h, r0:r0 + G, :] = out
                side.running.append((side.clock + cfg["b_span"], out))
            return run
        for r0 in range(0, T, G):
            side.add(cfg["b_cost"] + 2 * i, normalize(r0), cfg["b_wait"], urgent=True)

    late = cfg["b_late"]
    project(0)
    project(1)
    live, last, small = [], [], [(h, i) for i in reversed(range(late)) for h in range(2)]
    for i in range(late, S // T):
        for h in range(2):
            live.append((h, i, *scores(h, i)))
            if (i % N, h) == tuple(cfg["b_proj"]) and 0 < i // N < S // ROWS - 1:
                project(i // N + 1)
            if (i, h) == tuple(cfg["b_prep"]):
                side.rate = cfg["b_rate"][1]
                _queue_kv_weights(side, jnp.minimum(pair + 1, HB // 2 - 1), stk, stv, wops, cfg["b_order"])
            if small and (i, h) >= tuple(cfg["b_small"]):
                for _ in range(cfg["b_each"]):
                    u = small.pop(0)
                    last.append((*u, *scores(*u)))
            while len(live) > (2 if i < cfg["b_deep"] else 1):
                attend(*live.pop(0))
    for unit in live + last + [(*u, *scores(*u)) for u in small]:
        attend(*unit)
    side.results = []
    side.finish()


def _context_blocks(ctx):
    return {(r, c): [lambda i=(r * MT + m, c * KT + t): ctx[i] for m in range(MT) for t in range(KT)]
            for r in range(2 * N) for c in range(2 * N)}


def _weight_blocks(wob):
    return {(r, c): [lambda i=(2 * c + r // N, r % N * KT + t): _bf(_tile(wob, *i)).astype(F32) for t in range(KT)]
            for r in range(2 * N) for c in range(2 * N)}


def _lazy_factor(rule, g, n):
    quads = _quads(g, n)
    if len(rule) == 1:
        return quads[rule[0]]
    op = lax.add if rule[1] > 0 else lax.sub
    return {k: [functools.cache(lambda x=x, y=y: op(x(), y())) for x, y in zip(quads[rule[0]][k], quads[rule[2]][k])]
            for k in quads[0]}


def _stored_factors(side, rules, rule, g, slots):
    quads = _quads(g, 2 * N)
    first = _quads(quads[rule[0]], N)
    sums = [j for j, inner in enumerate(rules) if len(rule + inner) > 2]
    out = [{k: [] for k in first[0]} if j in sums else first[inner[0]] for j, inner in enumerate(rules)]
    jobs = []
    for k in first[0]:
        for t in range(len(first[0][k])):
            where = {j: next(slots) for j in sums}
            for j, (ref, idx) in where.items():
                out[j][k].append(lambda ref=ref, idx=idx: pltpu.bitcast(ref[idx], F32))

            def run(k=k, t=t, where=where):
                top = _factor(rule, lambda q: {i: side.after(x[k][t](), T // G) if q == rule[0] else x[k][t]()
                                               for i, x in enumerate(_quads(quads[q], N))})
                for j, (ref, idx) in where.items():
                    ref[idx] = _words(_factor(rules[j], lambda q: {0: top[q]})[0])
            jobs.append((len(sums) * T // 8, run))
    return out, jobs


def _slots(ref, *lead):
    return [(ref, (*lead, pl.ds(lo, T))) for lo in range(0, ref.shape[-2] - T + 1, T)]


def _phase_o(cfg, ctx, wob, even, odd, stage, out_h, sems):
    n, mt, kt = 2 * N, MT, KT
    rules = ORDERS["y"]
    zeros = stage.bitcast(U32)[S // 2:S // 2 + 8, 0:T]
    side = _SideWork(cfg["o_lag"], lambda shape: _cat([zeros] * (shape[0] // 8), 0) != 0)
    blocks = _context_blocks(ctx), _weight_blocks(wob)
    jobs, operands = [], []
    for i in range(7):
        slots = iter(odd if i % 2 else even)
        right, more = _stored_factors(side, rules[1], rules[1][i], blocks[1], slots)
        if i:
            left, work = _stored_factors(side, rules[0], rules[0][i], blocks[0], slots)
            jobs.append(work + more)
        else:
            left = [_lazy_factor(rule, _lazy_factor(rules[0][i], blocks[0], n), N) for rule in rules[0]]
        operands += [[_lazy_factor(rules[s][k], mid[j], 2)[0, 0] for s, mid in enumerate((left, right))]
                     for j in range(7) for k in range(7)]
    jobs.append([])

    def room(i):
        left, level = cfg["o_cap"], i
        for _ in range(3):
            left -= mt * 16 * (level % 7 != 6)
            if level % 7 not in (2, 4, 5, 6):
                break
            level //= 7
        for s, size in enumerate((mt * kt * 16,)) if i < NPROD else ():
            seen = {q for k in range(i % 7) for q in rules[s][k][::2]}
            left -= size * len(set(rules[s][i % 7][::2]) - seen) * (len(rules[s][i // 7 % 7]) > 1)
        return max(left, 0)

    ready, started = [], []

    def send(r, c, size):
        rows, cols = pl.ds(r * mt * T, size * mt * T), pl.ds(c * T, size * T)
        started.append(pltpu.make_async_copy(stage.at[rows, cols], out_h.at[rows, pl.ds(DM + c * T, size * T)], sems.at[0]))
        started[-1].start()

    def flush():
        if len(ready) == N * N:
            send(*min(ready), N)
        else:
            for r, c in ready:
                send(r, c, 1)
        ready.clear()

    def emit(r, c, val):
        stage[r * mt * T:(r + 1) * mt * T, c * T:(c + 1) * T] = val.astype(BF16)
        ready.append((r, c))

    def product(i):
        if i % NPROD == 0:
            while started:
                started.pop().wait()
            side.results = []
            spare = even[-1][0]
            started.append(pltpu.make_async_copy(wob.bitcast(U32).at[0, 0:8], spare.at[spare.shape[0] - 8:], sems.at[0]))
            started[-1].start()
        if i % NPROD == 0 or i in cfg["o_flush"]:
            flush()
        x, y = ([tile() for tile in g] for g in operands[i])
        out = _mm(_cat([_cat(x[m * kt:(m + 1) * kt], 1) for m in range(mt)], 0).astype(BF16), _cat(y, 0).astype(BF16))
        queue = jobs[i // NPROD]
        left = sum(room(k) for k in range(i, i - i % NPROD + cfg["o_span"]))
        share = sum(cost for cost, _ in queue) * (1 if left <= room(i) else room(i) / left)
        side.rate, side.credit = share / (mt * kt), 0.0
        while share > 0 and queue:
            share -= queue[0][0]
            side.add(*queue.pop(0))
        side.issued(mt * kt, out)
        side.finish()
        return out

    _combine(product, emit, n, 0, "y")
    flush()
    for cp in started:
        cp.wait()


def _kernel(cfg, xa_h, wqkv_h, woa_h, xb_h, ckv_h, wq_h, wuk_h, wuv_h, wob_h, out_h,
            cops, stk, stv, wops, qall, outa, wob, ahead, sems):
    copy_a = [pltpu.make_async_copy(outa.at[pl.ds(c * ROWS, ROWS)], out_h.at[pl.ds(c * ROWS, ROWS), pl.ds(0, DM)],
                                    sems.at[c]) for c in range(S // ROWS)]

    def first(x, wqkv, woa, staged, wops2, oops, kbuf, vbuf, ckv, xops, stq):
        def x_rows(lo, hi):
            return xa_h.at[pl.ds(lo, hi - lo)], x.at[pl.ds(lo, hi - lo)]

        def w_cols(sec):
            return wqkv_h.at[:, pl.ds(sec * DM, DM)], wqkv.at[:, pl.ds(sec * DM, DM)]

        def quarter(r):
            k = pl.ds(r * DM // N, DM // N)
            return [(wqkv_h.at[k, pl.ds(DM, DM)], wqkv.at[k, pl.ds(DM, DM)]),
                    (xa_h.at[pl.ds(0, ROWS), k], x.at[pl.ds(0, ROWS), k])]

        groups = {
            "y": quarter(0)[:1], "z": quarter(0)[1:], "a": quarter(1), "b": quarter(2), "k": quarter(3),
            "c": [x_rows(ROWS, 2 * ROWS)],
            "d": [x_rows(2 * ROWS, S)],
            "e": [w_cols(0), w_cols(2), (woa_h, woa)],
            "f": [(wq_h, qall.at[0:16])],
            "g": [(xb_h, x)],
            "h": [(wuv_h, qall.at[16:24])],
            "i": [(wuk_h, qall.at[24:32])],
            "j": [(ckv_h, ckv)] + [(wob_h.at[:, :, pl.ds(j * T, T)], wob.at[2 * j:2 * j + 2]) for j in range(8)],
        }
        slot = iter(range(4, 32))
        copies = {k: [pltpu.make_async_copy(src, dst, sems.at[next(slot)]) for src, dst in v]
                  for k, v in groups.items()}
        copies.update({str(c): [cp] for c, cp in enumerate(copy_a)})

        def barrier(wait, start=""):
            for name in wait:
                for cp in copies[name]:
                    cp.wait()
            for name in start:
                for cp in copies[name]:
                    cp.start()

        barrier("", "yza")
        kbuf[:, 0:HALO, :] = jnp.zeros((8, HALO, T), F32)
        vbuf[:, 0:HALO, :] = jnp.zeros((8, HALO, T), F32)
        vbuf[0, HALO + S:HALO + S + 8, :] = jnp.zeros((8, T), F32)
        _phase_a(cfg, barrier, x, wqkv, woa, staged, (wops2[:2], [wops, wops2[2]]), oops, kbuf, vbuf, ckv,
                 xops, cops, (stq, stk, stv), qall, outa, wob, ahead)

    factors = pltpu.VMEM((NPROD, 2, T, T), BF16)
    (pl.run_scoped if not cfg.get("skip_a") else (lambda *a: None))(
        first,
        pltpu.VMEM((S, DM), BF16), pltpu.VMEM((DM, 3 * DM), BF16), pltpu.VMEM((DM, DM), BF16),
        pltpu.VMEM((8, HA * PITCH_A, T), F32), [factors] * 3, [factors] * 2,
        pltpu.VMEM((8, HALO + S, T), F32), pltpu.VMEM((8, HALO + S + 8, T), F32),
        pltpu.VMEM((S, DC), BF16),
        [factors] * 4,
        pltpu.VMEM((DM * PITCH_B, T), U32))

    def second(ctx, sums):
        outa[S:S + 16, 0:T] = jnp.zeros((16, T), BF16)

        def pair(i, carry):
            _pair_body(cfg, i, cops, stk, stv, wops, qall, ctx)
            return carry
        if not cfg.get("skip_b"):
            if cfg.get("scopes"):
                with jax.named_scope("block_B"):
                    lax.fori_loop(0, HB // 2, pair, 0)
            else:
                lax.fori_loop(0, HB // 2, pair, 0)
        for cp in [] if cfg.get("skip_a") else copy_a:
            cp.wait()
        even = _slots(ahead) + _slots(sums)
        odd = _slots(stk) + _slots(stv) + [slot for h in range(HB) for slot in _slots(qall.bitcast(U32), h)]
        if cfg.get("skip_o"):
            cp = pltpu.make_async_copy(ctx.at[0, 0], ctx.at[1, 1], sems.at[0])
            cp.start()
            cp.wait()
        else:
            if cfg.get("scopes"):
                with jax.named_scope("block_O"):
                    _phase_o(cfg, ctx, wob, even, odd, outa, out_h, sems)
            else:
                _phase_o(cfg, ctx, wob, even, odd, outa, out_h, sems)

    if cfg.get("only_a"):
        for i, src in enumerate((qall.at[0], *[c.at[0, 0] for c in cops], wops.at[0, 0])):
            cp = pltpu.make_async_copy(src, out_h.at[pl.ds(0, src.shape[0]), pl.ds(DM + i * T, T)], sems.at[5])
            cp.start()
            cp.wait()
        if ">23" in cfg["steps"]:
            for cp in copy_a:
                cp.wait()
        return
    pl.run_scoped(second, pltpu.VMEM((S // T, HB, T, T), F32), pltpu.VMEM((224 * T + 8, T), U32))


def _call(cfg, A_x, A_wqkv, A_wo, B_x, B_c_kv, B_w_q, B_w_uk, B_w_uv, B_w_o):
    any_spec = pl.BlockSpec(memory_space=pl.ANY)
    out = pl.pallas_call(
        lambda *refs: _kernel(cfg, *refs),
        out_shape=jax.ShapeDtypeStruct((S, 2 * DM), BF16),
        in_specs=[any_spec] * 9,
        out_specs=any_spec,
        scratch_shapes=[
            [pltpu.VMEM((NPROD, 1, T, T), BF16)] * 4,
            pltpu.VMEM((DC * PITCH_B, T), U32),
            pltpu.VMEM((DC * PITCH_B, T), U32),
            pltpu.VMEM((NPROD, 2, T, T), BF16),
            pltpu.VMEM((HB, S, T), BF16),
            pltpu.VMEM((S + 16, DM), BF16),
            pltpu.VMEM((16, S, T), BF16),
            pltpu.VMEM((112 * T, T), U32),
            pltpu.SemaphoreType.DMA((32,)),
        ],
        compiler_params=pltpu.CompilerParams(vmem_limit_bytes=126 * 1024 * 1024),
        name="concat_heads",
    )(A_x.reshape(S, DM), A_wqkv, A_wo, B_x.reshape(S, DM), B_c_kv.reshape(S, DC),
      B_w_q.reshape(16, S, T), B_w_uk.reshape(8, S, T), B_w_uv.reshape(8, S, T),
      B_w_o.reshape(2, S, DM))
    return out.reshape(1, S, 2 * DM)


@jax.jit
def pallas_concat_heads__sliding_local_dilated__compressed_kv_cla__prompt_kernel(
    A_x: jax.Array,
    A_wqkv: jax.Array,
    A_wo: jax.Array,
    B_x: jax.Array,
    B_c_kv: jax.Array,
    B_w_q: jax.Array,
    B_w_uk: jax.Array,
    B_w_uv: jax.Array,
    B_w_o: jax.Array,
):
    return _call(CFG, A_x, A_wqkv, A_wo, B_x, B_c_kv, B_w_q, B_w_uk, B_w_uv, B_w_o)
```

```python
import functools

import numpy as np

import jax
import jax.numpy as jnp
from jax import lax
import jax.experimental.pallas as pl
import jax.experimental.pallas.tpu as pltpu

F32, BF16, U32 = jnp.float32, jnp.bfloat16, jnp.uint32
LOG2E = float(np.log2(np.e))
NEG = -1e9 * LOG2E
T = 128
N = 4
NPROD = 49
ROWS = N * T

S = 2048
DM = 1024
DC = 512
HB = 32
WIN, DIL, HA, DH_A = 8, 2, 32, 32
HALO = 16
E = 8
G = 16
PITCH_B = 17
MT, KT = S // T // (2 * N), HB // (2 * N)
PITCH_A = 33

STEPS = """
    l2 |y>b s1,0,2 |z>k F0,0 |a>c s1,2,4 r40 F0,1 F1,0 |b>d s1,4,6 F1,1 |k r88 s1,6,8 w1,0 F2,0 F2,1 |c>e
        r96 x1 F3,0 F3,1 r54 w1,1 K1,0 |d>f r64 x2 K1,1 r30 x3 K2,0 K2,1
    |e r50 s0 w0,0 x0 K3,0 K3,1 w0,1 Q1,0 >ghij r48 s2 w2,0 w2,1 Q2,0 Q0,0 Q0,1 p0 Q1,1 Q3,0 Q2,1 Q3,1
    |fg l8 r485 p1,0,32 tq p1,32,64 W0 b0 b1 V0,0 V0,1 V1,0 V1,1 b2 b3 V2,0 V2,1 V3,0 V3,1 W1 m0 P0,0 P0,1
        P0,2 P0,3 W2 p2,0,16 s3 w3,1 o0 P1,0 P1,1 P1,2 P1,3 W3 P2,0 P2,1 P2,2 P2,3
    |hij r48 W4 tv m1 w3,0 p2,16,64 P3,0 P3,1 P3,2 P3,3 W5 p3,0,48 P4,0 P4,1 P4,2 P4,3 O0,0 O0,1 W6 p3,48,64
        tk o1 m2 P5,0 P5,1 P5,2 P5,3 W7 o2 m3 P6,0 P6,1 P6,2 P6,3 O1,0 O1,1 >01 r41 o3 U c0 c1 R c2 P7,0
        P7,1 P7,2 P7,3 O2,0 O2,1 c3 O3,0 O3,1 >23"""
SPARE_QUAD = 2


def _mm(a, b):
    return jnp.dot(a, b, preferred_element_type=F32)


def _mm_nt(a, b):
    return lax.dot_general(a, b, (((1,), (1,)), ((), ())), preferred_element_type=F32)


def _cat(xs, axis):
    xs = list(xs)
    return xs[0] if len(xs) == 1 else lax.concatenate(xs, axis)


def _rows(x, start, size):
    return lax.slice_in_dim(x, start, start + size, axis=0)


def _fold(op, xs):
    xs = list(xs)
    acc = xs[0]
    for x in xs[1:]:
        acc = op(acc, x)
    return acc


def _bf(words):
    return pltpu.bitcast(words, BF16)


def _words(x):
    return pltpu.bitcast(x, U32)


def _reciprocal(x):
    r = pltpu.reciprocal(x, approx=True)
    return r * (2.0 - x * r)


def _quads(g, n):
    h = n // 2
    return [{(r, c): g[(r + i * h, c + j * h)] for r in range(h) for c in range(h)}
            for i in range(2) for j in range(2)]


def _gadd(x, y):
    return {k: lax.add(x[k], y[k]) for k in x}


def _gsub(x, y):
    return {k: lax.sub(x[k], y[k]) for k in x}


LEFT = ((2, 1, 3), (0, 1, 1), (3,), (1, -1, 3), (0, 1, 3), (0,), (2, -1, 0))
RIGHT = ((0,), (3,), (2, -1, 0), (2, 1, 3), (0, 1, 3), (1, -1, 3), (0, 1, 1))
LEFT_O = ((0,), (3,), (2, 1, 3), (2, -1, 0), (0, 1, 3), (0, 1, 1), (1, -1, 3))
RIGHT_O = ((1, -1, 3), (2, -1, 0), (0,), (0, 1, 1), (0, 1, 3), (3,), (2, 1, 3))


def _factor(rule, quad):
    if len(rule) == 1:
        return quad(rule[0])
    return (_gadd if rule[1] > 0 else _gsub)(quad(rule[0]), quad(rule[2]))


def _factors(rules, g, n=N):
    if n == 1:
        return [g[(0, 0)]]
    quads = _quads(g, n)
    return [x for rule in rules for x in _factors(rules, _factor(rule, quads.__getitem__), n // 2)]


def _combine(product, emit, n=N, base=0, left=LEFT):
    if n == 1:
        return emit(0, 0, product(base))
    h = n // 2
    a, b, s = {}, {}, {}

    def use(i, r, c, m):
        k = r, c
        if i < 2:
            (a, b)[i][k] = m
        elif i == 3:
            s[k] = lax.add(s[k], m)
        elif left is LEFT:
            if i == 2:
                emit(r + h, c, lax.add(a[k], m))
                s[k] = lax.sub(m, b[k])
            elif i == 4:
                emit(r, c, lax.add(s[k], m))
                s[k] = lax.sub(m, a[k])
            elif i == 5:
                emit(r, c + h, lax.add(b[k], m))
                s[k] = lax.add(s[k], m)
            else:
                emit(r + h, c + h, lax.add(s[k], m))
        elif i == 2:
            emit(r + h, c, lax.add(b[k], m))
            s[k] = lax.sub(a[k], m)
        elif i == 4:
            emit(r + h, c + h, lax.add(s[k], m))
            s[k] = lax.add(b[k], m)
        elif i == 5:
            emit(r, c + h, lax.add(a[k], m))
            s[k] = lax.sub(s[k], m)
        else:
            emit(r, c, lax.add(s[k], m))

    for i in range(7):
        _combine(product, functools.partial(use, i), h, base + i * 7 ** (h.bit_length() - 1), left)


class _SideWork:
    def __init__(self, lag, never=None):
        self.lag, self.never = lag, never
        self.urgent, self.todo, self.running, self.results = [], [], [], []
        self.clock, self.credit, self.rate, self.cache = 0, 0.0, 0.0, (None,)

    def after(self, x, groups=1):
        old = [r for r in self.results if r[0] <= self.clock - self.lag]
        if not old:
            return x
        key = (self.clock, x.shape, x.dtype == F32)
        if self.cache[0] != key:
            deps = [_rows(value, row, 8) for _, value, row in
                    (old[max(0, len(old) - 1 - 2 * n)] for n in reversed(range(groups)))]
            deps = [_cat([dep if x.dtype == F32 else _words(dep)] * (x.shape[1] // T), 1) for dep in deps]
            deps = _cat([dep for dep in deps for _ in range(x.shape[0] // 8 // groups)], 0)
            self.cache = (key, deps, self.never(x.shape))
        return lax.select(self.cache[2], self.cache[1], x)

    def before(self, words):
        if not self.running or self.running[0][0] > self.clock:
            return words
        x = self.running.pop(0)[1]
        dep = _fold(lax.bitwise_or, [_words(_rows(x, r, 8)) for r in range(0, x.shape[0], 8)])
        return _cat([lax.select(self.never((8, T)), dep, _rows(words, 0, 8)), _rows(words, 8, words.shape[0] - 8)], 0)

    def add(self, cost, run, wait=0, urgent=False):
        (self.urgent if urgent else self.todo).append((self.clock + wait, cost, run))

    def issued(self, tiles, result):
        for i in range(2 * tiles):
            self.clock += 0.5
            self.results = self.results[-40:] + [(self.clock, result, i * (result.shape[0] // G) // (2 * tiles) * G)]
            self.credit += 0.5 * self.rate
            while self.credit > 0:
                ready = [x for x in (self.urgent, self.todo) if x and x[0][0] <= self.clock]
                if not ready:
                    break
                _, cost, run = ready[0].pop(0)
                self.credit -= cost
                run()
            self.credit = min(self.credit, 0.0)

    def finish(self, done=lambda: False):
        while (self.urgent or self.todo) and not done():
            (self.urgent or self.todo).pop(0)[2]()


def _queue_factors(side, rules, load, dst):
    def piece(outer):
        def run():
            h = N // 2
            quad = lambda x: {(r, c): load(x // 2 * h + r, x % 2 * h + c) for r in range(h) for c in range(h)}
            for i, x in enumerate(_factors(rules, _factor(rules[outer], quad), h)):
                ref, idx = dst(outer * 7 + i)
                ref[idx] = lax.convert_element_type(x, BF16)
        return run
    for outer in range(7):
        side.add(50, piece(outer))


def _queue_activation(side, src, dst, chunk):
    kt = src.shape[1] // (N * T)
    for t in range(kt):
        for r0 in range(0, T, G):
            def load(r, c, t=t, r0=r0):
                lo, col = chunk * ROWS + r * T + r0, (c * kt + t) * T
                return lax.convert_element_type(_bf(side.after(_words(src[lo:lo + G, col:col + T]))), F32)
            _queue_factors(side, LEFT, load, lambda i, t=t, r0=r0: (dst[chunk], (i, t, pl.ds(r0, G))))


def _queue_head_weights(side, columns, kt, scale, wops):
    high, shift = jnp.full((G, T), 0xFFFF0000, U32), jnp.full((G, T), 16, U32)
    for t in range(kt):
        for r0 in range(0, T, G):
            def load(r, c, t=t, r0=r0):
                ref, word, half = columns[c]
                w = side.after(ref[pl.ds(word + ((kt * r + t) * T + r0) * PITCH_B, G, stride=PITCH_B), :])
                w = pltpu.bitcast(lax.bitwise_and(w, high) if half else lax.shift_left(w, shift), F32)
                return w if scale is None else w * scale
            _queue_factors(side, RIGHT, load, lambda i, t=t, r0=r0: (wops, (i, t, pl.ds(r0, G))))


def _queue_kv_weights(side, pair, stk, stv, wops):
    _queue_head_weights(side, [(stk, pair, 0), (stk, pair, 1), (stv, pair, 0), (stv, pair, 1)], 1, None, wops)


def _tile(ref, *idx):
    *lead, row = idx
    return ref.bitcast(U32)[(*lead, pl.ds(row * (T // 2), T // 2))]


def _phase_a(barrier, x, wqkv, woa, staged, wops, oops, kbuf, vbuf, ckv, xops, cops, stb, qall, outa, wob, ahead):
    side = _SideWork(0)
    q = {}
    done = set()

    def check(*keys):
        assert all(key in done for key in keys), keys

    def stage(sec, i, heads):
        def run():
            lo, hi = heads[0] * DH_A, (heads[-1] + 1) * DH_A
            if sec < 3:
                w = _bf(side.after(_words(wqkv[i * T:(i + 1) * T, sec * DM + lo:sec * DM + hi]))).T
            else:
                w = _bf(side.after(_words(woa[lo:hi, i * T:(i + 1) * T])))
            w = w.astype(F32)
            for h in heads:
                staged[i, h * PITCH_A:h * PITCH_A + DH_A, :] = _rows(w, h * DH_A - lo, DH_A)
        return run

    def weights(sec, g, t, r0):
        def permuted(slab, j):
            w = side.after(staged[slab, pl.ds(r0 % HA * PITCH_A + 4 * j + r0 // HA, G, stride=PITCH_A), :])
            return w * (float(DH_A ** -0.5) * LOG2E) if sec == 0 else w

        load = (lambda r, c: permuted(2 * r + t, g * N + c)) if sec < 3 else (
            lambda r, c: permuted(g * N + c, 2 * r + t))
        _queue_factors(side, RIGHT, load, lambda i: (wops[sec == 0][g], (i, t, pl.ds(r0, G))))

    def project(sec, c, g):
        left, right = xops[c] if sec < 3 else oops[c % 2], wops[sec == 0][g]

        def product(i):
            a, w = (_cat([_tile(left, i, t, 0) for t in range(2)], 1), [_tile(right, i, t, 0) for t in range(2)])
            out = _mm_nt(_bf(a), _bf(_cat(w, 1))) if sec < 3 else _mm(_bf(a), _bf(_cat(w, 0)))
            side.issued(2, out)
            return out

        def emit(r, col, val):
            r0, j = c * ROWS + r * T, g * N + col
            if sec == 0:
                q[(r0, j)] = val
            elif sec == 3:
                outa[r0:r0 + T, j * T:(j + 1) * T] = val.astype(BF16)
            else:
                (kbuf if sec == 1 else vbuf)[j, HALO + r0:HALO + r0 + T, :] = val

        _combine(product, emit)

    def first_keys(r, half):
        for j in range(N * half, N * half + N):
            w = _cat([_cat([staged[slab, pl.ds(4 * j + d, HA, stride=PITCH_A), :] for d in range(4)], 0)
                      for slab in (2 * r, 2 * r + 1)], 1)
            out = _mm_nt(x[0:ROWS, 2 * r * T:(2 * r + 2) * T], w.astype(BF16))
            side.issued(2 * N, _rows(out, ROWS - T, T))
            kbuf[j, HALO:HALO + ROWS, :] = out + kbuf[j, HALO:HALO + ROWS, :] if r else out

    def project_queries(quad, c):
        left, right = xops[c], wops[quad != SPARE_QUAD][quad % 2]

        def product(i):
            out = _mm(_bf(_cat([_tile(left, i, t, 0) for t in range(2)], 1)),
                      _bf(_cat([_tile(right, i, t, 0) for t in range(2)], 0)))
            side.issued(2, out)
            return out

        def emit(r, h, val):
            qall[4 * quad + h, c * ROWS + r * T:c * ROWS + (r + 1) * T, :] = val.astype(BF16)

        _combine(product, emit)

    row = lax.broadcasted_iota(jnp.int32, (E, T), 0)

    def probs(r0):
        qs = side.after(_cat([_rows(q[(r0 - r0 % T, j)], r0 % T, E) for j in range(8)], 0)).reshape(8, E, T)
        logits = []
        for w in range(WIN):
            lo = HALO + r0 - DIL * w
            s = jnp.sum(lax.mul(qs, kbuf[:, lo:lo + E, :]), axis=0)
            s = s + pltpu.roll(s, 2 * HA, 1)
            s = s + pltpu.roll(s, HA, 1)
            logits.append(jnp.where(row + r0 >= DIL * w, s, NEG) if r0 < DIL * w else s)
        m = _fold(jnp.maximum, logits)
        e = [jnp.exp2(s - m) for s in logits]
        inv = _reciprocal(_fold(jnp.add, e))
        for w in range(WIN):
            kbuf[w, r0:r0 + E, :] = e[w] * inv

    def mix(r0, j):
        p = side.after(kbuf[:, r0:r0 + E, :].reshape(WIN * E, T))
        vbuf[j:j + 2, r0:r0 + E, :] = _fold(lax.add, [
            lax.mul(lax.broadcast(_rows(p, w * E, E), (2,)),
                    vbuf[j:j + 2, HALO + r0 - DIL * w:HALO + r0 - DIL * w + E, :]) for w in range(WIN)])

    def queue_output(c):
        for t in range(2):
            for r0 in range(0, T, G):
                def load(r, col, t=t, r0=r0):
                    lo = c * ROWS + r * T + r0
                    return side.after(vbuf[2 * col + t, lo:lo + G, :])
                _queue_factors(side, LEFT, load, lambda i, t=t, r0=r0: (oops[c % 2], (i, t, pl.ds(r0, G))))

    def stage_heads(base, st, m0, count):
        def run():
            lo = m0 * HB // 2
            w = side.after(qall.bitcast(U32)[base + lo // (S // 2), pl.ds(lo % (S // 2), count * HB // 2), :])
            for i in range(count):
                st[(m0 + i) * PITCH_B:(m0 + i) * PITCH_B + HB // 2, :] = _rows(w, i * HB // 2, HB // 2)
        return run

    def needs(kind, num):
        if kind == "F":
            return [("s", 1, 2 * num[0] + 1)]
        if kind == "P":
            return [("W", num[0]), ("b", num[1]), ("t", "qqqqvvkk"[num[0]])]
        return [("w", "QKVO".index(kind), num[1]), ("o" if kind == "O" else "x", num[0])] if kind in "QKVO" else []

    def overwrites(kind, num):
        if kind == "w" and num[0] >= 2:
            return [("K", 3, num[1]) if num[0] == 2 else
                    ("P", SPARE_QUAD, 3) if SPARE_QUAD % 2 == num[1] else ("V", 3, num[1])]
        if kind == "W":
            before = num[0] - 2 - 2 * (num[0] - 2 == SPARE_QUAD)
            return [("V", 3, num[0] % 2) if num[0] == SPARE_QUAD else
                    ("P", before, 3) if before >= 0 else ("Q", 3, num[0]), ("t", "q")]
        if kind == "b":
            return [("V", num[0], 1)]
        return [("O", num[0] - 2, 1)] if kind == "o" and num[0] >= 2 else []

    for step in STEPS.split():
        kind, arg = step[0], step[1:]
        num = [int(a) for a in arg.split(",")] if arg[:1].isdigit() else []
        key = (kind, *num)
        side.finish(lambda: all(need in done for need in needs(kind, num)))
        check(*needs(kind, num))
        if kind == "|":
            side.finish()
            barrier(*arg.split(">"))
            zeros = vbuf[0, HALO + S:HALO + S + 8, :]
            side.results, side.credit = [], 0.0
            side.never = lambda shape, z=zeros: _cat([_cat([z] * (shape[1] // T), 1)] * (shape[0] // 8), 0) != 0
        elif kind == ">":
            if "g" in arg:
                side.finish(lambda: all(("x", c) in done for c in range(S // ROWS)))
            barrier("", arg)
        elif kind == "l":
            side.lag = num[0]
        elif kind == "r":
            side.rate = num[0] / (10 if num[0] > 200 else 1)
        elif kind in "QKVO":
            project("QKVO".index(kind), *num)
            done.add(key)
        elif kind == "F":
            first_keys(*num)
        elif kind == "P":
            project_queries(*num)
            done.add(key)
        elif kind == "s":
            for i in range(*num[1:] or [8]):
                for h in range(0, HA, 8):
                    side.add(80, stage(num[0], i, range(h, h + 8)))
                side.add(0, functools.partial(done.add, ("s", num[0], i)))
        elif kind in "wxobW":
            side.add(0, functools.partial(check, *overwrites(kind, num)))
            if kind == "w":
                for t in range(2):
                    for r0 in range(0, T, G):
                        weights(*num, t, r0)
            elif kind in "xb":
                _queue_activation(side, x, xops, *num)
            elif kind == "W":
                _queue_head_weights(side, [(stb[0], 2 * num[0] + h // 2, h % 2) for h in range(4)], 2,
                                    float(T ** -0.5) * LOG2E, wops[num[0] != SPARE_QUAD][num[0] % 2])
            else:
                queue_output(*num)
            side.add(0, functools.partial(done.add, key))
        elif kind in "pm":
            check(("Q" if kind == "p" else "V", num[0], 1))
            for r0 in range(num[0] * ROWS, (num[0] + 1) * ROWS, E)[slice(*num[1:] or [None])]:
                if kind == "p":
                    side.add(28 * E, functools.partial(probs, r0))
                else:
                    for j in range(0, 8, 2):
                        side.add(5 * E, functools.partial(mix, r0, j))
        elif kind == "c":
            _queue_activation(side, ckv, cops, *num)
        elif kind == "t":
            st = stb["qkv".index(arg)]
            for m0 in range(0, st.shape[0] // PITCH_B, 4):
                side.add(30, stage_heads({"q": 0, "v": 16, "k": 24}[arg], st, m0, 4))
            side.add(0, functools.partial(done.add, ("t", arg)))
        elif kind == "R":
            for cost, run in _stored_factors(side, RIGHT_O, RIGHT_O[0], _weight_blocks(wob), iter(_slots(ahead)))[1]:
                side.add(2.5 * cost, run)
        elif kind == "U":
            side.add(0, functools.partial(check, ("t", "v"), ("t", "k"), ("P", 6, 3)))
            _queue_kv_weights(side, 0, stb[1], stb[2], wops[1][0])
    side.finish()


def _pair_body(pair, cops, stk, stv, wops, qall, ctx):
    side = _SideWork(4, lambda shape: lax.broadcast(pair < 0, shape))
    side.rate = 40
    k, v = {}, {}

    def product(j, i):
        out = _mm(_bf(side.before(_tile(cops[j], i, 0, 0))), _bf(side.before(_tile(wops, i, 0, 0))))
        side.issued(1, out)
        return out

    def project(j):
        def emit(r, c, val):
            (k if c < 2 else v)[(c % 2, N * j + r)] = val

        _combine(functools.partial(product, j), emit)

    causal = lax.broadcasted_iota(jnp.int32, (T, T), 1) <= lax.broadcasted_iota(jnp.int32, (T, T), 0)

    def scores(h, i):
        s = _mm_nt(_bf(_tile(qall, 2 * pair + h, i)), _cat([k[(h, t)] for t in range(i + 1)], 0).astype(BF16))
        s = [s[:, t * T:(t + 1) * T] for t in range(i + 1)]
        for t in range(0, i + 1, 4):
            side.issued(min(4, i + 1 - t), s[t])
        s[i] = jnp.where(causal, s[i], NEG)
        return s, jnp.max(_fold(jnp.maximum, s), axis=1, keepdims=True)

    def attend(h, i, s, m):
        e = [jnp.exp2(x - m) for x in s]
        acc = None
        for t in range(0, i + 1, 4):
            ts = range(t, min(t + 4, i + 1))
            part = _mm(_cat([e[u] for u in ts], 1).astype(BF16), _cat([v[(h, u)] for u in ts], 0).astype(BF16))
            acc = part if acc is None else acc + part
            side.issued(len(ts), acc)

        def normalize(r0):
            def run():
                part = side.after(_fold(lax.add, [_rows(x, r0, G) for x in e]))
                out = _rows(acc, r0, G) * _reciprocal(jnp.sum(part, axis=1, keepdims=True))
                ctx[i, 2 * pair + h, r0:r0 + G, :] = out
                side.running.append((side.clock + 6, out))
            return run
        for r0 in range(0, T, G):
            side.add(40 + 2 * i, normalize(r0), wait=8, urgent=True)

    project(0)
    project(1)
    live = []
    for i in range(N, S // T):
        for h in range(2):
            live.append((h, i, *scores(h, i)))
            if (i % N, h) == (0, 1) and i // N + 1 < S // ROWS:
                project(i // N + 1)
            if (i, h) == (9, 0):
                _queue_kv_weights(side, jnp.minimum(pair + 1, HB // 2 - 1), stk, stv, wops)
            while len(live) > 1:
                attend(*live.pop(0))
    for unit in live + [(h, i, *scores(h, i)) for i in reversed(range(N)) for h in range(2)]:
        attend(*unit)
    side.results = []
    side.finish()


def _context_blocks(ctx):
    return {(r, c): [lambda i=(r * MT + m, c * KT + t): ctx[i] for m in range(MT) for t in range(KT)]
            for r in range(2 * N) for c in range(2 * N)}


def _weight_blocks(wob):
    return {(r, c): [lambda i=(2 * c + r // N, r % N * KT + t): _bf(_tile(wob, *i)).astype(F32) for t in range(KT)]
            for r in range(2 * N) for c in range(2 * N)}


def _lazy_factor(rule, g, n):
    quads = _quads(g, n)
    if len(rule) == 1:
        return quads[rule[0]]
    op = lax.add if rule[1] > 0 else lax.sub
    return {k: [functools.cache(lambda x=x, y=y: op(x(), y())) for x, y in zip(quads[rule[0]][k], quads[rule[2]][k])]
            for k in quads[0]}


def _stored_factors(side, rules, rule, g, slots):
    quads = _quads(g, 2 * N)
    first = _quads(quads[rule[0]], N)
    sums = [j for j, inner in enumerate(rules) if len(rule + inner) > 2]
    out = [{k: [] for k in first[0]} if j in sums else first[inner[0]] for j, inner in enumerate(rules)]
    jobs = []
    for k in first[0]:
        for t in range(len(first[0][k])):
            where = {j: next(slots) for j in sums}
            for j, (ref, idx) in where.items():
                out[j][k].append(lambda ref=ref, idx=idx: pltpu.bitcast(ref[idx], F32))

            def run(k=k, t=t, where=where):
                top = _factor(rule, lambda q: {i: side.after(x[k][t](), T // G) if q == rule[0] else x[k][t]()
                                               for i, x in enumerate(_quads(quads[q], N))})
                for j, (ref, idx) in where.items():
                    ref[idx] = pltpu.bitcast(_factor(rules[j], lambda q: {0: top[q]})[0], ref.dtype)
            jobs.append((len(sums) * T // 8, run))
    return out, jobs


def _slots(ref, *lead):
    return [(ref, (*lead, pl.ds(lo, T))) for lo in range(0, ref.shape[-2] - T + 1, T)]


def _phase_o(ctx, wob, even, odd, stage, out_h, sems):
    zeros = stage.bitcast(U32)[S // 2:S // 2 + 8, 0:T]
    side = _SideWork(1, lambda shape: _cat([zeros] * (shape[0] // 8), 0) != 0)
    blocks = _context_blocks(ctx), _weight_blocks(wob)
    jobs, operands = [], []
    for i in range(7):
        slots = iter(odd if i % 2 else even)
        right, more = _stored_factors(side, RIGHT_O, RIGHT_O[i], blocks[1], slots)
        if i:
            left, work = _stored_factors(side, LEFT_O, LEFT_O[i], blocks[0], slots)
            jobs.append(work + more)
        else:
            left = [_lazy_factor(rule, _lazy_factor(LEFT_O[i], blocks[0], 2 * N), N) for rule in LEFT_O]
        operands += [(_lazy_factor(LEFT_O[k], left[j], 2)[0, 0], _lazy_factor(RIGHT_O[k], right[j], 2)[0, 0])
                     for j in range(7) for k in range(7)]
    jobs.append([])

    def room(i):
        left, level = 235, i
        for _ in range(3):
            left -= MT * 16 * (level % 7 != 6)
            if level % 7 not in (2, 4, 5, 6):
                break
            level //= 7
        if i < NPROD and len(LEFT_O[i // 7]) > 1:
            seen = {q for k in range(i % 7) for q in LEFT_O[k][::2]}
            left -= MT * KT * 16 * len(set(LEFT_O[i % 7][::2]) - seen)
        return max(left, 0)

    ready, started = [], []

    def send(r, c, size):
        rows, cols = pl.ds(r * MT * T, size * MT * T), pl.ds(c * T, size * T)
        started.append(pltpu.make_async_copy(stage.at[rows, cols], out_h.at[rows, pl.ds(DM + c * T, size * T)],
                                             sems.at[0]))
        started[-1].start()

    def flush():
        if len(ready) == N * N:
            send(*min(ready), N)
        else:
            for r, c in ready:
                send(r, c, 1)
        ready.clear()

    def emit(r, c, val):
        stage[r * MT * T:(r + 1) * MT * T, c * T:(c + 1) * T] = val.astype(BF16)
        ready.append((r, c))

    def product(i):
        if i % NPROD == 0:
            while started:
                started.pop().wait()
            side.results = []
            spare = even[-1][0]
            started.append(pltpu.make_async_copy(ctx.at[0, 0, 0:8], spare.at[spare.shape[0] - 8:], sems.at[0]))
            started[-1].start()
        if i % NPROD == 0 or i in (315, 329, 336, 339, 341, 342):
            flush()
        x, y = ([tile() for tile in g] for g in operands[i])
        out = _mm(_cat([_cat(x[m * KT:(m + 1) * KT], 1) for m in range(MT)], 0).astype(BF16), _cat(y, 0).astype(BF16))
        queue = jobs[i // NPROD]
        left = sum(room(k) for k in range(i, i - i % NPROD + NPROD))
        share = sum(cost for cost, _ in queue) * (1 if left <= room(i) else room(i) / left)
        side.rate, side.credit = share / (MT * KT), 0.0
        while share > 0 and queue:
            share -= queue[0][0]
            side.add(*queue.pop(0))
        side.issued(MT * KT, out)
        side.finish()
        return out

    _combine(product, emit, 2 * N, 0, LEFT_O)
    flush()
    for cp in started:
        cp.wait()


def _kernel(xa_h, wqkv_h, woa_h, xb_h, ckv_h, wq_h, wuk_h, wuv_h, wob_h, out_h,
            cops, stk, stv, wops, qall, outa, wob, ahead, sems):
    copy_a = [pltpu.make_async_copy(outa.at[pl.ds(c * ROWS, ROWS)], out_h.at[pl.ds(c * ROWS, ROWS), pl.ds(0, DM)],
                                    sems.at[c]) for c in range(S // ROWS)]

    def first(x, wqkv, woa, staged, wops2, oops, kbuf, vbuf, ckv, xops, stq):
        def x_rows(lo, hi):
            return xa_h.at[pl.ds(lo, hi - lo)], x.at[pl.ds(lo, hi - lo)]

        def w_cols(sec):
            return wqkv_h.at[:, pl.ds(sec * DM, DM)], wqkv.at[:, pl.ds(sec * DM, DM)]

        def quarter(r):
            k = pl.ds(r * DM // N, DM // N)
            return [(wqkv_h.at[k, pl.ds(DM, DM)], wqkv.at[k, pl.ds(DM, DM)]),
                    (xa_h.at[pl.ds(0, ROWS), k], x.at[pl.ds(0, ROWS), k])]

        groups = {
            "y": quarter(0)[:1], "z": quarter(0)[1:], "a": quarter(1), "b": quarter(2), "k": quarter(3),
            "c": [x_rows(ROWS, 2 * ROWS)],
            "d": [x_rows(2 * ROWS, S)],
            "e": [w_cols(0), w_cols(2), (woa_h, woa)],
            "f": [(wq_h, qall.at[0:16])],
            "g": [(xb_h, x)],
            "h": [(wuv_h, qall.at[16:24])],
            "i": [(wuk_h, qall.at[24:32])],
            "j": [(ckv_h, ckv)] + [(wob_h.at[:, :, pl.ds(j * T, T)], wob.at[2 * j:2 * j + 2]) for j in range(8)],
        }
        slot = iter(range(4, 32))
        copies = {k: [pltpu.make_async_copy(src, dst, sems.at[next(slot)]) for src, dst in v]
                  for k, v in groups.items()}
        copies.update({str(c): [cp] for c, cp in enumerate(copy_a)})

        def barrier(wait, start=""):
            for name in wait:
                for cp in copies[name]:
                    cp.wait()
            for name in start:
                for cp in copies[name]:
                    cp.start()

        barrier("", "yza")
        kbuf[:, 0:HALO, :] = jnp.zeros((8, HALO, T), F32)
        vbuf[:, 0:HALO, :] = jnp.zeros((8, HALO, T), F32)
        vbuf[0, HALO + S:HALO + S + 8, :] = jnp.zeros((8, T), F32)
        _phase_a(barrier, x, wqkv, woa, staged, (wops2[:2], [wops, wops2[2]]), oops, kbuf, vbuf, ckv,
                 xops, cops, (stq, stk, stv), qall, outa, wob, ahead)

    factors = pltpu.VMEM((NPROD, 2, T, T), BF16)
    pl.run_scoped(
        first,
        pltpu.VMEM((S, DM), BF16), pltpu.VMEM((DM, 3 * DM), BF16), pltpu.VMEM((DM, DM), BF16),
        pltpu.VMEM((8, HA * PITCH_A, T), F32), [factors] * 3, [factors] * 2,
        pltpu.VMEM((8, HALO + S, T), F32), pltpu.VMEM((8, HALO + S + 8, T), F32),
        pltpu.VMEM((S, DC), BF16),
        [factors] * 4,
        pltpu.VMEM((DM * PITCH_B, T), U32))

    def second(ctx, sums):
        outa[S:S + 16, 0:T] = jnp.zeros((16, T), BF16)

        pl.loop(0, HB // 2)(lambda i: _pair_body(i, cops, stk, stv, wops, qall, ctx))
        for cp in copy_a:
            cp.wait()
        even = _slots(ahead) + _slots(sums)
        odd = _slots(stk) + _slots(stv) + [slot for h in range(HB) for slot in _slots(qall.bitcast(U32), h)]
        _phase_o(ctx, wob, even, odd, outa, out_h, sems)

    pl.run_scoped(second, pltpu.VMEM((S // T, HB, T, T), F32), pltpu.VMEM((7 * 4 * MT * KT * T + 8, T), F32))


def _call(A_x, A_wqkv, A_wo, B_x, B_c_kv, B_w_q, B_w_uk, B_w_uv, B_w_o):
    any_spec = pl.BlockSpec(memory_space=pl.ANY)
    out = pl.pallas_call(
        _kernel,
        out_shape=jax.ShapeDtypeStruct((S, 2 * DM), BF16),
        in_specs=[any_spec] * 9,
        out_specs=any_spec,
        scratch_shapes=[
            [pltpu.VMEM((NPROD, 1, T, T), BF16)] * 4,
            pltpu.VMEM((DC * PITCH_B, T), U32),
            pltpu.VMEM((DC * PITCH_B, T), U32),
            pltpu.VMEM((NPROD, 2, T, T), BF16),
            pltpu.VMEM((HB, S, T), BF16),
            pltpu.VMEM((S + 16, DM), BF16),
            pltpu.VMEM((16, S, T), BF16),
            pltpu.VMEM((7 * 4 * KT * T, T), U32),
            pltpu.SemaphoreType.DMA((32,)),
        ],
        compiler_params=pltpu.CompilerParams(vmem_limit_bytes=126 * 1024 * 1024),
        name="concat_heads",
    )(A_x.reshape(S, DM), A_wqkv, A_wo, B_x.reshape(S, DM), B_c_kv.reshape(S, DC),
      B_w_q.reshape(16, S, T), B_w_uk.reshape(8, S, T), B_w_uv.reshape(8, S, T),
      B_w_o.reshape(2, S, DM))
    return out.reshape(1, S, 2 * DM)


@jax.jit
def pallas_concat_heads__sliding_local_dilated__compressed_kv_cla__prompt_kernel(
    A_x: jax.Array,
    A_wqkv: jax.Array,
    A_wo: jax.Array,
    B_x: jax.Array,
    B_c_kv: jax.Array,
    B_w_q: jax.Array,
    B_w_uk: jax.Array,
    B_w_uv: jax.Array,
    B_w_o: jax.Array,
):
    return _call(A_x, A_wqkv, A_wo, B_x, B_c_kv, B_w_q, B_w_uk, B_w_uv, B_w_o)
```

```python
import functools

import numpy as np

import jax
import jax.numpy as jnp
from jax import lax
import jax.experimental.pallas as pl
import jax.experimental.pallas.tpu as pltpu

F32, BF16, U32 = jnp.float32, jnp.bfloat16, jnp.uint32
LOG2E = float(np.log2(np.e))
NEG = -1e9 * LOG2E
T = 128
N = 4
NPROD = 49
ROWS = N * T

S = 2048
DM = 1024
DC = 512
HB = 32
WIN, DIL, HA, DH_A = 8, 2, 32, 32
HALO = 16
E = 8
G = 16
PITCH_B = 17
PITCH_A = 33
MT, KT = S // T // (2 * N), HB // (2 * N)

STEPS = """
    l2 |y>b s1,0,2 |z>k F0,0 |a>c s1,2,4 r405 F0,1 F1,0 |b>d s1,4,6 F1,1 |k r88 s1,6,8 w1,0 F2,0 F2,1 |c>e
        r98 x1 F3,0 F3,1 r54 w1,1 K1,0 |d>f r64 x2 K1,1 r30 x3 K2,0 K2,1
    |e l2 r50 s0 w0,0 x0 K3,0 K3,1 w0,1 Q1,0 >ghij r475 s2 w2,0 w2,1 Q2,0 Q0,0 Q0,1 p0 Q3,0 Q1,1 Q2,1 Q3,1
    |fg l8 r485 p1,0,32 tq p1,32,64 W0 b0 b1 V0,0 V0,1 V1,0 V1,1 b2 b3 V2,0 V2,1 V3,0 V3,1 W1 m0 P0,0 P0,1
        P0,2 P0,3 W2 p2,0,16 s3 w3,1 o0 P1,0 P1,1 P1,2 P1,3 W3 P2,0 P2,1 P2,2 P2,3
    |hij l8 r48 W4 tv m1 w3,0 p2,16,64 P3,0 P3,1 P3,2 P3,3 W5 p3,0,48 P4,0 P4,1 P4,2 P4,3 O0,0 O0,1 W6
        p3,48,64 tk o1 m2 P5,0 P5,1 P5,2 P5,3 W7 o2 m3 P6,0 P6,1 P6,2 P6,3 O1,0 O1,1 >01 r41 o3 U c0 c1 R c2
        P7,0 P7,1 P7,2 P7,3 O2,0 O2,1 c3 O3,0 O3,1 >23"""
SPARE_QUAD = 2


def _mm(a, b):
    return jnp.dot(a, b, preferred_element_type=F32)


def _mm_nt(a, b):
    return lax.dot_general(a, b, (((1,), (1,)), ((), ())), preferred_element_type=F32)


def _cat(xs, axis):
    xs = list(xs)
    return xs[0] if len(xs) == 1 else lax.concatenate(xs, axis)


def _rows(x, start, size):
    return lax.slice_in_dim(x, start, start + size, axis=0)


def _fold(op, xs):
    xs = list(xs)
    acc = xs[0]
    for x in xs[1:]:
        acc = op(acc, x)
    return acc


def _bf(words):
    return pltpu.bitcast(words, BF16)


def _words(x):
    return pltpu.bitcast(x, U32)


def _reciprocal(x):
    r = pltpu.reciprocal(x, approx=True)
    return r * (2.0 - x * r)


def _quads(g, n):
    h = n // 2
    return [{(r, c): g[(r + i * h, c + j * h)] for r in range(h) for c in range(h)}
            for i in range(2) for j in range(2)]


def _gadd(x, y):
    return {k: lax.add(x[k], y[k]) for k in x}


def _gsub(x, y):
    return {k: lax.sub(x[k], y[k]) for k in x}


LEFT = ((2, 1, 3), (0, 1, 1), (3,), (1, -1, 3), (0, 1, 3), (0,), (2, -1, 0))
RIGHT = ((0,), (3,), (2, -1, 0), (2, 1, 3), (0, 1, 3), (1, -1, 3), (0, 1, 1))
LEFT_O = ((0,), (3,), (2, 1, 3), (2, -1, 0), (0, 1, 3), (0, 1, 1), (1, -1, 3))
RIGHT_O = ((1, -1, 3), (2, -1, 0), (0,), (0, 1, 1), (0, 1, 3), (3,), (2, 1, 3))


def _factor(rule, quad):
    if len(rule) == 1:
        return quad(rule[0])
    return (_gadd if rule[1] > 0 else _gsub)(quad(rule[0]), quad(rule[2]))


def _factors(rules, g, n=N):
    if n == 1:
        return [g[(0, 0)]]
    quads = _quads(g, n)
    return [x for rule in rules for x in _factors(rules, _factor(rule, quads.__getitem__), n // 2)]


def _combine(product, emit, n=N, base=0, left=LEFT, which=range(7), partial=None):
    if n == 1:
        return emit(0, 0, product(base))
    h = n // 2
    a, b, s = partial or ({}, {}, {})

    def use(i, r, c, m):
        k = r, c
        if i < 2:
            (a, b)[i][k] = m
        elif i == 3:
            s[k] = lax.add(s[k], m)
        elif left is LEFT:
            if i == 2:
                emit(r + h, c, lax.add(a[k], m))
                s[k] = lax.sub(m, b[k])
            elif i == 4:
                emit(r, c, lax.add(s[k], m))
                s[k] = lax.sub(m, a[k])
            elif i == 5:
                emit(r, c + h, lax.add(b[k], m))
                s[k] = lax.add(s[k], m)
            else:
                emit(r + h, c + h, lax.add(s[k], m))
        elif i == 2:
            emit(r + h, c, lax.add(b[k], m))
            s[k] = lax.sub(a[k], m)
        elif i == 4:
            emit(r + h, c + h, lax.add(s[k], m))
            s[k] = lax.add(b[k], m)
        elif i == 5:
            emit(r, c + h, lax.add(a[k], m))
            s[k] = lax.sub(s[k], m)
        else:
            emit(r, c, lax.add(s[k], m))

    for i in which:
        _combine(product, functools.partial(use, i), h, base + i * 7 ** (h.bit_length() - 1), left)


class _SideWork:
    def __init__(self, lag, never=None):
        self.lag, self.never = lag, never
        self.urgent, self.todo, self.running, self.results = [], [], [], []
        self.clock, self.credit, self.rate, self.cache = 0, 0.0, 0.0, (None,)

    def after(self, x, groups=1):
        old = [r for r in self.results if r[0] <= self.clock - self.lag]
        if not old:
            return x
        key = (self.clock, x.shape, x.dtype == F32)
        if self.cache[0] != key:
            deps = [_rows(value, row, 8) for _, value, row in
                    (old[max(0, len(old) - 1 - 2 * n)] for n in reversed(range(groups)))]
            deps = [_cat([dep if x.dtype == F32 else _words(dep)] * (x.shape[1] // T), 1) for dep in deps]
            deps = _cat([dep for dep in deps for _ in range(x.shape[0] // 8 // groups)], 0)
            self.cache = (key, deps, self.never(x.shape))
        return lax.select(self.cache[2], self.cache[1], x)

    def before(self, words):
        if not self.running or self.running[0][0] > self.clock:
            return words
        x = self.running.pop(0)[1]
        dep = _fold(lax.bitwise_or, [_words(_rows(x, r, 8)) for r in range(0, x.shape[0], 8)])
        return _cat([lax.select(self.never((8, T)), dep, _rows(words, 0, 8)), _rows(words, 8, words.shape[0] - 8)], 0)

    def add(self, cost, run, wait=0, urgent=False):
        (self.urgent if urgent else self.todo).append((self.clock + wait, cost, run))

    def issued(self, tiles, result):
        for i in range(2 * tiles):
            self.clock += 0.5
            self.results = self.results[-40:] + [(self.clock, result, i * (result.shape[0] // G) // (2 * tiles) * G)]
            self.credit += 0.5 * self.rate
            while self.credit > 0:
                ready = [x for x in (self.urgent, self.todo) if x and x[0][0] <= self.clock]
                if not ready:
                    break
                _, cost, run = ready[0].pop(0)
                self.credit -= cost
                run()
            self.credit = min(self.credit, 0.0)

    def finish(self, done=lambda: False):
        while (self.urgent or self.todo) and not done():
            (self.urgent or self.todo).pop(0)[2]()


def _queue_factors(side, rules, load, dst):
    def piece(outer):
        def run():
            h = N // 2
            quad = lambda x: {(r, c): load(x // 2 * h + r, x % 2 * h + c) for r in range(h) for c in range(h)}
            for i, x in enumerate(_factors(rules, _factor(rules[outer], quad), h)):
                ref, idx = dst(outer * 7 + i)
                ref[idx] = lax.convert_element_type(x, BF16)
        return run
    for outer in range(7):
        side.add(50, piece(outer))


def _queue_activation(side, src, dst, chunk):
    kt = src.shape[1] // (N * T)
    for t in range(kt):
        for r0 in range(0, T, G):
            def load(r, c, t=t, r0=r0):
                lo, col = chunk * ROWS + r * T + r0, (c * kt + t) * T
                return lax.convert_element_type(_bf(side.after(_words(src[lo:lo + G, col:col + T]))), F32)
            _queue_factors(side, LEFT, load, lambda i, t=t, r0=r0: (dst[chunk], (i, t, pl.ds(r0, G))))


def _queue_head_weights(side, columns, kt, scale, wops):
    high, shift = jnp.full((G, T), 0xFFFF0000, U32), jnp.full((G, T), 16, U32)
    for t in range(kt):
        for r0 in range(0, T, G):
            def load(r, c, t=t, r0=r0):
                ref, word, half = columns[c]
                w = side.after(ref[pl.ds(word + ((kt * r + t) * T + r0) * PITCH_B, G, stride=PITCH_B), :])
                w = pltpu.bitcast(lax.bitwise_and(w, high) if half else lax.shift_left(w, shift), F32)
                return w if scale is None else w * scale
            _queue_factors(side, RIGHT, load, lambda i, t=t, r0=r0: (wops, (i, t, pl.ds(r0, G))))


def _queue_kv_weights(side, pair, stk, stv, wops):
    _queue_head_weights(side, [(stk, pair, 0), (stk, pair, 1), (stv, pair, 0), (stv, pair, 1)], 1, None, wops)


def _tile(ref, *idx):
    *lead, row = idx
    return ref.bitcast(U32)[(*lead, pl.ds(row * (T // 2), T // 2))]


def _phase_a(barrier, x, wqkv, woa, staged, wops, oops, kbuf, vbuf, ckv, xops, cops, stb, qall, outa, wob, ahead):
    side = _SideWork(0)
    q = {}
    done = set()

    def check(*keys):
        assert all(key in done for key in keys), keys

    def stage(sec, i, heads):
        def run():
            lo, hi = heads[0] * DH_A, (heads[-1] + 1) * DH_A
            if sec < 3:
                w = _bf(side.after(_words(wqkv[i * T:(i + 1) * T, sec * DM + lo:sec * DM + hi]))).T
            else:
                w = _bf(side.after(_words(woa[lo:hi, i * T:(i + 1) * T])))
            w = w.astype(F32)
            for h in heads:
                staged[i, h * PITCH_A:h * PITCH_A + DH_A, :] = _rows(w, h * DH_A - lo, DH_A)
        return run

    def weights(sec, g, t, r0):
        def permuted(slab, j):
            w = side.after(staged[slab, pl.ds(r0 % HA * PITCH_A + 4 * j + r0 // HA, G, stride=PITCH_A), :])
            return w * (float(DH_A ** -0.5) * LOG2E) if sec == 0 else w

        load = (lambda r, c: permuted(2 * r + t, g * N + c)) if sec < 3 else (
            lambda r, c: permuted(g * N + c, 2 * r + t))
        _queue_factors(side, RIGHT, load, lambda i: (wops[sec == 0][g], (i, t, pl.ds(r0, G))))

    def project(sec, c, g):
        left, right = xops[c] if sec < 3 else oops[c % 2], wops[sec == 0][g]

        def product(i):
            a, w = (_cat([_tile(left, i, t, 0) for t in range(2)], 1), [_tile(right, i, t, 0) for t in range(2)])
            out = _mm_nt(_bf(a), _bf(_cat(w, 1))) if sec < 3 else _mm(_bf(a), _bf(_cat(w, 0)))
            side.issued(2, out)
            return out

        def emit(r, col, val):
            r0, j = c * ROWS + r * T, g * N + col
            if sec == 0:
                q[(r0, j)] = val
            elif sec == 3:
                outa[r0:r0 + T, j * T:(j + 1) * T] = val.astype(BF16)
            else:
                (kbuf if sec == 1 else vbuf)[j, HALO + r0:HALO + r0 + T, :] = val

        _combine(product, emit)

    def first_keys(r, half):
        for j in range(N * half, N * half + N):
            w = _cat([_cat([staged[slab, pl.ds(4 * j + d, HA, stride=PITCH_A), :] for d in range(4)], 0)
                      for slab in (2 * r, 2 * r + 1)], 1)
            out = _mm_nt(x[0:ROWS, 2 * r * T:(2 * r + 2) * T], w.astype(BF16))
            side.issued(2 * N, _rows(out, ROWS - T, T))
            kbuf[j, HALO:HALO + ROWS, :] = out + kbuf[j, HALO:HALO + ROWS, :] if r else out

    def project_queries(quad, c):
        left, right = xops[c], wops[quad != SPARE_QUAD][quad % 2]

        def product(i):
            out = _mm(_bf(_cat([_tile(left, i, t, 0) for t in range(2)], 1)),
                      _bf(_cat([_tile(right, i, t, 0) for t in range(2)], 0)))
            side.issued(2, out)
            return out

        def emit(r, h, val):
            qall[4 * quad + h, c * ROWS + r * T:c * ROWS + (r + 1) * T, :] = val.astype(BF16)

        _combine(product, emit)

    row = lax.broadcasted_iota(jnp.int32, (E, T), 0)

    def probs(r0):
        qs = side.after(_cat([_rows(q[(r0 - r0 % T, j)], r0 % T, E) for j in range(8)], 0)).reshape(8, E, T)
        logits = []
        for w in range(WIN):
            lo = HALO + r0 - DIL * w
            s = jnp.sum(lax.mul(qs, kbuf[:, lo:lo + E, :]), axis=0)
            s = s + pltpu.roll(s, 2 * HA, 1)
            s = s + pltpu.roll(s, HA, 1)
            logits.append(jnp.where(row + r0 >= DIL * w, s, NEG) if r0 < DIL * w else s)
        m = _fold(jnp.maximum, logits)
        e = [jnp.exp2(s - m) for s in logits]
        inv = _reciprocal(_fold(jnp.add, e))
        for w in range(WIN):
            kbuf[w, r0:r0 + E, :] = e[w] * inv

    def mix(r0, j):
        p = side.after(kbuf[:, r0:r0 + E, :].reshape(WIN * E, T))
        vbuf[j:j + 2, r0:r0 + E, :] = _fold(lax.add, [
            lax.mul(lax.broadcast(_rows(p, w * E, E), (2,)),
                    vbuf[j:j + 2, HALO + r0 - DIL * w:HALO + r0 - DIL * w + E, :]) for w in range(WIN)])

    def queue_output(c):
        for t in range(2):
            for r0 in range(0, T, G):
                def load(r, col, t=t, r0=r0):
                    lo = c * ROWS + r * T + r0
                    return side.after(vbuf[2 * col + t, lo:lo + G, :])
                _queue_factors(side, LEFT, load, lambda i, t=t, r0=r0: (oops[c % 2], (i, t, pl.ds(r0, G))))

    def stage_heads(base, st, m0, count):
        def run():
            lo = m0 * HB // 2
            w = side.after(qall.bitcast(U32)[base + lo // (S // 2), pl.ds(lo % (S // 2), count * HB // 2), :])
            for i in range(count):
                st[(m0 + i) * PITCH_B:(m0 + i) * PITCH_B + HB // 2, :] = _rows(w, i * HB // 2, HB // 2)
        return run

    def needs(kind, num):
        if kind == "F":
            return [("s", 1, 2 * num[0] + 1)]
        if kind == "P":
            return [("W", num[0]), ("b", num[1]), ("t", "qqqqvvkk"[num[0]])]
        return [("w", "QKVO".index(kind), num[1]), ("o" if kind == "O" else "x", num[0])] if kind in "QKVO" else []

    def overwrites(kind, num):
        if kind == "w" and num[0] >= 2:
            return [("K", 3, num[1]) if num[0] == 2 else
                    ("P", SPARE_QUAD, 3) if SPARE_QUAD % 2 == num[1] else ("V", 3, num[1])]
        if kind == "W":
            before = num[0] - 2 - 2 * (num[0] - 2 == SPARE_QUAD)
            return [("V", 3, num[0] % 2) if num[0] == SPARE_QUAD else
                    ("P", before, 3) if before >= 0 else ("Q", 3, num[0]), ("t", "q")]
        if kind == "b":
            return [("V", num[0], 1)]
        return [("O", num[0] - 2, 1)] if kind == "o" and num[0] >= 2 else []

    for step in STEPS.split():
        kind, arg = step[0], step[1:]
        num = [int(a) for a in arg.split(",")] if arg[:1].isdigit() else []
        key = (kind, *num)
        side.finish(lambda: all(need in done for need in needs(kind, num)))
        check(*needs(kind, num))
        if kind == "|":
            side.finish()
            barrier(*arg.split(">"))
            zeros = vbuf[0, HALO + S:HALO + S + 8, :]
            side.results, side.credit = [], 0.0
            side.never = lambda shape, z=zeros: _cat([_cat([z] * (shape[1] // T), 1)] * (shape[0] // 8), 0) != 0
        elif kind == ">":
            if "g" in arg:
                side.finish(lambda: all(("x", c) in done for c in range(S // ROWS)))
            barrier("", arg)
        elif kind == "l":
            side.lag = num[0]
        elif kind == "r":
            side.rate = num[0] / (10 if num[0] > 200 else 1)
        elif kind in "QKVO":
            project("QKVO".index(kind), *num)
            done.add(key)
        elif kind == "F":
            first_keys(*num)
        elif kind == "P":
            project_queries(*num)
            done.add(key)
        elif kind == "s":
            for i in range(*num[1:] or [8]):
                for h in range(0, HA, 8):
                    side.add(80, stage(num[0], i, range(h, h + 8)))
                side.add(0, functools.partial(done.add, ("s", num[0], i)))
        elif kind in "wxobW":
            side.add(0, functools.partial(check, *overwrites(kind, num)))
            if kind == "w":
                for t in range(2):
                    for r0 in range(0, T, G):
                        weights(*num, t, r0)
            elif kind in "xb":
                _queue_activation(side, x, xops, *num)
            elif kind == "W":
                _queue_head_weights(side, [(stb[0], 2 * num[0] + h // 2, h % 2) for h in range(4)], 2,
                                    float(T ** -0.5) * LOG2E, wops[num[0] != SPARE_QUAD][num[0] % 2])
            else:
                queue_output(*num)
            side.add(0, functools.partial(done.add, key))
        elif kind in "pm":
            check(("Q" if kind == "p" else "V", num[0], 1))
            for r0 in range(num[0] * ROWS, (num[0] + 1) * ROWS, E)[slice(*num[1:] or [None])]:
                if kind == "p":
                    side.add(28 * E, functools.partial(probs, r0))
                else:
                    for j in range(0, 8, 2):
                        side.add(5 * E, functools.partial(mix, r0, j))
        elif kind == "c":
            _queue_activation(side, ckv, cops, *num)
        elif kind == "t":
            st = stb["qkv".index(arg)]
            for m0 in range(0, st.shape[0] // PITCH_B, 4):
                side.add(30, stage_heads({"q": 0, "v": 16, "k": 24}[arg], st, m0, 4))
            side.add(0, functools.partial(done.add, ("t", arg)))
        elif kind == "R":
            for cost, run in _stored_factors(side, RIGHT_O, RIGHT_O[0], _weight_blocks(wob), iter(_slots(ahead)))[1]:
                side.add(2.5 * cost, run)
        elif kind == "U":
            side.add(0, functools.partial(check, ("t", "v"), ("t", "k"), ("P", 6, 3)))
            _queue_kv_weights(side, 0, stb[1], stb[2], wops[1][0])
    side.finish()


def _pair_body(pair, cops, stk, stv, wops, qall, ctx):
    side = _SideWork(4, lambda shape: lax.broadcast(pair < 0, shape))
    side.rate = 40
    k, v = {}, {}

    def product(j, i):
        out = _mm(_bf(side.before(_tile(cops[j], i, 0, 0))), _bf(side.before(_tile(wops, i, 0, 0))))
        side.issued(1, out)
        return out

    def project(j):
        def emit(r, c, val):
            (k if c < 2 else v)[(c % 2, N * j + r)] = val

        _combine(functools.partial(product, j), emit)

    causal = lax.broadcasted_iota(jnp.int32, (T, T), 1) <= lax.broadcasted_iota(jnp.int32, (T, T), 0)

    def scores(h, i):
        s = _mm_nt(_bf(_tile(qall, 2 * pair + h, i)), _cat([k[(h, t)] for t in range(i + 1)], 0).astype(BF16))
        s = [s[:, t * T:(t + 1) * T] for t in range(i + 1)]
        for t in range(0, i + 1, 4):
            side.issued(min(4, i + 1 - t), s[t])
        s[i] = jnp.where(causal, s[i], NEG)
        return s, jnp.max(_fold(jnp.maximum, s), axis=1, keepdims=True)

    def attend(h, i, s, m):
        e = [jnp.exp2(x - m) for x in s]
        acc = None
        for t in range(0, i + 1, 4):
            ts = range(t, min(t + 4, i + 1))
            part = _mm(_cat([e[u] for u in ts], 1).astype(BF16), _cat([v[(h, u)] for u in ts], 0).astype(BF16))
            acc = part if acc is None else acc + part
            side.issued(len(ts), acc)

        def normalize(r0):
            def run():
                part = side.after(_fold(lax.add, [_rows(x, r0, G) for x in e]))
                out = _rows(acc, r0, G) * _reciprocal(jnp.sum(part, axis=1, keepdims=True))
                ctx[i, 2 * pair + h, r0:r0 + G, :] = out
                side.running.append((side.clock + 6, out))
            return run
        for r0 in range(0, T, G):
            side.add(40 + 2 * i, normalize(r0), wait=8, urgent=True)

    project(0)
    project(1)
    live = []
    for i in range(N, S // T):
        for h in range(2):
            live.append((h, i, *scores(h, i)))
            if (i % N, h) == (0, 1) and i // N + 1 < S // ROWS:
                project(i // N + 1)
            if (i, h) == (9, 0):
                _queue_kv_weights(side, jnp.minimum(pair + 1, HB // 2 - 1), stk, stv, wops)
            while len(live) > 1:
                attend(*live.pop(0))
    for unit in live + [(h, i, *scores(h, i)) for i in reversed(range(N)) for h in range(2)]:
        attend(*unit)
    side.results = []
    side.finish()


def _context_blocks(ctx):
    return {(r, c): [lambda i=(r * MT + m, c * KT + t): ctx[i] for m in range(MT) for t in range(KT)]
            for r in range(2 * N) for c in range(2 * N)}


def _weight_blocks(wob):
    return {(r, c): [lambda i=(2 * c + r // N, r % N * KT + t): _bf(_tile(wob, *i)).astype(F32) for t in range(KT)]
            for r in range(2 * N) for c in range(2 * N)}


def _lazy_factor(rule, g, n):
    quads = _quads(g, n)
    if len(rule) == 1:
        return quads[rule[0]]
    op = lax.add if rule[1] > 0 else lax.sub
    return {k: [functools.cache(lambda x=x, y=y: op(x(), y())) for x, y in zip(quads[rule[0]][k], quads[rule[2]][k])]
            for k in quads[0]}


def _stored_factors(side, rules, rule, g, slots):
    quads = _quads(g, 2 * N)
    first = _quads(quads[rule[0]], N)
    sums = [j for j, inner in enumerate(rules) if len(rule + inner) > 2]
    out = [{k: [] for k in first[0]} if j in sums else first[inner[0]] for j, inner in enumerate(rules)]
    jobs = []
    for k in first[0]:
        for t in range(len(first[0][k])):
            where = {j: next(slots) for j in sums}
            for j, (ref, idx) in where.items():
                out[j][k].append(lambda ref=ref, idx=idx: pltpu.bitcast(ref[idx], F32))

            def run(k=k, t=t, where=where):
                top = _factor(rule, lambda q: {i: side.after(x[k][t](), T // G) if q == rule[0] else x[k][t]()
                                               for i, x in enumerate(_quads(quads[q], N))})
                for j, (ref, idx) in where.items():
                    ref[idx] = pltpu.bitcast(_factor(rules[j], lambda q: {0: top[q]})[0], ref.dtype)
            jobs.append((len(sums) * T // 8, run))
    return out, jobs


def _slots(ref, *lead):
    return [(ref, (*lead, pl.ds(lo, T))) for lo in range(0, ref.shape[-2] - T + 1, T)]


def _phase_o(ctx, wob, even, odd, partial, stage, out_h, sems):
    zeros = stage.bitcast(U32)[S // 2:S // 2 + 8, 0:T]
    side = _SideWork(1, lambda shape: _cat([zeros] * (shape[0] // 8), 0) != 0)
    blocks = _context_blocks(ctx), _weight_blocks(wob)
    jobs, operands = [], []
    for i in range(7):
        slots = iter(odd if i % 2 else even)
        right, more = _stored_factors(side, RIGHT_O, RIGHT_O[i], blocks[1], slots)
        if i:
            left, work = _stored_factors(side, LEFT_O, LEFT_O[i], blocks[0], slots)
            jobs.append(work + more)
        else:
            left = [_lazy_factor(rule, _lazy_factor(LEFT_O[i], blocks[0], 2 * N), N) for rule in LEFT_O]
        operands += [(_lazy_factor(LEFT_O[k], left[j], 2)[0, 0], _lazy_factor(RIGHT_O[k], right[j], 2)[0, 0])
                     for j in range(7) for k in range(7)]
    jobs.append([])

    def room(i):
        left, level = 320, i
        for _ in range(3):
            left -= MT * 16 * (level % 7 != 6)
            if level % 7 not in (2, 4, 5, 6):
                break
            level //= 7
        if i < NPROD and len(LEFT_O[i // 7]) > 1:
            seen = {q for k in range(i % 7) for q in LEFT_O[k][::2]}
            left -= MT * KT * 16 * len(set(LEFT_O[i % 7][::2]) - seen)
        return max(left, 0)

    ready, started = [], []

    def send(r, c, size):
        rows, cols = pl.ds(r * MT * T, size * MT * T), pl.ds(c * T, size * T)
        started.append(pltpu.make_async_copy(stage.at[rows, cols], out_h.at[rows, pl.ds(DM + c * T, size * T)],
                                             sems.at[0]))
        started[-1].start()

    def flush():
        size = N if len(ready) % (N * N) == 0 else 1
        for r, c in ready:
            if r % size == 0 and c % size == 0:
                send(r, c, size)
        ready.clear()

    def emit(r, c, val):
        stage[r * MT * T:(r + 1) * MT * T, c * T:(c + 1) * T] = val.astype(BF16)
        ready.append((r, c))

    zero = pltpu.bitcast(zeros, jnp.int32)[0, 0]

    def product(i):
        if i % NPROD == 0:
            side.results, side.cache = [], (None,)

            @pl.when(zero > 0)
            def _():
                even[-1][0][pl.ds(pl.multiple_of(8 * jnp.clip(zero, 0, 1), 8), 8), :] = jnp.zeros((8, T), F32)
        if i in (315, 329, 336, 339, 341, 342):
            flush()
        x, y = ([tile() for tile in g] for g in operands[i])
        out = _mm(_cat([_cat(x[m * KT:(m + 1) * KT], 1) for m in range(MT)], 0).astype(BF16), _cat(y, 0).astype(BF16))
        queue = jobs[i // NPROD]
        left = sum(room(k) for k in range(i, i - i % NPROD + NPROD))
        share = sum(cost for cost, _ in queue) * (1 if left <= room(i) else room(i) / left)
        side.rate, side.credit = share / (MT * KT), 0.0
        while share > 0 and queue:
            share -= queue[0][0]
            side.add(*queue.pop(0))
        side.issued(MT * KT, out)
        side.finish()
        return out

    for i in range(0, 6, 2):
        lax.fori_loop(0, jnp.clip(zero + 1, 1, 2),
                      lambda _, carry: _combine(product, emit, 2 * N, 0, LEFT_O, (i, i + 1), partial), None)
        flush()
    _combine(product, emit, 2 * N, 0, LEFT_O, (6,), partial)
    flush()
    for cp in started:
        cp.wait()


def _kernel(xa_h, wqkv_h, woa_h, xb_h, ckv_h, wq_h, wuk_h, wuv_h, wob_h, out_h,
            cops, stk, stv, wops, qall, outa, wob, ahead, sems):
    copy_a = [pltpu.make_async_copy(outa.at[pl.ds(c * ROWS, ROWS)], out_h.at[pl.ds(c * ROWS, ROWS), pl.ds(0, DM)],
                                    sems.at[c]) for c in range(S // ROWS)]

    def first(x, wqkv, woa, staged, wops2, oops, kbuf, vbuf, ckv, xops, stq):
        def x_rows(lo, hi):
            return xa_h.at[pl.ds(lo, hi - lo)], x.at[pl.ds(lo, hi - lo)]

        def w_cols(sec):
            return wqkv_h.at[:, pl.ds(sec * DM, DM)], wqkv.at[:, pl.ds(sec * DM, DM)]

        def quarter(r):
            k = pl.ds(r * DM // N, DM // N)
            return [(wqkv_h.at[k, pl.ds(DM, DM)], wqkv.at[k, pl.ds(DM, DM)]),
                    (xa_h.at[pl.ds(0, ROWS), k], x.at[pl.ds(0, ROWS), k])]

        groups = {
            "y": quarter(0)[:1], "z": quarter(0)[1:], "a": quarter(1), "b": quarter(2), "k": quarter(3),
            "c": [x_rows(ROWS, 2 * ROWS)],
            "d": [x_rows(2 * ROWS, S)],
            "e": [w_cols(0), w_cols(2), (woa_h, woa)],
            "f": [(wq_h, qall.at[0:16])],
            "g": [(xb_h, x)],
            "h": [(wuv_h, qall.at[16:24])],
            "i": [(wuk_h, qall.at[24:32])],
            "j": [(ckv_h, ckv)] + [(wob_h.at[:, :, pl.ds(j * T, T)], wob.at[2 * j:2 * j + 2]) for j in range(8)],
        }
        slot = iter(range(4, 32))
        copies = {k: [pltpu.make_async_copy(src, dst, sems.at[next(slot)]) for src, dst in v]
                  for k, v in groups.items()}
        copies.update({str(c): [cp] for c, cp in enumerate(copy_a)})

        def barrier(wait, start=""):
            for name in wait:
                for cp in copies[name]:
                    cp.wait()
            for name in start:
                for cp in copies[name]:
                    cp.start()

        barrier("", "yza")
        kbuf[:, 0:HALO, :] = jnp.zeros((8, HALO, T), F32)
        vbuf[:, 0:HALO, :] = jnp.zeros((8, HALO, T), F32)
        vbuf[0, HALO + S:HALO + S + 8, :] = jnp.zeros((8, T), F32)
        _phase_a(barrier, x, wqkv, woa, staged, (wops2[:2], [wops, wops2[2]]), oops, kbuf, vbuf, ckv,
                 xops, cops, (stq, stk, stv), qall, outa, wob, ahead)

    factors = pltpu.VMEM((NPROD, 2, T, T), BF16)
    pl.run_scoped(
        first,
        pltpu.VMEM((S, DM), BF16), pltpu.VMEM((DM, 3 * DM), BF16), pltpu.VMEM((DM, DM), BF16),
        pltpu.VMEM((8, HA * PITCH_A, T), F32), [factors] * 3, [factors] * 2,
        pltpu.VMEM((8, HALO + S, T), F32), pltpu.VMEM((8, HALO + S + 8, T), F32),
        pltpu.VMEM((S, DC), BF16),
        [factors] * 4,
        pltpu.VMEM((DM * PITCH_B, T), U32))

    def second(ctx, sums, partial):
        outa[S:S + 16, 0:T] = jnp.zeros((16, T), BF16)

        pl.loop(0, HB // 2)(lambda i: _pair_body(i, cops, stk, stv, wops, qall, ctx))
        for cp in copy_a:
            cp.wait()
        even = _slots(ahead) + _slots(sums)
        odd = _slots(stk) + _slots(stv) + [slot for h in range(HB) for slot in _slots(qall.bitcast(U32), h)]
        _phase_o(ctx, wob, even, odd, partial, outa, out_h, sems)

    pl.run_scoped(second, pltpu.VMEM((S // T, HB, T, T), F32), pltpu.VMEM((7 * 4 * MT * KT * T, T), F32),
                  [pltpu.VMEM((N, N, MT * T, T), F32)] * 3)


def _call(A_x, A_wqkv, A_wo, B_x, B_c_kv, B_w_q, B_w_uk, B_w_uv, B_w_o):
    any_spec = pl.BlockSpec(memory_space=pl.ANY)
    out = pl.pallas_call(
        _kernel,
        out_shape=jax.ShapeDtypeStruct((S, 2 * DM), BF16),
        in_specs=[any_spec] * 9,
        out_specs=any_spec,
        scratch_shapes=[
            [pltpu.VMEM((NPROD, 1, T, T), BF16)] * 4,
            pltpu.VMEM((DC * PITCH_B, T), U32),
            pltpu.VMEM((DC * PITCH_B, T), U32),
            pltpu.VMEM((NPROD, 2, T, T), BF16),
            pltpu.VMEM((HB, S, T), BF16),
            pltpu.VMEM((S + 16, DM), BF16),
            pltpu.VMEM((16, S, T), BF16),
            pltpu.VMEM((7 * 4 * KT * T, T), U32),
            pltpu.SemaphoreType.DMA((32,)),
        ],
        compiler_params=pltpu.CompilerParams(vmem_limit_bytes=126 * 1024 * 1024),
        name="concat_heads",
    )(A_x.reshape(S, DM), A_wqkv, A_wo, B_x.reshape(S, DM), B_c_kv.reshape(S, DC),
      B_w_q.reshape(16, S, T), B_w_uk.reshape(8, S, T), B_w_uv.reshape(8, S, T),
      B_w_o.reshape(2, S, DM))
    return out.reshape(1, S, 2 * DM)


@jax.jit
def pallas_concat_heads__sliding_local_dilated__compressed_kv_cla__prompt_kernel(
    A_x: jax.Array,
    A_wqkv: jax.Array,
    A_wo: jax.Array,
    B_x: jax.Array,
    B_c_kv: jax.Array,
    B_w_q: jax.Array,
    B_w_uk: jax.Array,
    B_w_uv: jax.Array,
    B_w_o: jax.Array,
):
    return _call(A_x, A_wqkv, A_wo, B_x, B_c_kv, B_w_q, B_w_uk, B_w_uv, B_w_o)
```

```python
import functools

import numpy as np

import jax
import jax.numpy as jnp
from jax import lax
import jax.experimental.pallas as pl
import jax.experimental.pallas.tpu as pltpu

F32, BF16, U32 = jnp.float32, jnp.bfloat16, jnp.uint32
LOG2E = float(np.log2(np.e))
NEG = -1e9 * LOG2E
T = 128
N = 4
NPROD = 49
ROWS = N * T

S = 2048
DM = 1024
DC = 512
HB = 32
WIN, DIL, HA, DH_A = 8, 2, 32, 32
HALO = 16
E = 8
G = 16
PITCH_B = 17
PITCH_A = 33
MT, KT = S // T // (2 * N), HB // (2 * N)

STEPS = """
    l3 |y>b s1,0,2 !all |z>k F0,0 |a>c s1,2,4 r405 F0,1 F1,0 |b>d s1,4,6 F1,1 |k r88 s1,6,8 w1,0 F2,0 F2,1
        |c>e r98 x1 F3,0 F3,1 r545 w1,1 K1,0 |d>f r66 x2 K1,1 r30 x3 K2,0 K2,1
    |e l2 r50 s0 w0,0 x0 K3,0 K3,1 w0,1 Q1,0 >ghi r475 s2 w2,0 w2,1 Q2,0 Q0,0 Q0,1 p0 Q3,0 Q1,1 Q2,1 Q3,1
    |fg>j l3 r485 p1,0,32 tq p1,32,64 W0 b0 b1 V0,0 V0,1 V1,0 V1,1 b2 b3 V2,0 V2,1 V3,0 V3,1 W1 m0 P0,0 P0,1
        P0,2 P0,3 W2 p2,0,16 s3 w3,1 o0 P1,0 P1,1 P1,2 P1,3 W3 P2,0 P2,1 P2,2 P2,3
    |hij l4 r48 W4 tv m1 w3,0 p2,16,64 P3,0 P3,1 P3,2 P3,3 W5 p3,0,48 P4,0 P4,1 P4,2 P4,3 O0,0 O0,1 W6
        p3,48,64 tk o1 m2 P5,0 P5,1 P5,2 P5,3 W7 o2 m3 P6,0 P6,1 P6,2 P6,3 O1,0 O1,1 >01 r45 P7,0 P7,1 !
        r435 o3 U R c0 c1 c2 c3 P7,2 P7,3 O2,0 O2,1 O3,0 O3,1 >23"""
SPARE_QUAD = 2


def _mm(a, b):
    return jnp.dot(a, b, preferred_element_type=F32)


def _mm_nt(a, b):
    return lax.dot_general(a, b, (((1,), (1,)), ((), ())), preferred_element_type=F32)


def _cat(xs, axis):
    xs = list(xs)
    return xs[0] if len(xs) == 1 else lax.concatenate(xs, axis)


def _rows(x, start, size):
    return lax.slice_in_dim(x, start, start + size, axis=0)


def _fold(op, xs):
    xs = list(xs)
    acc = xs[0]
    for x in xs[1:]:
        acc = op(acc, x)
    return acc


def _conceal(zero, refs):
    @pl.when(zero > 0)
    def _():
        for ref in refs:
            rows = pl.ds(pl.multiple_of(G * jnp.clip(zero, 0, 1), G), G)
            ref[(*[0] * (len(ref.shape) - 2), rows)] = jnp.zeros((G, T), ref.dtype)


def _bf(words):
    return pltpu.bitcast(words, BF16)


def _words(x):
    return pltpu.bitcast(x, U32)


def _reciprocal(x):
    r = pltpu.reciprocal(x, approx=True)
    return r * (2.0 - x * r)


def _quads(g, n):
    h = n // 2
    return [{(r, c): g[(r + i * h, c + j * h)] for r in range(h) for c in range(h)}
            for i in range(2) for j in range(2)]


def _gadd(x, y):
    return {k: lax.add(x[k], y[k]) for k in x}


def _gsub(x, y):
    return {k: lax.sub(x[k], y[k]) for k in x}


LEFT = ((2, 1, 3), (0, 1, 1), (3,), (1, -1, 3), (0, 1, 3), (0,), (2, -1, 0))
RIGHT = ((0,), (3,), (2, -1, 0), (2, 1, 3), (0, 1, 3), (1, -1, 3), (0, 1, 1))
LEFT_O = ((0,), (3,), (2, 1, 3), (2, -1, 0), (0, 1, 3), (0, 1, 1), (1, -1, 3))
RIGHT_O = ((1, -1, 3), (2, -1, 0), (0,), (0, 1, 1), (0, 1, 3), (3,), (2, 1, 3))


def _factor(rule, quad):
    if len(rule) == 1:
        return quad(rule[0])
    return (_gadd if rule[1] > 0 else _gsub)(quad(rule[0]), quad(rule[2]))


def _factors(rules, g, n=N):
    if n == 1:
        return [g[(0, 0)]]
    quads = _quads(g, n)
    return [x for rule in rules for x in _factors(rules, _factor(rule, quads.__getitem__), n // 2)]


def _combine(product, emit, n=N, base=0, left=LEFT, which=range(7), partial=None):
    if n == 1:
        return emit(0, 0, product(base))
    h = n // 2
    a, b, s = partial or ({}, {}, {})

    def use(i, r, c, m):
        k = r, c
        if i < 2:
            (a, b)[i][k] = m
        elif i == 3:
            s[k] = lax.add(s[k], m)
        elif left is LEFT:
            if i == 2:
                emit(r + h, c, lax.add(a[k], m))
                s[k] = lax.sub(m, b[k])
            elif i == 4:
                emit(r, c, lax.add(s[k], m))
                s[k] = lax.sub(m, a[k])
            elif i == 5:
                emit(r, c + h, lax.add(b[k], m))
                s[k] = lax.add(s[k], m)
            else:
                emit(r + h, c + h, lax.add(s[k], m))
        elif i == 2:
            emit(r + h, c, lax.add(b[k], m))
            s[k] = lax.sub(a[k], m)
        elif i == 4:
            emit(r + h, c + h, lax.add(s[k], m))
            s[k] = lax.add(b[k], m)
        elif i == 5:
            emit(r, c + h, lax.add(a[k], m))
            s[k] = lax.sub(s[k], m)
        else:
            emit(r, c, lax.add(s[k], m))

    for i in which:
        _combine(product, functools.partial(use, i), h, base + i * 7 ** (h.bit_length() - 1), left)


class _SideWork:
    def __init__(self, lag, never=None):
        self.lag, self.never = lag, never
        self.urgent, self.todo, self.running, self.results = [], [], [], []
        self.clock, self.credit, self.rate, self.cache = 0, 0.0, 0.0, (None,)

    def after(self, x, groups=1):
        old = [r for r in self.results if r[0] <= self.clock - self.lag]
        if not old:
            return x
        key = (self.clock, x.shape, x.dtype == F32)
        if self.cache[0] != key:
            deps = [_rows(value, row, 8) for _, value, row in
                    (old[max(0, len(old) - 1 - 2 * n)] for n in reversed(range(groups)))]
            deps = [_cat([dep if x.dtype == F32 else _words(dep)] * (x.shape[1] // T), 1) for dep in deps]
            deps = _cat([dep for dep in deps for _ in range(x.shape[0] // 8 // groups)], 0)
            self.cache = (key, deps, self.never(x.shape))
        return lax.select(self.cache[2], self.cache[1], x)

    def before(self, words):
        if not self.running or self.running[0][0] > self.clock:
            return words
        x = self.running.pop(0)[1]
        dep = _fold(lax.bitwise_or, [_words(_rows(x, r, 8)) for r in range(0, x.shape[0], 8)])
        return _cat([lax.select(self.never((8, T)), dep, _rows(words, 0, 8)), _rows(words, 8, words.shape[0] - 8)], 0)

    def add(self, cost, run, wait=0, urgent=False):
        (self.urgent if urgent else self.todo).append((self.clock + wait, cost, run))

    def issued(self, tiles, result):
        for i in range(2 * tiles):
            self.clock += 0.5
            self.results = self.results[-40:] + [(self.clock, result, i * (result.shape[0] // G) // (2 * tiles) * G)]
            self.credit += 0.5 * self.rate
            while self.credit > 0:
                ready = [x for x in (self.urgent, self.todo) if x and x[0][0] <= self.clock]
                if not ready:
                    break
                _, cost, run = ready[0].pop(0)
                self.credit -= cost
                run()
            self.credit = min(self.credit, 0.0)

    def finish(self, done=lambda: False):
        while (self.urgent or self.todo) and not done():
            (self.urgent or self.todo).pop(0)[2]()


def _queue_factors(side, rules, load, dst):
    def piece(outer):
        def run():
            h = N // 2
            quad = lambda x: {(r, c): load(x // 2 * h + r, x % 2 * h + c) for r in range(h) for c in range(h)}
            for i, x in enumerate(_factors(rules, _factor(rules[outer], quad), h)):
                ref, idx = dst(outer * 7 + i)
                ref[idx] = lax.convert_element_type(x, BF16)
        return run
    for outer in range(7):
        side.add(50, piece(outer))


def _queue_activation(side, src, dst, top, left=0):
    kt = dst.shape[1]
    for t in range(kt):
        for r0 in range(0, T, G):
            def load(r, c, t=t, r0=r0):
                lo, col = top + r * T + r0, left + (c * kt + t) * T
                return lax.convert_element_type(_bf(side.after(_words(src[lo:lo + G, col:col + T]))), F32)
            _queue_factors(side, LEFT, load, lambda i, t=t, r0=r0: (dst, (i, t, pl.ds(r0, G))))


def _queue_head_weights(side, columns, kt, scale, wops):
    high, shift = jnp.full((G, T), 0xFFFF0000, U32), jnp.full((G, T), 16, U32)
    for t in range(kt):
        for r0 in range(0, T, G):
            def load(r, c, t=t, r0=r0):
                ref, word, half = columns[c]
                w = side.after(ref[pl.ds(word + ((kt * r + t) * T + r0) * PITCH_B, G, stride=PITCH_B), :])
                w = pltpu.bitcast(lax.bitwise_and(w, high) if half else lax.shift_left(w, shift), F32)
                return w if scale is None else w * scale
            _queue_factors(side, RIGHT, load, lambda i, t=t, r0=r0: (wops, (i, t, pl.ds(r0, G))))


def _queue_kv_weights(side, pair, stk, stv, wops):
    _queue_head_weights(side, [(stk, pair, 0), (stk, pair, 1), (stv, pair, 0), (stv, pair, 1)], 1, None, wops)


def _tile(ref, *idx):
    *lead, row = idx
    return ref.bitcast(U32)[(*lead, pl.ds(row * (T // 2), T // 2))]


def _phase_a(barrier, x, wqkv, woa, staged, wops, oops, kbuf, vbuf, xops, cops, stb, qall, outa, wob, ahead):
    side = _SideWork(0)
    q = {}
    done = set()

    def check(*keys):
        assert all(key in done for key in keys), keys

    def stage(sec, i, heads):
        def run():
            lo, hi = heads[0] * DH_A, (heads[-1] + 1) * DH_A
            if sec < 3:
                w = _bf(side.after(_words(wqkv[i * T:(i + 1) * T, sec * DM + lo:sec * DM + hi]))).T
            else:
                w = _bf(side.after(_words(woa[lo:hi, i * T:(i + 1) * T])))
            w = w.astype(F32)
            for h in heads:
                staged[i, h * PITCH_A:h * PITCH_A + DH_A, :] = _rows(w, h * DH_A - lo, DH_A)
        return run

    def weights(sec, g, t, r0):
        def permuted(slab, j):
            w = side.after(staged[slab, pl.ds(r0 % HA * PITCH_A + 4 * j + r0 // HA, G, stride=PITCH_A), :])
            return w * (float(DH_A ** -0.5) * LOG2E) if sec == 0 else w

        load = (lambda r, c: permuted(2 * r + t, g * N + c)) if sec < 3 else (
            lambda r, c: permuted(g * N + c, 2 * r + t))
        _queue_factors(side, RIGHT, load, lambda i: (wops[sec == 0][g], (i, t, pl.ds(r0, G))))

    def project(sec, c, g):
        left, right = xops[c] if sec < 3 else oops[c % 2], wops[sec == 0][g]

        def product(i):
            a, w = (_cat([_tile(left, i, t, 0) for t in range(2)], 1), [_tile(right, i, t, 0) for t in range(2)])
            out = _mm_nt(_bf(a), _bf(_cat(w, 1))) if sec < 3 else _mm(_bf(a), _bf(_cat(w, 0)))
            side.issued(2, out)
            return out

        def emit(r, col, val):
            r0, j = c * ROWS + r * T, g * N + col
            if sec == 0:
                q[(r0, j)] = val
            elif sec == 3:
                outa[r0:r0 + T, j * T:(j + 1) * T] = val.astype(BF16)
            else:
                (kbuf if sec == 1 else vbuf)[j, HALO + r0:HALO + r0 + T, :] = val

        _combine(product, emit)

    def first_keys(r, half):
        for j in range(N * half, N * half + N):
            w = _cat([_cat([staged[slab, pl.ds(4 * j + d, HA, stride=PITCH_A), :] for d in range(4)], 0)
                      for slab in (2 * r, 2 * r + 1)], 1)
            out = _mm_nt(x[0:ROWS, 2 * r * T:(2 * r + 2) * T], w.astype(BF16))
            side.issued(2 * N, _rows(out, ROWS - T, T))
            kbuf[j, HALO:HALO + ROWS, :] = out + kbuf[j, HALO:HALO + ROWS, :] if r else out

    def project_queries(quad, c):
        left, right = xops[c], wops[quad != SPARE_QUAD][quad % 2]

        def product(i):
            out = _mm(_bf(_cat([_tile(left, i, t, 0) for t in range(2)], 1)),
                      _bf(_cat([_tile(right, i, t, 0) for t in range(2)], 0)))
            side.issued(2, out)
            return out

        def emit(r, h, val):
            qall[4 * quad + h, c * ROWS + r * T:c * ROWS + (r + 1) * T, :] = val.astype(BF16)

        _combine(product, emit)

    row = lax.broadcasted_iota(jnp.int32, (E, T), 0)

    def probs(r0):
        qs = side.after(_cat([_rows(q[(r0 - r0 % T, j)], r0 % T, E) for j in range(8)], 0)).reshape(8, E, T)
        logits = []
        for w in range(WIN):
            lo = HALO + r0 - DIL * w
            s = jnp.sum(lax.mul(qs, kbuf[:, lo:lo + E, :]), axis=0)
            s = s + pltpu.roll(s, 2 * HA, 1)
            s = s + pltpu.roll(s, HA, 1)
            logits.append(jnp.where(row + r0 >= DIL * w, s, NEG) if r0 < DIL * w else s)
        m = _fold(jnp.maximum, logits)
        e = [jnp.exp2(s - m) for s in logits]
        inv = _reciprocal(_fold(jnp.add, e))
        for w in range(WIN):
            kbuf[w, r0:r0 + E, :] = e[w] * inv

    def mix(r0, j):
        p = side.after(kbuf[:, r0:r0 + E, :].reshape(WIN * E, T))
        vbuf[j:j + 2, r0:r0 + E, :] = _fold(lax.add, [
            lax.mul(lax.broadcast(_rows(p, w * E, E), (2,)),
                    vbuf[j:j + 2, HALO + r0 - DIL * w:HALO + r0 - DIL * w + E, :]) for w in range(WIN)])

    def queue_output(c):
        for t in range(2):
            for r0 in range(0, T, G):
                def load(r, col, t=t, r0=r0):
                    lo = c * ROWS + r * T + r0
                    return side.after(vbuf[2 * col + t, lo:lo + G, :])
                _queue_factors(side, LEFT, load, lambda i, t=t, r0=r0: (oops[c % 2], (i, t, pl.ds(r0, G))))

    def stage_heads(base, st, m0, count):
        def run():
            lo = m0 * HB // 2
            w = side.after(qall.bitcast(U32)[base + lo // (S // 2), pl.ds(lo % (S // 2), count * HB // 2), :])
            for i in range(count):
                st[(m0 + i) * PITCH_B:(m0 + i) * PITCH_B + HB // 2, :] = _rows(w, i * HB // 2, HB // 2)
        return run

    def needs(kind, num):
        if kind == "F":
            return [("s", 1, 2 * num[0] + 1)]
        if kind == "P":
            return [("W", num[0]), ("b", num[1]), ("t", "qqqqvvkk"[num[0]])]
        return [("w", "QKVO".index(kind), num[1]), ("o" if kind == "O" else "x", num[0])] if kind in "QKVO" else []

    def overwrites(kind, num):
        if kind == "w" and num[0] >= 2:
            return [("K", 3, num[1]) if num[0] == 2 else
                    ("P", SPARE_QUAD, 3) if SPARE_QUAD % 2 == num[1] else ("V", 3, num[1])]
        if kind == "W":
            before = num[0] - 2 - 2 * (num[0] - 2 == SPARE_QUAD)
            return [("V", 3, num[0] % 2) if num[0] == SPARE_QUAD else
                    ("P", before, 3) if before >= 0 else ("Q", 3, num[0]), ("t", "q")]
        if kind == "b":
            return [("V", num[0], 1)]
        return [("O", num[0] - 2, 1)] if kind == "o" and num[0] >= 2 else []

    for step in STEPS.split():
        kind, arg = step[0], step[1:]
        num = [int(a) for a in arg.split(",")] if arg[:1].isdigit() else []
        key = (kind, *num)
        side.finish(lambda: all(need in done for need in needs(kind, num)))
        check(*needs(kind, num))
        if kind == "|":
            side.finish()
            check(*([("s", 2, 7)] if ">j" in arg else []))
            barrier(*arg.split(">"))
            zeros = vbuf[0, HALO + S:HALO + S + 8, :]
            side.results, side.credit = [], 0.0
            side.never = lambda shape, z=zeros: _cat([_cat([z] * (shape[1] // T), 1)] * (shape[0] // 8), 0) != 0
        elif kind == "!":
            zero = pltpu.bitcast(vbuf[0, HALO + S:HALO + S + 8, :], jnp.int32)[0, 0]
            _conceal(zero, (*xops, *oops, *wops[0], wops[1][1], *cops) if arg else cops)
            side.results = []
        elif kind == ">":
            if "g" in arg:
                side.finish(lambda: all(("x", c) in done for c in range(S // ROWS)))
            barrier("", arg)
        elif kind == "l":
            side.lag = num[0]
        elif kind == "r":
            side.rate = num[0] / (10 if num[0] > 200 else 1)
        elif kind in "QKVO":
            check(*([("b", 3)] if kind == "O" else []))
            project("QKVO".index(kind), *num)
            done.add(key)
        elif kind == "F":
            first_keys(*num)
        elif kind == "P":
            project_queries(*num)
            done.add(key)
        elif kind == "s":
            for i in range(*num[1:] or [8]):
                for h in range(0, HA, 8):
                    side.add(80, stage(num[0], i, range(h, h + 8)))
                side.add(0, functools.partial(done.add, ("s", num[0], i)))
        elif kind in "wxobW":
            side.add(0, functools.partial(check, *overwrites(kind, num)))
            if kind == "w":
                for t in range(2):
                    for r0 in range(0, T, G):
                        weights(*num, t, r0)
            elif kind in "xb":
                _queue_activation(side, x, xops[num[0]], num[0] * ROWS)
            elif kind == "W":
                _queue_head_weights(side, [(stb[0], 2 * num[0] + h // 2, h % 2) for h in range(4)], 2,
                                    float(T ** -0.5) * LOG2E, wops[num[0] != SPARE_QUAD][num[0] % 2])
            else:
                queue_output(*num)
            side.add(0, functools.partial(done.add, key))
        elif kind in "pm":
            check(("Q" if kind == "p" else "V", num[0], 1))
            for r0 in range(num[0] * ROWS, (num[0] + 1) * ROWS, E)[slice(*num[1:] or [None])]:
                if kind == "p":
                    side.add(28 * E, functools.partial(probs, r0))
                else:
                    for j in range(0, 8, 2):
                        side.add(5 * E, functools.partial(mix, r0, j))
        elif kind == "c":
            top = num[0] * ROWS
            _queue_activation(side, wqkv, cops[num[0]], top % DM, top // DM * DC)
        elif kind == "t":
            st = stb["qkv".index(arg)]
            for m0 in range(0, st.shape[0] // PITCH_B, 4):
                side.add(30, stage_heads({"q": 0, "v": 16, "k": 24}[arg], st, m0, 4))
            side.add(0, functools.partial(done.add, ("t", arg)))
        elif kind == "R":
            for cost, run in _stored_factors(side, RIGHT_O, RIGHT_O[0], _weight_blocks(wob), iter(_slots(ahead)))[1]:
                side.add(2.5 * cost, run)
        elif kind == "U":
            side.add(0, functools.partial(check, ("t", "v"), ("t", "k"), ("P", 6, 3)))
            _queue_kv_weights(side, 0, stb[1], stb[2], wops[1][0])
    side.finish()


def _pair_body(pair, cops, stk, stv, wops, qall, ctx):
    side = _SideWork(4, lambda shape: lax.broadcast(pair < 0, shape))
    side.rate = 40
    k, v = {}, {}

    def product(j, i):
        out = _mm(_bf(side.before(_tile(cops[j], i, 0, 0))), _bf(side.before(_tile(wops, i, 0, 0))))
        side.issued(1, out)
        return out

    def project(j):
        def emit(r, c, val):
            (k if c < 2 else v)[(c % 2, N * j + r)] = val

        _combine(functools.partial(product, j), emit)

    causal = lax.broadcasted_iota(jnp.int32, (T, T), 1) <= lax.broadcasted_iota(jnp.int32, (T, T), 0)

    def scores(h, i):
        s = _mm_nt(_bf(_tile(qall, 2 * pair + h, i)), _cat([k[(h, t)] for t in range(i + 1)], 0).astype(BF16))
        s = [s[:, t * T:(t + 1) * T] for t in range(i + 1)]
        for t in range(0, i + 1, 4):
            side.issued(min(4, i + 1 - t), s[t])
        s[i] = jnp.where(causal, s[i], NEG)
        return s, jnp.max(_fold(jnp.maximum, s), axis=1, keepdims=True)

    def attend(h, i, s, m):
        e = [jnp.exp2(x - m) for x in s]
        acc = None
        for t in range(0, i + 1, 4):
            ts = range(t, min(t + 4, i + 1))
            part = _mm(_cat([e[u] for u in ts], 1).astype(BF16), _cat([v[(h, u)] for u in ts], 0).astype(BF16))
            acc = part if acc is None else acc + part
            side.issued(len(ts), acc)

        def normalize(r0):
            def run():
                part = side.after(_fold(lax.add, [_rows(x, r0, G) for x in e]))
                out = _rows(acc, r0, G) * _reciprocal(jnp.sum(part, axis=1, keepdims=True))
                ctx[i, 2 * pair + h, r0:r0 + G, :] = out
                side.running.append((side.clock + 6, out))
            return run
        for r0 in range(0, T, G):
            side.add(40 + 2 * i, normalize(r0), wait=8, urgent=True)

    project(0)
    project(1)
    live = []
    for i in range(N, S // T):
        for h in range(2):
            live.append((h, i, *scores(h, i)))
            if (i % N, h) == (0, 1) and i // N + 1 < S // ROWS:
                project(i // N + 1)
            if (i, h) == (9, 0):
                _queue_kv_weights(side, jnp.minimum(pair + 1, HB // 2 - 1), stk, stv, wops)
            while len(live) > 1:
                attend(*live.pop(0))
    for unit in live + [(h, i, *scores(h, i)) for i in reversed(range(N)) for h in range(2)]:
        attend(*unit)
    side.results = []
    side.finish()


def _context_blocks(ctx):
    return {(r, c): [lambda i=(r * MT + m, c * KT + t): ctx[i] for m in range(MT) for t in range(KT)]
            for r in range(2 * N) for c in range(2 * N)}


def _weight_blocks(wob):
    return {(r, c): [lambda i=(2 * c + r // N, r % N * KT + t): _bf(_tile(wob, *i)).astype(F32) for t in range(KT)]
            for r in range(2 * N) for c in range(2 * N)}


def _lazy_factor(rule, g, n):
    quads = _quads(g, n)
    if len(rule) == 1:
        return quads[rule[0]]
    op = lax.add if rule[1] > 0 else lax.sub
    return {k: [functools.cache(lambda x=x, y=y: op(x(), y())) for x, y in zip(quads[rule[0]][k], quads[rule[2]][k])]
            for k in quads[0]}


def _stored_factors(side, rules, rule, g, slots):
    quads = _quads(g, 2 * N)
    first = _quads(quads[rule[0]], N)
    sums = [j for j, inner in enumerate(rules) if len(rule + inner) > 2]
    out = [{k: [] for k in first[0]} if j in sums else first[inner[0]] for j, inner in enumerate(rules)]
    jobs = []
    for k in first[0]:
        for t in range(len(first[0][k])):
            where = {j: next(slots) for j in sums}
            for j, (ref, idx) in where.items():
                out[j][k].append(lambda ref=ref, idx=idx: pltpu.bitcast(ref[idx], F32))

            def run(k=k, t=t, where=where):
                top = _factor(rule, lambda q: {i: side.after(x[k][t](), T // G) if q == rule[0] else x[k][t]()
                                               for i, x in enumerate(_quads(quads[q], N))})
                for j, (ref, idx) in where.items():
                    ref[idx] = pltpu.bitcast(_factor(rules[j], lambda q: {0: top[q]})[0], ref.dtype)
            jobs.append((len(sums) * T // 8, run))
    return out, jobs


def _slots(ref, *lead):
    return [(ref, (*lead, pl.ds(lo, T))) for lo in range(0, ref.shape[-2] - T + 1, T)]


def _phase_o(ctx, wob, even, odd, partial, stage, out_h, sems):
    zeros = stage.bitcast(U32)[S // 2:S // 2 + 8, 0:T]
    side = _SideWork(1, lambda shape: _cat([zeros] * (shape[0] // 8), 0) != 0)
    blocks = _context_blocks(ctx), _weight_blocks(wob)
    jobs, operands = [], []
    for i in range(7):
        slots = iter(odd if i % 2 else even)
        right, more = _stored_factors(side, RIGHT_O, RIGHT_O[i], blocks[1], slots)
        if i:
            left, work = _stored_factors(side, LEFT_O, LEFT_O[i], blocks[0], slots)
            jobs.append(work + more)
        else:
            left = [_lazy_factor(rule, _lazy_factor(LEFT_O[i], blocks[0], 2 * N), N) for rule in LEFT_O]
        operands += [(_lazy_factor(LEFT_O[k], left[j], 2)[0, 0], _lazy_factor(RIGHT_O[k], right[j], 2)[0, 0])
                     for j in range(7) for k in range(7)]
    jobs.append([])

    def room(i):
        left, level = 320, i
        for _ in range(3):
            left -= MT * 16 * (level % 7 != 6)
            if level % 7 not in (2, 4, 5, 6):
                break
            level //= 7
        if i < NPROD and len(LEFT_O[i // 7]) > 1:
            seen = {q for k in range(i % 7) for q in LEFT_O[k][::2]}
            left -= MT * KT * 16 * len(set(LEFT_O[i % 7][::2]) - seen)
        return max(left, 0)

    ready, started = [], []

    def send(r, c, size):
        rows, cols = pl.ds(r * MT * T, size * MT * T), pl.ds(c * T, size * T)
        started.append(pltpu.make_async_copy(stage.at[rows, cols], out_h.at[rows, pl.ds(DM + c * T, size * T)],
                                             sems.at[0]))
        started[-1].start()

    def flush():
        size = N if len(ready) % (N * N) == 0 else 1
        for r, c in ready:
            if r % size == 0 and c % size == 0:
                send(r, c, size)
        ready.clear()

    def emit(r, c, val):
        stage[r * MT * T:(r + 1) * MT * T, c * T:(c + 1) * T] = val.astype(BF16)
        ready.append((r, c))

    zero = pltpu.bitcast(zeros, jnp.int32)[0, 0]

    def product(i):
        if i % NPROD == 0:
            side.results, side.cache = [], (None,)
            _conceal(zero, [even[-1][0]])
        if i in (315, 329, 336, 339, 341, 342):
            flush()
        x, y = ([tile() for tile in g] for g in operands[i])
        out = _mm(_cat([_cat(x[m * KT:(m + 1) * KT], 1) for m in range(MT)], 0).astype(BF16), _cat(y, 0).astype(BF16))
        queue = jobs[i // NPROD]
        left = sum(room(k) for k in range(i, i - i % NPROD + NPROD))
        share = sum(cost for cost, _ in queue) * (1 if left <= room(i) else room(i) / left)
        side.rate, side.credit = share / (MT * KT), 0.0
        while share > 0 and queue:
            share -= queue[0][0]
            side.add(*queue.pop(0))
        side.issued(MT * KT, out)
        side.finish()
        return out

    for i in range(0, 6, 2):
        lax.fori_loop(0, jnp.clip(zero + 1, 1, 2),
                      lambda _, carry: _combine(product, emit, 2 * N, 0, LEFT_O, (i, i + 1), partial), None)
        flush()
    _combine(product, emit, 2 * N, 0, LEFT_O, (6,), partial)
    flush()
    for cp in started:
        cp.wait()


def _kernel(xa_h, wqkv_h, woa_h, xb_h, ckv_h, wq_h, wuk_h, wuv_h, wob_h, out_h,
            cops, stk, stv, wops, qall, outa, wob, ahead, sems):
    copy_a = [pltpu.make_async_copy(outa.at[pl.ds(c * ROWS, ROWS)], out_h.at[pl.ds(c * ROWS, ROWS), pl.ds(0, DM)],
                                    sems.at[c]) for c in range(S // ROWS)]

    def first(wqkv, woa, staged, wops2, oops, kbuf, vbuf, xops, stq):
        x = outa

        def x_rows(lo, hi):
            return xa_h.at[pl.ds(lo, hi - lo)], x.at[pl.ds(lo, hi - lo)]

        def w_cols(sec):
            return wqkv_h.at[:, pl.ds(sec * DM, DM)], wqkv.at[:, pl.ds(sec * DM, DM)]

        def quarter(r):
            k = pl.ds(r * DM // N, DM // N)
            return [(wqkv_h.at[k, pl.ds(DM, DM)], wqkv.at[k, pl.ds(DM, DM)]),
                    (xa_h.at[pl.ds(0, ROWS), k], x.at[pl.ds(0, ROWS), k])]

        groups = {
            "y": quarter(0)[:1], "z": quarter(0)[1:], "a": quarter(1), "b": quarter(2), "k": quarter(3),
            "c": [x_rows(ROWS, 2 * ROWS)],
            "d": [x_rows(2 * ROWS, S)],
            "e": [w_cols(0), w_cols(2), (woa_h, woa)],
            "f": [(wq_h, qall.at[0:16])],
            "g": [(xb_h, x.at[0:S])],
            "h": [(wuv_h, qall.at[16:24])],
            "i": [(wuk_h, qall.at[24:32])],
            "j": [(ckv_h.at[pl.ds(i * DM, DM)], wqkv.at[:, pl.ds(i * DC, DC)]) for i in range(S // DM)]
                 + [(wob_h.at[:, :, pl.ds(j * T, T)], wob.at[2 * j:2 * j + 2]) for j in range(8)],
        }
        slot = iter(range(4, 32))
        copies = {k: [pltpu.make_async_copy(src, dst, sems.at[next(slot)]) for src, dst in v]
                  for k, v in groups.items()}
        copies.update({str(c): [cp] for c, cp in enumerate(copy_a)})

        def barrier(wait, start=""):
            for name in wait:
                for cp in copies[name]:
                    cp.wait()
            for name in start:
                for cp in copies[name]:
                    cp.start()

        barrier("", "yza")
        kbuf[:, 0:HALO, :] = jnp.zeros((8, HALO, T), F32)
        vbuf[:, 0:HALO, :] = jnp.zeros((8, HALO, T), F32)
        vbuf[0, HALO + S:HALO + S + 8, :] = jnp.zeros((8, T), F32)
        _phase_a(barrier, x, wqkv, woa, staged, (wops2[:2], [wops, wops2[2]]), oops, kbuf, vbuf,
                 xops, cops, (stq, stk, stv), qall, outa, wob, ahead)

    factors = pltpu.VMEM((NPROD, 2, T, T), BF16)
    pl.run_scoped(
        first,
        pltpu.VMEM((DM, 3 * DM), BF16), pltpu.VMEM((DM, DM), BF16),
        pltpu.VMEM((8, HA * PITCH_A, T), F32), [factors] * 3, [factors] * 2,
        pltpu.VMEM((8, HALO + S, T), F32), pltpu.VMEM((8, HALO + S + 8, T), F32),
        [factors] * 4,
        pltpu.VMEM((DM * PITCH_B, T), U32))

    def second(ctx, sums, partial):
        outa[S:S + 16, 0:T] = jnp.zeros((16, T), BF16)
        pl.loop(0, HB // 2)(lambda i: _pair_body(i, cops, stk, stv, wops, qall, ctx))
        for cp in copy_a:
            cp.wait()
        even = _slots(ahead) + _slots(sums)
        odd = _slots(stk) + _slots(stv) + [slot for h in range(HB) for slot in _slots(qall.bitcast(U32), h)]
        _phase_o(ctx, wob, even, odd, partial, outa, out_h, sems)

    pl.run_scoped(second, pltpu.VMEM((S // T, HB, T, T), F32), pltpu.VMEM((7 * 4 * MT * KT * T, T), F32),
                  [pltpu.VMEM((N, N, MT * T, T), F32)] * 3)


def _call(A_x, A_wqkv, A_wo, B_x, B_c_kv, B_w_q, B_w_uk, B_w_uv, B_w_o):
    any_spec = pl.BlockSpec(memory_space=pl.ANY)
    out = pl.pallas_call(
        _kernel,
        out_shape=jax.ShapeDtypeStruct((S, 2 * DM), BF16),
        in_specs=[any_spec] * 9,
        out_specs=any_spec,
        scratch_shapes=[
            [pltpu.VMEM((NPROD, 1, T, T), BF16)] * 4,
            pltpu.VMEM((DC * PITCH_B, T), U32),
            pltpu.VMEM((DC * PITCH_B, T), U32),
            pltpu.VMEM((NPROD, 2, T, T), BF16),
            pltpu.VMEM((HB, S, T), BF16),
            pltpu.VMEM((S + 16, DM), BF16),
            pltpu.VMEM((16, S, T), BF16),
            pltpu.VMEM((7 * 4 * KT * T, T), U32),
            pltpu.SemaphoreType.DMA((32,)),
        ],
        compiler_params=pltpu.CompilerParams(vmem_limit_bytes=126 * 1024 * 1024),
        name="concat_heads",
    )(A_x.reshape(S, DM), A_wqkv, A_wo, B_x.reshape(S, DM), B_c_kv.reshape(S, DC),
      B_w_q.reshape(16, S, T), B_w_uk.reshape(8, S, T), B_w_uv.reshape(8, S, T),
      B_w_o.reshape(2, S, DM))
    return out.reshape(1, S, 2 * DM)


@jax.jit
def pallas_concat_heads__sliding_local_dilated__compressed_kv_cla__prompt_kernel(
    A_x: jax.Array,
    A_wqkv: jax.Array,
    A_wo: jax.Array,
    B_x: jax.Array,
    B_c_kv: jax.Array,
    B_w_q: jax.Array,
    B_w_uk: jax.Array,
    B_w_uv: jax.Array,
    B_w_o: jax.Array,
):
    return _call(A_x, A_wqkv, A_wo, B_x, B_c_kv, B_w_q, B_w_uk, B_w_uv, B_w_o)
```
